```python
import jax
import jax.numpy as jnp

def _softmax(x, axis=-1):
    return jax.nn.softmax(x, axis=axis)

def _gelu(x):
    return jax.nn.gelu(x, approximate=True)

def _silu(x):
    return jax.nn.silu(x)

def _sigmoid(x):
    return jax.nn.sigmoid(x)

def _layernorm(x, axis=-1, eps=1e-05):
    m = jnp.mean(x, axis=axis, keepdims=True)
    v = jnp.var(x, axis=axis, keepdims=True)
    return (x - m) / jnp.sqrt(v + eps)

def _scatter_add(tgt, idx, src, axis=0):
    return tgt.at[idx].add(src)

def _segment_sum(src, seg, n):
    return jax.ops.segment_sum(src, seg, n)

class _Rng:

    def __init__(self, key):
        self._k = key

    def _next(self):
        self._k, sub = jax.random.split(self._k)
        return sub

    def normal(self, shape):
        return jax.random.normal(self._next(), shape, dtype=jnp.bfloat16)

    def randint(self, lo, hi, shape):
        return jax.random.randint(self._next(), shape, lo, hi, dtype=jnp.int32)

    def uniform(self, shape, lo=0.0, hi=1.0):
        return jax.random.uniform(self._next(), shape, jnp.bfloat16, lo, hi)

    def permutation(self, n):
        return jax.random.permutation(self._next(), n)
kernel_name = 'interleave_layers__memory_aug_recurrent_mem_tr__glu_gated_swiglu__prompt'

def setup_inputs():
    _rng = _Rng(jax.random.key(int.from_bytes(__import__("os").urandom(4), "little")))
    _w = lambda a: (lambda t: t.astype(jnp.bfloat16) if jnp.issubdtype(t.dtype, jnp.floating) else t)(jnp.asarray(a))

    def _A_setup():
        B, S, Dm = (1, 2048, 576)
        H, Dh = (32, 128)
        M, seg = (8, 32)
        seg = min(seg, S)
        S = S // seg * seg
        return {'x': _w((lambda *s: _rng.normal(s) * 0.05)(B, S, Dm)), 'mem0': _w((lambda *s: _rng.normal(s) * 0.05)(B, M, Dm)), 'Wq': _w((lambda *s: _rng.normal(s) * 0.05)(Dm, H, Dh) * Dm ** (-0.5)), 'Wk': _w((lambda *s: _rng.normal(s) * 0.05)(Dm, H, Dh) * Dm ** (-0.5)), 'Wv': _w((lambda *s: _rng.normal(s) * 0.05)(Dm, H, Dh) * Dm ** (-0.5)), 'Wo': _w((lambda *s: _rng.normal(s) * 0.05)(H, Dh, Dm) * (H * Dh) ** (-0.5)), 'seg_len': seg}
    _A_in = _A_setup()

    def _B_setup():
        B, S, D, F = (1, 2048, 576, 4608)
        return {'x': _w((lambda *s: _rng.normal(s) * 0.05)(B, S, D)), 'w1': _w((lambda *s: _rng.normal(s) * 0.05)(D, F) * (2.0 / D) ** 0.5), 'w3': _w((lambda *s: _rng.normal(s) * 0.05)(D, F) * (2.0 / D) ** 0.5), 'w2': _w((lambda *s: _rng.normal(s) * 0.05)(F, D) * (2.0 / F) ** 0.5)}
    _B_in = _B_setup()
    return {'A_x': _A_in['x'], 'A_mem0': _A_in['mem0'], 'A_Wq': _A_in['Wq'], 'A_Wk': _A_in['Wk'], 'A_Wv': _A_in['Wv'], 'A_Wo': _A_in['Wo'], 'A_seg_len': _A_in['seg_len'], 'B_x': _B_in['x'], 'B_w1': _B_in['w1'], 'B_w3': _B_in['w3'], 'B_w2': _B_in['w2']}

def reference(A_x, A_mem0, A_Wq, A_Wk, A_Wv, A_Wo, A_seg_len, B_x, B_w1, B_w3, B_w2):

    def _A_ref(x, mem0, Wq, Wk, Wv, Wo, seg_len):
        B, S, Dm = x.shape
        H, Dh = (Wq.shape[1], Wq.shape[2])
        M = mem0.shape[1]
        scale = Dh ** (-0.5)
        n_seg = S // seg_len
        L = M + seg_len
        idx = jnp.arange(L)
        mask = (idx[:, None] < M) | (idx[:, None] >= idx[None, :])
        mem = mem0
        outs = []
        for s in range(n_seg):
            xs = x[:, s * seg_len:(s + 1) * seg_len, :].copy()
            h = jnp.concatenate([mem, xs], axis=1)
            q = jnp.einsum('btd,dhe->bhte', h, Wq)
            k = jnp.einsum('btd,dhe->bhte', h, Wk)
            v = jnp.einsum('btd,dhe->bhte', h, Wv)
            scores = jnp.einsum('bhqe,bhke->bhqk', q, k) * scale
            scores = jnp.where(mask[None, None], scores, -1000000000.0)
            p = _softmax(scores, axis=-1)
            o = jnp.einsum('bhqk,bhke->bhqe', p, v)
            o = jnp.einsum('bhte,hed->btd', o, Wo)
            mem = o[:, :M, :].copy()
            outs.append(o[:, M:, :])
        return jnp.concatenate(outs, axis=1)

    def _B_ref(x, w1, w3, w2):
        gate = jnp.einsum('bsd,df->bsf', x, w1)
        up = jnp.einsum('bsd,df->bsf', x, w3)
        h = _silu(gate) * up
        out = jnp.einsum('bsf,fd->bsd', h, w2)
        return out
    x = A_x
    x = x + _A_ref(_layernorm(x, axis=-1), A_mem0, A_Wq, A_Wk, A_Wv, A_Wo, A_seg_len)
    x = x + _B_ref(_layernorm(x, axis=-1), B_w1, B_w3, B_w2)
    x = x + _A_ref(_layernorm(x, axis=-1), A_mem0, A_Wq, A_Wk, A_Wv, A_Wo, A_seg_len)
    x = x + _B_ref(_layernorm(x, axis=-1), B_w1, B_w3, B_w2)
    return x
```

```python
import functools
import math

import jax
import jax.numpy as jnp
import jax.experimental.pallas as pl
import jax.experimental.pallas.tpu as pltpu

_EPS = 1e-05
_MASKED = -1000000000.0
_LOG2E = math.log2(math.e)
_LANES = 128
_LAG = 4
_KNOWN = 16
_STAGES = 3

_BLOCKS = ((0, 1, 2, 3), (0, 1, 2, 4))
_SHARED = 5
_CUBE = (({k: k for k in range(4)}, {k: 4 + k for k in range(4)},
          ((0, 1), (0, 2), (0, 3), (3, 1), (3, 2), (2, 1), (2, 3), (1, 2), (1, 3), (3, 0),
           (2, 0), (1, 0))),)
_PAIR = (({0: 0}, {1: 1}, ((0, 1),)), ({2: 0}, {3: 1}, ((2, 3),)))


def _products(covers):
    out, seen = [], []

    for t, ids in enumerate(_BLOCKS):
        for first, second, edges in covers:
            started = []

            def start(kind, k):
                if (kind, k) in started:
                    return
                started.append((kind, k))
                own, other = (first, second) if kind == 0 else (second, first)
                n = own[k]
                if n not in seen:
                    seen.append(n)
                    out.append((((1, None, _SHARED),), ((1, _SHARED, (0, n)),),
                                ((1, None, (0, n)), (1, None, (1, n)))))
                rest = [e[1 - kind] for e in edges if e[kind] == k]
                out.append((((1, 0, ids[k]), (1, 1, ids[k])),
                            ((1, ids[k], (t, n)),) + tuple((-1, ids[k], (t, other[l])) for l in rest),
                            ((1, kind, (t, n)),)))
                out.append((((1, 1 - kind, ids[k]),),
                            ((1, ids[k], (t, n)),) + tuple((-1, ids[l], (t, n)) for l in rest),
                            ((1, 1 - kind, (t, n)), (-1, kind, (t, n)))))

            for k, l in edges:
                start(0, k)
                start(1, l)
                c, d = (t, first[k]), (t, second[l])
                lo, hi = sorted((ids[k], ids[l]))
                out.append((((1, 0, lo), (1, 0, hi)), ((1, ids[k], d),), ((1, 0, c), (1, 0, d))))
                out.append((((1, 1, lo), (1, 1, hi)), ((1, ids[l], c),), ((1, 1, c), (1, 1, d))))
                out.append((((1, 1, ids[k]), (-1, 0, ids[l])), ((1, ids[k], d), (-1, ids[l], c)),
                            ((1, 0, c), (1, 1, d))))
    return out


def _single(covers):
    half = {}
    for first, second, _ in covers:
        half.update({n: 1 for n in first.values()})
        half.update({n: 0 for n in second.values()})
    out = []
    for j, (narrow, _, wide) in enumerate(_products(covers)):
        wide = tuple((s, 0, n) for s, h, n in wide if h in (None, half[n[1]]))
        if wide:
            out.append((j, tuple((s, 0, b) for s, _, b in narrow), wide))
    return out


def _double(covers):
    return [(j, narrow, wide) for j, (narrow, _, wide) in enumerate(_products(covers))]


def _halves(terms):
    if terms[0][1] is None:
        return [tuple((s, h, x) for s, _, x in terms) for h in range(2)]
    return [terms]


def _slots(plan):
    slots = {}
    for _, narrow, _ in plan:
        for terms in _halves(narrow):
            slots.setdefault(terms, len(slots))
    return slots


def _combine(terms, value):
    total = None
    for sign, *key in terms:
        v = value(*key)
        total = v if total is None else total + v if sign > 0 else total - v
    return total


def _scatter(acc, terms, value):
    parts = _halves(terms)
    rows = value.shape[0] // len(parts)
    for i, part in enumerate(parts):
        piece = value if len(parts) == 1 else value[i * rows:(i + 1) * rows]
        for sign, *key in part:
            key = tuple(key)
            if key in acc:
                acc[key] = acc[key] + piece if sign > 0 else acc[key] - piece
            else:
                acc[key] = piece if sign > 0 else -piece


def _stack(parts):
    return parts[0] if len(parts) == 1 else jnp.concatenate(parts, axis=0)


def _expand(plan, lhs, weight, done):
    last = {n: i for i, (_, _, wide) in enumerate(plan) for _, _, n in wide}
    acc = {}
    for i, (j, narrow, wide) in enumerate(plan):
        _scatter(acc, wide, _dot(_stack([lhs(t) for t in _halves(narrow)]), weight(j)))
        for n, at in last.items():
            if at == i:
                done(2 * n[1] + n[0], [acc.pop((h, n)) for h in range(2) if (h, n) in acc])
        yield


def _reduce(plan, tile, weight, acc, dtype):
    for j, narrow, wide in plan:
        lhs = _stack([_combine(t, lambda h, n: tile(h, 2 * n[1] + n[0])) for t in _halves(wide)])
        _scatter(acc, narrow, _dot(lhs.astype(dtype), weight(j)))
        yield


def _split(x):
    cut = 3 * _LANES + _LANES // 2
    tail = x[:, 4 * _LANES:]
    return [x[:, k * _LANES:(k + 1) * _LANES] for k in range(4)] + [
        jnp.concatenate([tail, x[:, cut:4 * _LANES]], axis=1),
        jnp.concatenate([x[:, 3 * _LANES:cut], tail], axis=1)]


def _merge(blocks):
    h = _LANES // 2
    return jnp.concatenate(
        blocks[:3] + [blocks[3] + jnp.concatenate([blocks[5][:, :h], blocks[4][:, h:]], axis=1),
                      blocks[4][:, :h] + blocks[5][:, h:]], axis=1)


def _weight_blocks(raw):
    a, hi, e, end = 3 * _LANES, 3 * _LANES + _LANES // 2, 4 * _LANES, 4 * _LANES + _LANES // 2

    @functools.lru_cache(maxsize=None)
    def block(b, node):
        c, d = 2 * node[1], 2 * node[1] + 1
        if b < 3:
            return raw(c + node[0], b * _LANES, (b + 1) * _LANES)
        if b == 3:
            return _stack([raw(c, a, hi) - raw(d, a, hi), raw(c, hi, e)])
        if b == 4:
            return _stack([raw(d, e, end) - raw(c, e, end), raw(d, hi, e)])
        return _stack([raw(d, a, hi), raw(c, e, end)])

    return block


def _weave(main, side=(), first=0, every=1):
    side = iter(side)
    for i, _ in enumerate(main):
        if i >= first and (i - first) % every == 0:
            next(side, None)
    for _ in side:
        pass


def _take(gen, n):
    for _ in range(n):
        next(gen, None)


def _layernorm(x):
    m = jnp.mean(x, axis=-1, keepdims=True)
    d = x - m
    v = jnp.mean(d * d, axis=-1, keepdims=True)
    return d * jax.lax.rsqrt(v + _EPS)


def _dot(a, b):
    return jax.lax.dot_general(a, b, (((1,), (0,)), ((), ())),
                               preferred_element_type=jnp.float32)


def _dot_nt(a, b):
    return jax.lax.dot_general(a, b, (((1,), (1,)), ((), ())),
                               preferred_element_type=jnp.float32)


def _pack(x):
    return pltpu.bitcast(x, jnp.uint32)


def _unpack(words):
    return pltpu.bitcast(words, jnp.bfloat16)


def _attention_masks(n_layers, n_mem, seg):
    rows = n_layers * (n_mem + seg)
    i = jax.lax.broadcasted_iota(jnp.int32, (rows, rows), 0)
    j = jax.lax.broadcasted_iota(jnp.int32, (rows, rows), 1)
    visible = (i < n_layers * n_mem) | (i >= j)
    if n_layers == 1:
        return visible, _MASKED * _LOG2E

    def second_layer(r):
        return ((r >= n_mem) & (r < 2 * n_mem)) | (r >= 2 * n_mem + seg)

    same = second_layer(i) == second_layer(j)
    fill = jnp.where(same, _MASKED * _LOG2E, -jnp.inf).astype(jnp.float32)
    return same & visible, fill


_GROUP = 16
_N_CUBE = len(_products(_CUBE))
_N_PAIR = len(_products(_PAIR))
_N_FFN = 2 * _N_CUBE + _N_PAIR
_W_OUT = 6 * _N_CUBE
_W_FFN = 8 * _N_CUBE
_SLOTS = _slots(_double(_CUBE))


def _kernel(xt_hbm, mem0_hbm, wq_hbm, wk_hbm, wv_hbm, wot_hbm, w1_hbm, w3_hbm, w2t_hbm,
            outt_hbm, mem0_ref, tile_ref, res_ref, mem_ref, early_lhs_ref, early_ref, lhs_ref,
            up_ref, down_ref, stage_ref, wot_ref, w1_ref, w3_ref, w2t_ref, w_ref,
            stage_sem, weight_sem, tile_sem, *, seg):
    d_model, n_tok = xt_hbm.shape
    n_mem = mem0_ref.shape[0]
    _, n_heads, d_head = wq_hbm.shape
    n_seg = n_tok // seg
    n_pairs = (n_seg - _LAG) // 2
    n_io = n_tok // _LANES
    score_scale = d_head ** -0.5 * _LOG2E

    def block(r, n=1):
        return pl.ds(pl.multiple_of(r * seg, seg), n * seg)

    def stored(base):
        return lambda j: _unpack(w_ref[base + j])

    def built(base, covers, raw, transpose=False):
        products, blocks = _products(covers), _weight_blocks(raw)

        def weight(j):
            tile = _combine(products[j][1], blocks).astype(jnp.bfloat16)
            tile = tile.T if transpose else tile
            w_ref[base + j] = _pack(tile)
            return tile

        return weight

    def store_lhs(ref, halves):
        blocks = [_split(h) for h in halves]
        for terms, slot in _SLOTS.items():
            value = _combine(terms, lambda h, b: blocks[h][b])
            if ref.dtype == jnp.uint32:
                ref[slot] = _pack(value.astype(jnp.bfloat16))
            else:
                ref[slot, :value.shape[0], :] = value

    def transpose_out(i):
        rows = pl.ds(pl.multiple_of(i * _LANES, _LANES), _LANES)
        tile_ref[i] = res_ref[rows, :].T.astype(tile_ref.dtype)

    def attention(n_layers, plan, lhs, arrange):
        visible, fill = _attention_masks(n_layers, n_mem, seg)
        qkv, probs, heads, acc = {}, {}, {}, {}

        def project(which, g):
            def done(i, halves):
                qkv[which, g * _GROUP + i] = arrange(which * n_heads + g * _GROUP + i, halves)

            return _expand(plan, lhs, stored((2 * which + g) * _N_CUBE), done)

        def order(g):
            return [h for w, h in qkv if w == 0 and h // _GROUP == g]

        def scores(g):
            for h in order(g):
                s = jnp.where(visible, _dot_nt(qkv[0, h], qkv[1, h]) * score_scale, fill)
                p = jnp.exp2(s - jnp.max(s, axis=-1, keepdims=True))
                probs[h] = p.astype(jnp.bfloat16), 1.0 / jnp.sum(p, axis=-1, keepdims=True)
                yield

        def values(g):
            for h in order(g):
                o = _dot(probs[h][0], qkv[2, h]) * probs[h][1]
                tokens = n_layers * n_mem
                heads[h] = [_stack([o[i * n_mem:(i + 1) * n_mem],
                                    o[tokens + i * seg:tokens + (i + 1) * seg]])
                            for i in range(n_layers)]
                yield

        def output(g):
            return _reduce(plan, lambda h, i: heads[g * _GROUP + i][h],
                           stored(_W_OUT + g * _N_CUBE), acc, jnp.float32)

        n = len(plan)
        _weave(project(0, 0))
        _weave(project(1, 0))
        _weave(project(2, 0), scores(0), 0, n // 18)
        _weave(project(0, 1), values(0), 0, n // 16)
        _weave(project(1, 1))
        _weave(project(2, 1), scores(1), 0, n // 18)
        _weave(output(0), values(1), 0, n // 20)
        _weave(output(1))
        return [_merge([acc[h, b] for b in range(6)]) for h in range(n_layers)]

    def swiglu(finish, build=False):
        groups = ((_CUBE, 0, 0), (_CUBE, _GROUP, _N_CUBE), (_PAIR, 2 * _GROUP, 2 * _N_CUBE))
        gates, acts, acc = {}, {}, {}

        def weights(which, covers, first, offset):
            base = _W_FFN + which * _N_FFN + offset
            if not build:
                return stored(base)
            ref = (w1_ref, w3_ref, w2t_ref)[which]

            def raw(i, lo, hi):
                cols = slice((first + i) * _LANES, (first + i + 1) * _LANES)
                return _unpack(ref[lo // 2:hi // 2, cols]).astype(jnp.float32)

            return built(base, covers, raw, transpose=which == 2)

        def lhs(terms):
            return _unpack(up_ref[_SLOTS[terms]])

        for covers, first, offset in groups:
            def gate(i, halves, first=first):
                gates[first + i] = [g * jax.nn.sigmoid(g) for g in halves]

            def up(i, halves, first=first):
                acts[first + i] = [g * u for g, u in zip(gates[first + i], halves)]

            yield from _expand(_double(covers), lhs, weights(0, covers, first, offset), gate)
            yield from _expand(_double(covers), lhs, weights(1, covers, first, offset), up)
        for covers, first, offset in groups:
            yield from _reduce(_double(covers), lambda h, i, first=first: acts[first + i][h],
                               weights(2, covers, first, offset), acc, jnp.bfloat16)
        finish([[acc[h, b] for b in range(6)] for h in range(2)])

    def park(blocks):
        for h in range(2):
            for b in range(6):
                down_ref[h, b] = blocks[h][b]

    def parked(h):
        return _merge([down_ref[h, b] for b in range(6)])

    def single_step(r, mem):
        x = res_ref[block(r), :]
        blocks = _split(_stack([mem, _layernorm(x)]))
        lhs = functools.lru_cache(maxsize=None)(lambda terms: _combine(terms, lambda h, b: blocks[b]))
        out, = attention(1, _single(_CUBE), lhs, lambda i, halves: halves[0].astype(jnp.bfloat16))
        res_ref[block(r), :] = x + out[n_mem:]
        return out[:n_mem]

    def double_step(mems, x1, x2, pair=None):
        h2 = _layernorm(x2)
        if pair is None:
            halves = [_stack([mems[0], _layernorm(x1)]), _stack([mems[1], h2])]
        else:
            moved = _KNOWN // 2
            halves = [_stack([mems[0], _layernorm(x1[_KNOWN:]), h2[:moved]]),
                      _stack([mems[1], h2[moved:]])]
        ref = lhs_ref.at[int(pair is None)]
        store_lhs(ref, halves)
        rows = halves[0].shape[0]

        def arrange(i, parts):
            mem = _stack([p[:n_mem] for p in parts])
            tokens = _stack([p[n_mem:] for p in parts])
            if pair is None:
                return _stack([mem, tokens]).astype(jnp.bfloat16)
            words = pl.ds(pl.multiple_of(pair * (_KNOWN // 2), _KNOWN // 2), _KNOWN // 2)
            return _stack([mem.astype(jnp.bfloat16), _unpack(early_ref[i, words, :]),
                           tokens.astype(jnp.bfloat16)])

        def run():
            out = attention(2, _double(_CUBE), lambda t: ref[_SLOTS[t], :rows, :], arrange)
            return [o[:n_mem] for o in out], x1 + out[0][n_mem:], x2 + out[1][n_mem:]

        return run

    def pair_step(j, with_ffn):
        ffn = swiglu(park) if with_ffn else iter(())
        x1 = res_ref[block(2 * j + _LAG, 2), :]
        x2 = res_ref[block(2 * j, 2), :] + parked(0)
        if with_ffn:
            old = block(jnp.maximum(2 * j - _LAG, 0), 2)
            res_ref[old, :] = res_ref[old, :] + parked(1)
            transpose_out(jnp.maximum(j - 3, 0) // 2)
        else:
            down_ref[0] = down_ref[1]
            down_ref[1] = jnp.zeros(down_ref.shape[1:], down_ref.dtype)
        run = double_step([mem_ref[0], mem_ref[1]], x1[:seg], x2[:seg], j)
        _take(ffn, 2 * _N_CUBE)
        mems, a1, a2 = run()
        run = double_step(mems, x1[seg:], x2[seg:])
        _take(ffn, 2 * _N_CUBE + 2 * _N_PAIR)
        mems, b1, b2 = run()
        mem_ref[0], mem_ref[1] = mems
        x1, x2 = _stack([a1, b1]), _stack([a2, b2])
        res_ref[block(2 * j + _LAG, 2), :] = x1
        res_ref[block(2 * j, 2), :] = x2
        store_lhs(up_ref, [_layernorm(x1), _layernorm(x2)])
        _weave(ffn)

    def head_copies(w, g, slot):
        return [pltpu.make_async_copy(w.bitcast(jnp.uint32).at[:, g * _GROUP // 2 + p, :],
                                      stage_ref.at[slot, p], stage_sem.at[slot])
                for p in range(_GROUP // 2)]

    def start(copies):
        for c in copies:
            c.start()

    def start_group(i):
        start(head_copies((wq_hbm, wk_hbm, wv_hbm)[i // 2], i % 2, i % _STAGES))

    x_copies = [pltpu.make_async_copy(xt_hbm.at[:, pl.ds(i * _LANES, _LANES)], tile_ref.at[i],
                                      tile_sem.at[i]) for i in range(n_io)]
    wo_copies = [pltpu.make_async_copy(wot_hbm.bitcast(jnp.uint32), wot_ref, weight_sem.at[0]),
                 pltpu.make_async_copy(mem0_hbm, mem0_ref, weight_sem.at[1])]
    ffn_copies = [
        pltpu.make_async_copy(src.bitcast(jnp.uint32), dst, weight_sem.at[2 + i])
        for i, (src, dst) in enumerate(((w1_hbm, w1_ref), (w3_hbm, w3_ref), (w2t_hbm, w2t_ref)))]
    out_copies = [
        pltpu.make_async_copy(tile_ref.at[i],
                              outt_hbm.at[:, pl.ds(i * _LANES, _LANES)], tile_sem.at[i])
        for i in range(n_io)]

    start(x_copies)
    for c in x_copies[:n_io // 2]:
        c.wait()
    start_group(0)
    for c in x_copies[n_io // 2:]:
        c.wait()
    for i in range(n_io):
        res_ref[i * _LANES:(i + 1) * _LANES, :] = tile_ref[i].astype(jnp.float32).T
    start_group(1)
    known = [res_ref[pl.ds((2 * j + _LAG) * seg, _KNOWN), :] for j in range(n_pairs)]
    store_lhs(early_lhs_ref, [_layernorm(_stack(known[:n_pairs // 2])),
                              _layernorm(_stack(known[n_pairs // 2:]))])

    @pl.loop(0, 6)
    def _load_group(g):
        slot = g % _STAGES
        for i in range(_STAGES - 1, 6):
            pl.when(g + _STAGES - 1 == i)(functools.partial(start_group, i))
        pl.when(g == 3)(lambda: start(wo_copies))
        pl.when(g == 4)(lambda: start(ffn_copies))
        for c in head_copies(wq_hbm, 0, slot):
            c.wait()

        def raw(i, lo, hi):
            words = stage_ref[slot, i // 2, lo:hi, :]
            words = words & jnp.uint32(0xFFFF0000) if i % 2 else words << 16
            return pltpu.bitcast(words, jnp.float32)

        def done(i, halves):
            early_ref[g * _GROUP + i] = _pack(_stack(halves).astype(jnp.bfloat16))

        _weave(_expand(_double(_CUBE), lambda t: _unpack(early_lhs_ref[_SLOTS[t]]),
                       built(g * _N_CUBE, _CUBE, raw), done))

    for c in wo_copies:
        c.wait()

    @pl.loop(0, 2)
    def _build_output(g):
        def raw(i, lo, hi):
            return _unpack(wot_ref[g * _GROUP + i, lo // 2:hi // 2, :]).astype(jnp.float32)

        weight = built(_W_OUT + g * _N_CUBE, _CUBE, raw, transpose=True)
        for j in range(_N_CUBE):
            weight(j)

    mem0 = mem0_ref[...].astype(jnp.float32)
    mem_ref[0] = jax.lax.fori_loop(0, _LAG, single_step, mem0)
    mem_ref[1] = mem0
    for c in ffn_copies:
        c.wait()
    store_lhs(up_ref, [_layernorm(res_ref[block(2 * h, 2), :]) for h in range(2)])
    _weave(swiglu(park, build=True))
    pair_step(0, False)
    pl.loop(1, n_pairs)(functools.partial(pair_step, with_ffn=True))

    last = n_seg - _LAG
    n_done = (n_pairs - 4) // 2 + 1
    start(out_copies[:n_done])
    for h, r in enumerate((last, last - _LAG)):
        res_ref[block(r, 2), :] = res_ref[block(r, 2), :] + parked(h)

    def add(blocks):
        for h, r in enumerate((last + 2, last + 2 - _LAG)):
            res_ref[block(r, 2), :] = res_ref[block(r, 2), :] + _merge(blocks[h])

    _weave(swiglu(add))
    jax.lax.fori_loop(last, n_seg, single_step, mem_ref[1])
    for i in range(n_done, n_io - 1):
        transpose_out(i)
        out_copies[i].start()
    store_lhs(up_ref, [_layernorm(res_ref[block(last + 2 * h, 2), :]) for h in range(2)])

    def emit(blocks):
        y = res_ref[block(last, _LAG), :] + _stack([_merge(b) for b in blocks])
        tile_ref[n_io - 1] = y.T.astype(tile_ref.dtype)

    _weave(swiglu(emit))
    out_copies[n_io - 1].start()
    for c in out_copies:
        c.wait()


@functools.partial(jax.jit, static_argnames=("A_seg_len",))
def pallas_interleave_layers__memory_aug_recurrent_mem_tr__glu_gated_swiglu__prompt_kernel(
    A_x: jax.Array,
    A_mem0: jax.Array,
    A_Wq: jax.Array,
    A_Wk: jax.Array,
    A_Wv: jax.Array,
    A_Wo: jax.Array,
    A_seg_len: int,
    B_x: jax.Array,
    B_w1: jax.Array,
    B_w3: jax.Array,
    B_w2: jax.Array,
):
    del B_x
    _, n_tok, d_model = A_x.shape
    n_mem = A_mem0.shape[1]
    _, n_heads, d_head = A_Wq.shape
    d_ff = B_w1.shape[1]
    seg = A_seg_len
    n_known = (n_tok // seg - _LAG) // 2 * _KNOWN
    hbm = pl.BlockSpec(memory_space=pltpu.HBM)
    out_t = pl.pallas_call(
        functools.partial(_kernel, seg=seg),
        out_shape=jax.ShapeDtypeStruct((d_model, n_tok), A_x.dtype),
        in_specs=[hbm] * 9,
        out_specs=hbm,
        scratch_shapes=[
            pltpu.VMEM((n_mem, d_model), A_mem0.dtype),
            pltpu.VMEM((n_tok // _LANES, d_model, _LANES), A_x.dtype),
            pltpu.VMEM((n_tok, d_model), jnp.float32),
            pltpu.VMEM((2, n_mem, d_model), jnp.float32),
            pltpu.VMEM((len(_SLOTS), n_known // 4, _LANES), jnp.uint32),
            pltpu.VMEM((3 * n_heads, n_known // 2, d_head), jnp.uint32),
            pltpu.VMEM((2, len(_SLOTS), n_mem + seg, _LANES), jnp.float32),
            pltpu.VMEM((len(_SLOTS), seg, _LANES), jnp.uint32),
            pltpu.VMEM((2, 6, 2 * seg, _LANES), jnp.float32),
            pltpu.VMEM((_STAGES, _GROUP // 2, d_model, d_head), jnp.uint32),
            pltpu.VMEM((n_heads, d_model // 2, d_head), jnp.uint32),
            pltpu.VMEM((d_model // 2, d_ff), jnp.uint32),
            pltpu.VMEM((d_model // 2, d_ff), jnp.uint32),
            pltpu.VMEM((d_model // 2, d_ff), jnp.uint32),
            pltpu.VMEM((_W_FFN + 3 * _N_FFN, _LANES // 2, _LANES), jnp.uint32),
            pltpu.SemaphoreType.DMA((_STAGES,)),
            pltpu.SemaphoreType.DMA((5,)),
            pltpu.SemaphoreType.DMA((n_tok // _LANES,)),
        ],
        compiler_params=pltpu.CompilerParams(vmem_limit_bytes=120 * 1024 * 1024),
    )(A_x.reshape(n_tok, d_model).T, A_mem0.reshape(n_mem, d_model), A_Wq, A_Wk, A_Wv,
      A_Wo.transpose(0, 2, 1), B_w1, B_w3, B_w2.T)
    return out_t.T.reshape(A_x.shape)
```

```python
import functools
import math

import jax
import jax.numpy as jnp
import jax.experimental.pallas as pl
import jax.experimental.pallas.tpu as pltpu

_EPS = 1e-05
_MASKED = -1000000000.0
_LOG2E = math.log2(math.e)
_LANES = 128
_LAG = 4
_KNOWN = 16
_STAGES = 3
_ONLY = None
_F1, _F2, _F3, _SPILL = 48, 200, 48, 60
_EARLY_DTYPE = jnp.bfloat16

_BLOCKS = ((0, 1, 2, 3), (0, 1, 2, 4))
_SHARED = 5
_CUBE = (({k: k for k in range(4)}, {k: 4 + k for k in range(4)},
          ((0, 1), (0, 2), (0, 3), (3, 1), (3, 2), (2, 1), (2, 3), (1, 2), (1, 3), (3, 0),
           (2, 0), (1, 0))),)
_PAIR = (({0: 0}, {1: 1}, ((0, 1),)), ({2: 0}, {3: 1}, ((2, 3),)))


def _products(covers):
    out, seen = [], []

    for t, ids in enumerate(_BLOCKS):
        for first, second, edges in covers:
            started = []

            def start(kind, k):
                if (kind, k) in started:
                    return
                started.append((kind, k))
                own, other = (first, second) if kind == 0 else (second, first)
                n = own[k]
                if n not in seen:
                    seen.append(n)
                    out.append((((1, None, _SHARED),), ((1, _SHARED, (0, n)),),
                                ((1, None, (0, n)), (1, None, (1, n)))))
                rest = [e[1 - kind] for e in edges if e[kind] == k]
                out.append((((1, 0, ids[k]), (1, 1, ids[k])),
                            ((1, ids[k], (t, n)),) + tuple((-1, ids[k], (t, other[l])) for l in rest),
                            ((1, kind, (t, n)),)))
                out.append((((1, 1 - kind, ids[k]),),
                            ((1, ids[k], (t, n)),) + tuple((-1, ids[l], (t, n)) for l in rest),
                            ((1, 1 - kind, (t, n)), (-1, kind, (t, n)))))

            for k, l in edges:
                start(0, k)
                start(1, l)
                c, d = (t, first[k]), (t, second[l])
                lo, hi = sorted((ids[k], ids[l]))
                out.append((((1, 0, lo), (1, 0, hi)), ((1, ids[k], d),), ((1, 0, c), (1, 0, d))))
                out.append((((1, 1, lo), (1, 1, hi)), ((1, ids[l], c),), ((1, 1, c), (1, 1, d))))
                out.append((((1, 1, ids[k]), (-1, 0, ids[l])), ((1, ids[k], d), (-1, ids[l], c)),
                            ((1, 0, c), (1, 1, d))))
    return out


def _single(covers):
    half = {}
    for first, second, _ in covers:
        half.update({n: 1 for n in first.values()})
        half.update({n: 0 for n in second.values()})
    out = []
    for j, (narrow, _, wide) in enumerate(_products(covers)):
        wide = tuple((s, 0, n) for s, h, n in wide if h in (None, half[n[1]]))
        if wide:
            out.append((j, tuple((s, 0, b) for s, _, b in narrow), wide))
    return out


def _double(covers):
    return [(j, narrow, wide) for j, (narrow, _, wide) in enumerate(_products(covers))]


def _halves(terms):
    if terms[0][1] is None:
        return [tuple((s, h, x) for s, _, x in terms) for h in range(2)]
    return [terms]


def _slots(plan):
    slots = {}
    for _, narrow, _ in plan:
        for terms in _halves(narrow):
            slots.setdefault(terms, len(slots))
    return slots


def _combine(terms, value):
    total = None
    for sign, *key in terms:
        v = value(*key)
        total = v if total is None else total + v if sign > 0 else total - v
    return total


def _scatter(acc, terms, value):
    parts = _halves(terms)
    rows = value.shape[0] // len(parts)
    for i, part in enumerate(parts):
        piece = value if len(parts) == 1 else value[i * rows:(i + 1) * rows]
        for sign, *key in part:
            key = tuple(key)
            if key in acc:
                acc[key] = acc[key] + piece if sign > 0 else acc[key] - piece
            else:
                acc[key] = piece if sign > 0 else -piece


def _stack(parts):
    return parts[0] if len(parts) == 1 else jnp.concatenate(parts, axis=0)


def _expand(plan, lhs, weight, done):
    last = {n: i for i, (_, _, wide) in enumerate(plan) for _, _, n in wide}
    acc = {}
    for i, (j, narrow, wide) in enumerate(plan):
        _scatter(acc, wide, _dot(_stack([lhs(t) for t in _halves(narrow)]), weight(j)))
        for n, at in last.items():
            if at == i:
                done(2 * n[1] + n[0], [acc.pop((h, n)) for h in range(2) if (h, n) in acc])
        yield


def _reduce(plan, tile, weight, acc, dtype):
    for j, narrow, wide in plan:
        lhs = _stack([_combine(t, lambda h, n: tile(h, 2 * n[1] + n[0])) for t in _halves(wide)])
        _scatter(acc, narrow, _dot(lhs.astype(dtype), weight(j)))
        yield


def _split(x):
    cut = 3 * _LANES + _LANES // 2
    tail = x[:, 4 * _LANES:]
    return [x[:, k * _LANES:(k + 1) * _LANES] for k in range(4)] + [
        jnp.concatenate([tail, x[:, cut:4 * _LANES]], axis=1),
        jnp.concatenate([x[:, 3 * _LANES:cut], tail], axis=1)]


def _merge(blocks):
    h = _LANES // 2
    return jnp.concatenate(
        blocks[:3] + [blocks[3] + jnp.concatenate([blocks[5][:, :h], blocks[4][:, h:]], axis=1),
                      blocks[4][:, :h] + blocks[5][:, h:]], axis=1)


def _weight_blocks(raw):
    a, hi, e, end = 3 * _LANES, 3 * _LANES + _LANES // 2, 4 * _LANES, 4 * _LANES + _LANES // 2

    @functools.lru_cache(maxsize=None)
    def block(b, node):
        c, d = 2 * node[1], 2 * node[1] + 1
        if b < 3:
            return raw(c + node[0], b * _LANES, (b + 1) * _LANES)
        if b == 3:
            return _stack([raw(c, a, hi) - raw(d, a, hi), raw(c, hi, e)])
        if b == 4:
            return _stack([raw(d, e, end) - raw(c, e, end), raw(d, hi, e)])
        return _stack([raw(d, a, hi), raw(c, e, end)])

    return block


def _weave(main, side=(), first=0, every=1):
    side = iter(side)
    for i, _ in enumerate(main):
        if i >= first and (i - first) % every == 0:
            next(side, None)
    for _ in side:
        pass


def _take(gen, n):
    for _ in range(n):
        next(gen, None)


def _chain(*gens):
    for gen in gens:
        yield from gen


def _first(gen, n):
    for _ in range(n):
        yield next(gen, None)


def _layernorm(x):
    m = jnp.mean(x, axis=-1, keepdims=True)
    d = x - m
    v = jnp.mean(d * d, axis=-1, keepdims=True)
    return d * jax.lax.rsqrt(v + _EPS)


def _reciprocal(x):
    return pltpu.reciprocal(x, approx=True)


def _dot(a, b):
    return jax.lax.dot_general(a, b, (((1,), (0,)), ((), ())),
                               preferred_element_type=jnp.float32)


def _dot_nt(a, b):
    return jax.lax.dot_general(a, b, (((1,), (1,)), ((), ())),
                               preferred_element_type=jnp.float32)


def _pack(x):
    return pltpu.bitcast(x, jnp.uint32)


def _unpack(words):
    return pltpu.bitcast(words, jnp.bfloat16)


def _attention_masks(n_layers, n_mem, seg):
    rows = n_layers * (n_mem + seg)
    i = jax.lax.broadcasted_iota(jnp.int32, (rows, rows), 0)
    j = jax.lax.broadcasted_iota(jnp.int32, (rows, rows), 1)
    visible = (i < n_layers * n_mem) | (i >= j)
    if n_layers == 1:
        return visible, _MASKED * _LOG2E

    def second_layer(r):
        return ((r >= n_mem) & (r < 2 * n_mem)) | (r >= 2 * n_mem + seg)

    same = second_layer(i) == second_layer(j)
    fill = jnp.where(same, _MASKED * _LOG2E, -jnp.inf).astype(jnp.float32)
    return same & visible, fill


_GROUP = 16
_N_CUBE = len(_products(_CUBE))
_N_PAIR = len(_products(_PAIR))
_N_FFN = 2 * _N_CUBE + _N_PAIR
_W_OUT = 6 * _N_CUBE
_W_FFN = 8 * _N_CUBE
_SLOTS = _slots(_double(_CUBE))


def _kernel(xt_hbm, mem0_hbm, wq_hbm, wk_hbm, wv_hbm, wot_hbm, w1_hbm, w3_hbm, w2t_hbm,
            outt_hbm, mem0_ref, tile_ref, res_ref, early_lhs_ref, early_ref, act_ref,
            out_ref, stage_ref, wot_ref, w1_ref, w3_ref, w2t_ref, w_ref,
            stage_sem, weight_sem, tile_sem, *, seg):
    d_model, n_tok = xt_hbm.shape
    n_mem = mem0_ref.shape[0]
    _, n_heads, d_head = wq_hbm.shape
    n_seg = n_tok // seg
    n_pairs = (n_seg - _LAG) // 2
    n_io = n_tok // _LANES
    score_scale = d_head ** -0.5 * _LOG2E

    def block(r, n=1):
        return pl.ds(pl.multiple_of(r * seg, seg), n * seg)

    def stored(base):
        return lambda j: _unpack(w_ref[base + j])

    def built(base, covers, raw, transpose=False):
        products, blocks = _products(covers), _weight_blocks(raw)

        def weight(j):
            tile = _combine(products[j][1], blocks).astype(jnp.bfloat16)
            tile = tile.T if transpose else tile
            w_ref[base + j] = _pack(tile)
            return tile

        return weight

    def operands(halves, dtype):
        blocks = [_split(h) for h in halves]
        return functools.lru_cache(maxsize=None)(
            lambda terms: _combine(terms, lambda h, b: blocks[h][b]).astype(dtype))

    def transpose_out(i):
        rows = pl.ds(pl.multiple_of(i * _LANES, _LANES), _LANES)
        tile_ref[i] = res_ref[rows, :].T.astype(tile_ref.dtype)

    def attention(n_layers, plan, lhs, arrange, filler=None, n_filler=0):
        visible, fill = _attention_masks(n_layers, n_mem, seg)
        qkv, probs, heads, acc = {}, {}, {}, {}

        def project(which, g):
            def done(i, halves):
                qkv[which, g * _GROUP + i] = arrange(which * n_heads + g * _GROUP + i, halves)

            return _expand(plan, lhs, stored((2 * which + g) * _N_CUBE), done)

        def order(g):
            return [h for w, h in qkv if w == 0 and h // _GROUP == g]

        def scores(g):
            for h in order(g):
                s = jnp.where(visible, _dot_nt(qkv[0, h], qkv[1, h]) * score_scale, fill)
                p = jnp.exp2(s - jnp.max(s, axis=-1, keepdims=True))
                p = p * _reciprocal(jnp.sum(p, axis=-1, keepdims=True))
                probs[h] = p.astype(jnp.bfloat16)
                yield

        def values(g):
            for h in order(g):
                o = _dot(probs[h], qkv[2, h])
                tokens = n_layers * n_mem
                heads[h] = [_stack([o[i * n_mem:(i + 1) * n_mem],
                                    o[tokens + i * seg:tokens + (i + 1) * seg]])
                            for i in range(n_layers)]
                yield

        def output(g):
            return _reduce(plan, lambda h, i: heads[g * _GROUP + i][h],
                           stored(_W_OUT + g * _N_CUBE), acc, jnp.float32)

        n = len(plan)
        _weave(project(0, 0))
        _weave(project(1, 0))
        _weave(_chain(project(0, 1), project(1, 1)), scores(0), 0, n // 8)
        if filler:
            _weave(_chain(project(2, 0), project(2, 1)), scores(1), 0, n // 8)
            _weave(_chain(_first(filler, n_filler), output(0)), _chain(values(0), values(1)), 0,
                   (n_filler + _SPILL) // n_heads)
        else:
            _weave(project(2, 0), scores(1), 0, n // 16)
            _weave(project(2, 1), values(0), 0, n // 18)
            _weave(output(0), values(1), 0, n // 20)
        _weave(output(1))
        return [[acc[h, b] for b in range(6)] for h in range(n_layers)]

    groups = ((_CUBE, 0, 0), (_CUBE, _GROUP, _N_CUBE), (_PAIR, 2 * _GROUP, 2 * _N_CUBE))

    def ffn_weights(which, build, covers, first, offset):
        base = _W_FFN + which * _N_FFN + offset
        if not build:
            return stored(base)
        ref = (w1_ref, w3_ref, w2t_ref)[which]

        def raw(i, lo, hi):
            cols = slice((first + i) * _LANES, (first + i + 1) * _LANES)
            return _unpack(ref[lo // 2:hi // 2, cols]).astype(jnp.float32)

        return built(base, covers, raw, transpose=which == 2)

    def gated(halves, build=False):
        lhs = operands([_layernorm(x) for x in halves], jnp.bfloat16)
        gates = {}
        for covers, first, offset in groups:
            def gate(i, halves):
                gates[i] = [g * _reciprocal(1.0 + jnp.exp2(g * -_LOG2E)) for g in halves]

            def up(i, halves):
                for h in range(2):
                    act_ref[first + i, h] = gates[i][h] * halves[h]

            for which, done in enumerate((gate, up)):
                yield from _expand(_double(covers), lhs,
                                   ffn_weights(which, build, covers, first, offset), done)

    def down(build=False):
        acc = {}
        for covers, first, offset in groups:
            _weave(_reduce(_double(covers), lambda h, i: act_ref[first + i, h],
                           ffn_weights(2, build, covers, first, offset), acc, jnp.bfloat16))
        return [_merge([acc[h, b] for b in range(6)]) for h in range(2)]

    def single_step(r, mem):
        x = res_ref[block(r), :]
        lhs = operands([_stack([mem, _layernorm(x)])], jnp.float32)
        out = _merge(*attention(1, _single(_CUBE), lhs,
                                lambda i, halves: halves[0].astype(jnp.bfloat16)))
        res_ref[block(r), :] = x + out[n_mem:]
        return out[:n_mem]

    def double_step(filler, n_filler, mems, x1, x2, pair=None):
        h2 = _layernorm(x2)
        if pair is None:
            halves = [_stack([mems[0], _layernorm(x1)]), _stack([mems[1], h2])]
        else:
            moved = _KNOWN // 2
            halves = [_stack([mems[0], _layernorm(x1[_KNOWN:]), h2[:moved]]),
                      _stack([mems[1], h2[moved:]])]

        def arrange(i, parts):
            mem = _stack([p[:n_mem] for p in parts])
            tokens = _stack([p[n_mem:] for p in parts])
            if pair is None:
                return _stack([mem, tokens]).astype(jnp.bfloat16)
            words = pl.ds(pl.multiple_of(pair * (_KNOWN // 2), _KNOWN // 2), _KNOWN // 2)
            return _unpack(_stack([_pack(mem.astype(jnp.bfloat16)), early_ref[i, words, :],
                                   _pack(tokens.astype(jnp.bfloat16))]))

        dtype = jnp.float32 if pair is None else _EARLY_DTYPE
        return attention(2, _double(_CUBE), operands(halves, dtype), arrange, filler, n_filler)

    def pair_step(j, mems, x2, ffn=None):
        x1 = res_ref[block(2 * j + _LAG, 2), :]
        out = [_merge(b) for b in double_step(ffn, _F2, mems, x1[:seg], x2[:seg], j)]
        res_ref[block(2 * j + _LAG), :] = x1[:seg] + out[0][n_mem:]
        res_ref[block(2 * j), :] = x2[:seg] + out[1][n_mem:]
        res_ref[block(2 * j + 1), :] = x2[seg:]
        if ffn:
            _take(ffn, _F3)
        blocks = double_step(ffn, 2 * _N_FFN - _F1 - _F2 - _F3, [o[:n_mem] for o in out],
                             x1[seg:], x2[seg:])
        for h in range(2):
            for b in range(6):
                out_ref[h, b] = blocks[h][b]

    def finish_pair(j):
        out = [_merge([out_ref[h, b] for b in range(6)]) for h in range(2)]
        xs = []
        for r, o in zip((2 * j + _LAG, 2 * j), out):
            x = res_ref[block(r, 2), :]
            xs.append(_stack([x[:seg], x[seg:] + o[n_mem:]]))
        for r, x in zip((2 * j + _LAG, 2 * j), xs):
            res_ref[block(r + 1), :] = x[seg:]
        return [o[:n_mem] for o in out], xs

    def steady(j):
        mems, xs = finish_pair(j - 1)
        y = down()
        x2 = res_ref[block(2 * j, 2), :] + y[0]
        old = block(2 * j - _LAG, 2)
        res_ref[old, :] = res_ref[old, :] + y[1]
        transpose_out(jnp.maximum(j - 3, 0) // 2)
        ffn = gated(xs)
        _take(ffn, _F1)
        pair_step(j, mems, x2, ffn)

    def head_copies(w, g, slot):
        return [pltpu.make_async_copy(w.bitcast(jnp.uint32).at[:, g * _GROUP // 2 + p, :],
                                      stage_ref.at[slot, p], stage_sem.at[slot])
                for p in range(_GROUP // 2)]

    def start(copies):
        for c in copies:
            c.start()

    def start_group(i):
        start(head_copies((wq_hbm, wk_hbm, wv_hbm)[i // 2], i % 2, i % _STAGES))

    x_copies = [pltpu.make_async_copy(xt_hbm.at[:, pl.ds(i * _LANES, _LANES)], tile_ref.at[i],
                                      tile_sem.at[i]) for i in range(n_io)]
    wo_copies = [pltpu.make_async_copy(wot_hbm.bitcast(jnp.uint32), wot_ref, weight_sem.at[0]),
                 pltpu.make_async_copy(mem0_hbm, mem0_ref, weight_sem.at[1])]
    ffn_copies = [
        pltpu.make_async_copy(src.bitcast(jnp.uint32), dst, weight_sem.at[2 + i])
        for i, (src, dst) in enumerate(((w1_hbm, w1_ref), (w3_hbm, w3_ref), (w2t_hbm, w2t_ref)))]
    out_copies = [
        pltpu.make_async_copy(tile_ref.at[i],
                              outt_hbm.at[:, pl.ds(i * _LANES, _LANES)], tile_sem.at[i])
        for i in range(n_io)]

    if _ONLY == "pair":
        pl.loop(2, n_pairs)(steady)
        out_copies[0].start()
        out_copies[0].wait()
        return
    start(x_copies)
    for c in x_copies[:n_io // 2]:
        c.wait()
    start_group(0)
    for c in x_copies[n_io // 2:]:
        c.wait()
    for i in range(n_io):
        res_ref[i * _LANES:(i + 1) * _LANES, :] = tile_ref[i].astype(jnp.float32).T
    start_group(1)
    known = [res_ref[pl.ds((2 * j + _LAG) * seg, _KNOWN), :] for j in range(n_pairs)]
    lhs = operands([_layernorm(_stack(known[:n_pairs // 2])),
                    _layernorm(_stack(known[n_pairs // 2:]))], jnp.bfloat16)
    for terms, slot in _SLOTS.items():
        early_lhs_ref[slot] = _pack(lhs(terms))

    @pl.loop(0, 6)
    def _load_group(g):
        slot = g % _STAGES
        for i in range(_STAGES - 1, 6):
            pl.when(g + _STAGES - 1 == i)(functools.partial(start_group, i))
        pl.when(g == 3)(lambda: start(wo_copies))
        pl.when(g == 4)(lambda: start(ffn_copies))
        for c in head_copies(wq_hbm, 0, slot):
            c.wait()

        def raw(i, lo, hi):
            words = stage_ref[slot, i // 2, lo:hi, :]
            words = words & jnp.uint32(0xFFFF0000) if i % 2 else words << 16
            return pltpu.bitcast(words, jnp.float32)

        def done(i, halves):
            early_ref[g * _GROUP + i] = _pack(_stack(halves).astype(jnp.bfloat16))

        _weave(_expand(_double(_CUBE), lambda t: _unpack(early_lhs_ref[_SLOTS[t]]),
                       built(g * _N_CUBE, _CUBE, raw), done))

    for c in wo_copies:
        c.wait()

    @pl.loop(0, 2)
    def _build_output(g):
        def raw(i, lo, hi):
            return _unpack(wot_ref[g * _GROUP + i, lo // 2:hi // 2, :]).astype(jnp.float32)

        weight = built(_W_OUT + g * _N_CUBE, _CUBE, raw, transpose=True)
        for j in range(_N_CUBE):
            weight(j)

    mem0 = mem0_ref[...].astype(jnp.float32)
    mem1 = jax.lax.fori_loop(0, _LAG, single_step, mem0)
    for c in ffn_copies:
        c.wait()
    xs = [res_ref[block(2 * h, 2), :] for h in range(2)]
    _weave(gated(xs, build=True))
    xs = [x + y for x, y in zip(xs, down(build=True))]
    pair_step(0, [mem1, mem0], xs[0])
    mems, ready = finish_pair(0)
    ffn = gated(ready)
    _take(ffn, _F1)
    pair_step(1, mems, xs[1], ffn)
    pl.loop(2, n_pairs)(steady)

    last = n_seg - _LAG
    n_done = (n_pairs - 4) // 2 + 1
    start(out_copies[:n_done])
    mems, xs = finish_pair(n_pairs - 1)
    for r, y in zip((last, last - _LAG), down()):
        res_ref[block(r, 2), :] = res_ref[block(r, 2), :] + y
    _weave(gated(xs))
    for r, x, y in zip((last + 2, last + 2 - _LAG), xs, down()):
        res_ref[block(r, 2), :] = x + y
    jax.lax.fori_loop(last, n_seg, single_step, mems[1])
    for i in range(n_done, n_io - 1):
        transpose_out(i)
        out_copies[i].start()
    xs = [res_ref[block(last + 2 * h, 2), :] for h in range(2)]
    _weave(gated(xs))
    tile_ref[n_io - 1] = (_stack(xs) + _stack(down())).T.astype(tile_ref.dtype)
    out_copies[n_io - 1].start()
    for c in out_copies:
        c.wait()


@functools.partial(jax.jit, static_argnames=("A_seg_len",))
def pallas_interleave_layers__memory_aug_recurrent_mem_tr__glu_gated_swiglu__prompt_kernel(
    A_x: jax.Array,
    A_mem0: jax.Array,
    A_Wq: jax.Array,
    A_Wk: jax.Array,
    A_Wv: jax.Array,
    A_Wo: jax.Array,
    A_seg_len: int,
    B_x: jax.Array,
    B_w1: jax.Array,
    B_w3: jax.Array,
    B_w2: jax.Array,
):
    del B_x
    _, n_tok, d_model = A_x.shape
    n_mem = A_mem0.shape[1]
    _, n_heads, d_head = A_Wq.shape
    d_ff = B_w1.shape[1]
    seg = A_seg_len
    n_known = (n_tok // seg - _LAG) // 2 * _KNOWN
    hbm = pl.BlockSpec(memory_space=pltpu.HBM)
    out_t = pl.pallas_call(
        functools.partial(_kernel, seg=seg),
        out_shape=jax.ShapeDtypeStruct((d_model, n_tok), A_x.dtype),
        in_specs=[hbm] * 9,
        out_specs=hbm,
        scratch_shapes=[
            pltpu.VMEM((n_mem, d_model), A_mem0.dtype),
            pltpu.VMEM((n_tok // _LANES, d_model, _LANES), A_x.dtype),
            pltpu.VMEM((n_tok, d_model), jnp.float32),
            pltpu.VMEM((len(_SLOTS), n_known // 4, _LANES), jnp.uint32),
            pltpu.VMEM((3 * n_heads, n_known // 2, d_head), jnp.uint32),
            pltpu.VMEM((d_ff // _LANES, 2, 2 * seg, _LANES), jnp.float32),
            pltpu.VMEM((2, 6, n_mem + seg, _LANES), jnp.float32),
            pltpu.VMEM((_STAGES, _GROUP // 2, d_model, d_head), jnp.uint32),
            pltpu.VMEM((n_heads, d_model // 2, d_head), jnp.uint32),
            pltpu.VMEM((d_model // 2, d_ff), jnp.uint32),
            pltpu.VMEM((d_model // 2, d_ff), jnp.uint32),
            pltpu.VMEM((d_model // 2, d_ff), jnp.uint32),
            pltpu.VMEM((_W_FFN + 3 * _N_FFN, _LANES // 2, _LANES), jnp.uint32),
            pltpu.SemaphoreType.DMA((_STAGES,)),
            pltpu.SemaphoreType.DMA((5,)),
            pltpu.SemaphoreType.DMA((n_tok // _LANES,)),
        ],
        compiler_params=pltpu.CompilerParams(vmem_limit_bytes=120 * 1024 * 1024),
    )(A_x.reshape(n_tok, d_model).T, A_mem0.reshape(n_mem, d_model), A_Wq, A_Wk, A_Wv,
      A_Wo.transpose(0, 2, 1), B_w1, B_w3, B_w2.T)
    return out_t.T.reshape(A_x.shape)
```

```python
import functools
import itertools
import math

import jax
import jax.numpy as jnp
import jax.experimental.pallas as pl
import jax.experimental.pallas.tpu as pltpu
import numpy as np

_EPS = 1e-05
_MASKED = -1000000000.0
_LOG2E = math.log2(math.e)
_LANES = 128
_UNIT = _LANES // 2
_UNITS = 9
_MXUS = 4
_LAG = 4
_KNOWN = 16
_ONLY = None
_FLAGS = None
_D0, _F0, _F1, _F2, _F3 = 100, 40, 71, 160, 72
_LEAD, _SPILL, _FIRST = 72, 40, 19
_LEAD_B, _SPILL_B = 72, 40
_CHORES, _AHEAD, _W2_RATE = (0.6, 1.4, 0.6, 0.8), 30, 0.5
_PIN = 1
_X_CUTS = (0, 5, 10, 14, 16)
_Q_CUTS = (0, 4, 8, 12, 16)
_WO_START, _WO_AT = 80, 128


class _Scheme:
    def __init__(self, period, blocks, links, orient=tuple, late=True, first=()):
        links = [tuple((orbit, (s + shift) % period) for orbit, shift in link)
                 for s in range(period) for link in links]
        nodes = list(dict.fromkeys([*first] + [node for link in links for node in link]))
        self.nodes = nodes
        links = [tuple(nodes.index(node) for node in link) for link in links]
        kinds = [orbit // 2 for orbit, _ in nodes]
        self.blocks = [orient([u if u >= period else (u + s) % period for u in blocks[orbit]])
                       for orbit, s in nodes]
        cells, products = [], {}

        def form(side, v, p):
            if len(v) > (2 if p == 2 else 1):
                key = ((1, form(side, v[:-1], p)[1]), (1, form(side, v[-1:], p)[1]))
            elif p == 2:
                key = ((1, form(side, v, 0)[1]), (1 - 2 * side, form(side, v, 1)[1]))
            else:
                key = (p, self.blocks[v[0]]) if side == 0 else (1 - p, v[0])
            return (-1 if p == 2 * (1 - side) else 1), key

        def use(narrow, wide, sign):
            weight = products.setdefault((narrow[1], wide[1]), {})
            weight[len(cells) - 1] = sign * narrow[0] * wide[0]

        def square(v, p, q, sign):
            use(form(0, v, p), form(1, v, q), sign)

        def cross(u, v, both, p):
            q, r = (p + 1) % 3, (p + 2) % 3
            mixed = []
            for side in range(2):
                (s, a), (t, b) = form(side, u, q), form(side, v, p)
                mixed.append((s, ((1, a), (-s * t, b))))
            cells.append((u, v))
            square(both, p, q, 1), square(u, r, q, 1), square(v, p, r, 1), use(*mixed, 1)
            cells.append((v, u))
            square(both, q, p, -1), square(u, q, r, -1), square(v, r, p, -1), use(*mixed, -1)

        for link in links:
            for x in link:
                if ((x,), (x,)) not in cells:
                    cells.append(((x,), (x,)))
                    square((x,), (kinds[x] + 1) % 3, (kinds[x] + 2) % 3, 1)
                    square((x,), (kinds[x] + 2) % 3, (kinds[x] + 1) % 3, -1)
            cross(link[:1], link[1:2], link[:2], 0)
            if len(link) == 3 and kinds[link[2]]:
                cross(link[2:], link[:2], link, 1)
            elif len(link) == 3:
                cross(link[:2], link[2:], link, 2)
        if late:
            products = dict(sorted(products.items(), key=lambda item: max(item[1])))
        self.double = [(j, narrow, wide) for j, (narrow, wide) in enumerate(products)]

        sums = list(products.values())
        own = [products[form(0, (x,), 1 - kinds[x])[1], form(1, (x,), 2)[1]]
               for x in range(len(nodes))]
        self.single = []
        for j, (rows, cols) in enumerate(cells):
            weight = own[rows[0]] if rows == cols else {j: -1} if {j: -1} in sums else {j: 1}
            if weight not in sums:
                sums.append(weight)
            if rows != cols:
                rows, cols = (rows + cols[:len(cols) == 1 and j in own[cols[0]]],
                              cols + rows[:len(rows) == 1 and j in own[rows[0]]])
            self.single.append((sums.index(weight), form(0, rows, 0)[1],
                                ((weight[j], form(1, cols, 1)[1]),)))

        basis = np.zeros((_UNITS, len(nodes), len(cells), 2))
        for j, (rows, cols) in enumerate(cells):
            for x, y, lane in itertools.product(rows, cols, range(2)):
                basis[self.blocks[x][lane], y, j, lane] += 1
        inverse = np.rint(np.linalg.inv(basis.reshape(2 * len(cells), -1))).reshape(
            len(cells), 2, _UNITS, -1)
        raw = [[_sum((int(lane[u, x]), (int(u), int(x))) for u, x in np.argwhere(lane))
                for lane in cell] for cell in inverse]
        self.weights = [[_sum((sign, raw[j][lane]) for j, sign in weight.items())
                         for lane in range(2)] for weight in sums]
        self.places = sorted({(u, lane) for b in self.blocks for lane, u in enumerate(b)})


def _sum(terms):
    terms = sorted(terms, key=lambda term: -term[0])
    return terms[0][1] if len(terms) == 1 and terms[0][0] == 1 else tuple(terms)


def _is_leaf(key):
    return isinstance(key[0], int)


def _leaves(key):
    return [key] if _is_leaf(key) else [leaf for _, term in key for leaf in _leaves(term)]


def _add(total, sign, value):
    if total is None:
        return value if sign > 0 else -value
    return total + value if sign > 0 else total - value


def _gather(leaf):
    @functools.lru_cache(maxsize=None)
    def value(key):
        if _is_leaf(key):
            return leaf(*key)
        total = None
        for sign, term in key:
            total = _add(total, sign, value(term))
        return total

    return value


def _scatter(keys, done):
    missing, totals = {}, {}

    def count(key):
        missing[key] = missing.get(key, 0) + 1
        if missing[key] == 1 and not _is_leaf(key):
            for _, term in key:
                count(term)

    def add(key, value, sign=1):
        if key in totals:
            old_sign, old = totals[key]
            if old_sign >= sign:
                sign, value = old_sign, _add(old, sign * old_sign, value)
            else:
                value = value - old
        totals[key] = sign, value
        missing[key] -= 1
        if missing[key]:
            return
        if _is_leaf(key):
            done(*key, _add(None, sign, value))
        else:
            for factor, term in key:
                add(term, value, sign * factor)

    for key in keys:
        count(key)
    return add


def _by_parity(block):
    low, high = sorted(block)
    if high == _UNITS - 1:
        return (high, low) if low % 2 else (low, high)
    return (low, high) if high % 2 else (high, low)


_H8 = (8, ((7, 0), (7, 3), (8, 6), (5, 6)),
                 (((0, 6), (2, 6), (0, 3)), ((0, 6), (3, 4)), ((1, 1), (3, 4)),
                  ((1, 1), (3, 1), (2, 5)), ((1, 1), (2, 7))))
_H9 = (9, ((0, 3), (3, 2), (6, 5), (5, 8)),
                  (((0, 3), (2, 3), (0, 4)), ((0, 3), (3, 2)), ((1, 3), (3, 3), (3, 2)),
                   ((1, 3), (2, 4)), ((1, 0), (2, 4))), _by_parity)
_HEADS = _Scheme(*_H8)
_HIDDEN = _Scheme(*_H9)


def _stack(parts):
    return parts[0] if len(parts) == 1 else jnp.concatenate(parts, axis=0)


def _join(low, high):
    return low if low is high else jnp.concatenate([low[:, :_UNIT], high[:, _UNIT:]], axis=1)


def _swap(x):
    return jnp.concatenate([x[:, _UNIT:], x[:, :_UNIT]], axis=1)


def _operands(sets, dtype):
    @functools.lru_cache(maxsize=None)
    def tile(h, i, swapped):
        if i == _UNITS // 2:
            return jnp.concatenate([sets[h][:, -_UNIT:]] * 2, axis=1)
        return _swap(tile(h, i, 0)) if swapped else sets[h][:, i * _LANES:(i + 1) * _LANES]

    value = _gather(lambda h, block: _join(
        *[tile(h, unit // 2, (unit + lane) % 2) for lane, unit in enumerate(block)]))
    return functools.lru_cache(maxsize=None)(lambda key: value(key).astype(dtype))


def _expand(plan, lhs, weight, n_sets, done):
    parts = {}

    def finished(h, x, value):
        parts[h, x] = value
        if all((i, x) in parts for i in range(n_sets)):
            done(x, [parts[i, x] for i in range(n_sets)])

    add = _scatter([wide for _, _, wide in plan], finished)
    for j, narrow, wide in plan:
        product = _dot(lhs(narrow), weight(j))
        add(wide, product)
        yield product


def _reduce(plan, tile, weight, totals, dtype):
    def finished(h, block, value):
        for lane, unit in enumerate(block):
            totals[h][unit, lane] = _add(totals[h].get((unit, lane)), 1, value)

    lhs = _gather(tile)
    add = _scatter([narrow for _, narrow, _ in plan], finished)
    for j, narrow, wide in plan:
        product = _dot(lhs(wide).astype(dtype), weight(j))
        add(narrow, product)
        yield product


def _fold(totals):
    return {(u // 2, u % 2): _join(x, totals.get((u ^ 1, 1), x))
            for (u, lane), x in sorted(totals.items()) if lane == 0} | {
                (u // 2, 1 - u % 2): x
                for (u, lane), x in sorted(totals.items()) if lane and (u ^ 1, 0) not in totals}


def _merge(tiles):
    out = [tiles[i, 0] + _swap(tiles[i, 1]) if (i, 1) in tiles else tiles[i, 0]
           for i in range(_UNITS // 2 + 1)]
    return jnp.concatenate(out[:-1] + [out[-1][:, :_UNIT]], axis=1)


def _weave(main, side=(), first=0, every=1):
    side = iter(side)
    for i, _ in enumerate(main):
        if i >= first and (i - first) % every == 0:
            next(side, None)
    for _ in side:
        pass


def _take(gen, n):
    _weave(itertools.islice(gen, n))


def _layernorm(x):
    m = jnp.mean(x, axis=-1, keepdims=True)
    d = x - m
    v = jnp.mean(d * d, axis=-1, keepdims=True)
    return d * jax.lax.rsqrt(v + _EPS)


def _reciprocal(x):
    return pltpu.reciprocal(x, approx=True)


def _dot(a, b):
    return jax.lax.dot_general(a, b, (((1,), (0,)), ((), ())),
                               preferred_element_type=jnp.float32)


def _dot_nt(a, b):
    return jax.lax.dot_general(a, b, (((1,), (1,)), ((), ())),
                               preferred_element_type=jnp.float32)


def _unpack(words):
    return pltpu.bitcast(words, jnp.bfloat16)


class _Tiles:
    def __init__(self, ref, first=0, rows=_LANES):
        self.ref, self.first, self.rows = ref, first, rows

    def shifted(self, by, limit):
        rows = pl.ds(pl.multiple_of(by, 16), self.ref.shape[0] - limit)
        return _Tiles(self.ref.at[rows], self.first, self.rows)

    def load_words(self, j, rows=None):
        start = (self.first + j * self.rows) // 2
        return self.ref.bitcast(jnp.uint32)[pl.ds(start, (rows or self.rows) // 2), :]

    def store_words(self, j, words, at=0):
        start = (self.first + j * self.rows + at) // 2
        self.ref.bitcast(jnp.uint32)[pl.ds(start, words.shape[0]), :] = words

    def load(self, j):
        return _unpack(self.load_words(j))

    def store(self, j, value, at=0):
        start = self.first + j * self.rows + at
        self.ref[pl.ds(start, value.shape[0]), :] = value.astype(jnp.bfloat16)


def _attention_masks(n_layers, n_mem, seg):
    rows = n_layers * (n_mem + seg)
    i = jax.lax.broadcasted_iota(jnp.int32, (rows, rows), 0)
    j = jax.lax.broadcasted_iota(jnp.int32, (rows, rows), 1)
    visible = (i < n_layers * n_mem) | (i >= j)
    if n_layers == 1:
        return visible, _MASKED * _LOG2E

    def second_layer(r):
        return ((r >= n_mem) & (r < 2 * n_mem)) | (r >= 2 * n_mem + seg)

    same = second_layer(i) == second_layer(j)
    fill = jnp.where(same, _MASKED * _LOG2E, -jnp.inf).astype(jnp.float32)
    return same & visible, fill


def _start(copies):
    for c in copies:
        c.start()


_SCOPES = False
_WAITS = itertools.count()


def _wait(copies):
    if _SCOPES:
        with jax.named_scope(f"wait{next(_WAITS):02d}"):
            for c in copies:
                c.wait()
        return
    for c in copies:
        c.wait()


class _Pacer:
    def __init__(self, zero):
        self.zero, self.after = zero.astype(jnp.uint32), None

    def hold(self, words):
        if self.after is None:
            return words
        return words | _stack([self.after] * (words.shape[0] // 8))

    def run(self, products, chores, rate):
        for i, product in enumerate(products):
            count = int((i + 1) * rate) - int(i * rate)
            if count:
                self.after = pltpu.bitcast(product[:8], jnp.uint32) & self.zero
                _take(chores, count)
            yield product


def _build_rows(tiles, weights, words):
    value = _gather(lambda u, x: _unpack(words(u, x)).astype(jnp.float32))
    for j, halves in enumerate(weights):
        for lane, key in enumerate(halves):
            if _is_leaf(key):
                tiles.store_words(j, words(*key), lane * _UNIT)
            else:
                tiles.store(j, value(key), lane * _UNIT)
        yield


def _build_transposed(tiles, weights, chosen, words, pacer):
    for j in chosen:
        first = _leaves(weights[j][0])[0]

        def rows(*key):
            return pacer.hold(words(*key)) if key == first else words(*key)

        if all(_is_leaf(key) for key in weights[j]):
            tile = _unpack(_stack([rows(*key) for key in weights[j]]))
        else:
            value = _gather(lambda u, x: _unpack(rows(u, x)).astype(jnp.float32))
            tile = _stack([value(key) for key in weights[j]]).astype(jnp.bfloat16)
        tiles.store_words(j, pltpu.bitcast(tile.T, jnp.uint32))
        yield


def _build_output(tiles, raw_ref, for_single, pacer):
    single = [j for j, _, _ in _HEADS.single]
    return _build_transposed(
        tiles, _HEADS.weights, [j for j in range(len(_HEADS.weights)) if (j in single) == for_single],
        lambda u, x: raw_ref[x, u * _UNIT // 2:(u + 1) * _UNIT // 2, :], pacer)


def _prologue(xt_hbm, w_hbms, wot_hbm, later_copies, tile_ref, res_ref, early, weights, zero,
              raw_ref, normed_ref, stage0_ref, stage1_ref, sems, *, seg):
    n_heads = raw_ref.shape[0]
    stages = (stage0_ref, stage1_ref, stage0_ref)
    next_sem = itertools.count()

    def copies(pairs):
        sem = sems.at[next(next_sem)]
        return [pltpu.make_async_copy(src, dst, sem) for src, dst in pairs]

    def head_copies(which, pairs):
        return copies((w_hbms[which].bitcast(jnp.uint32).at[:, p, :], stages[which].at[p])
                      for p in pairs)

    x_chunks = [range(a, b) for a, b in zip(_X_CUTS, _X_CUTS[1:])]
    q_chunks = [range(a, b) for a, b in zip(_Q_CUTS, _Q_CUTS[1:])]
    queue = [copies((xt_hbm.at[:, pl.ds(i * _LANES, _LANES)], tile_ref.at[i]) for i in chunk)
             for chunk in x_chunks]
    queue += [head_copies(0, chunk) for chunk in q_chunks]
    queue += [head_copies(1, range(n_heads // 2))]
    v_copies = head_copies(2, range(n_heads // 2))
    wo_copies = copies([(wot_hbm.bitcast(jnp.uint32), raw_ref)])
    arrived = itertools.count()

    def advance():
        i = next(arrived)
        _wait(queue[i])
        if i + 2 < len(queue):
            _start(queue[i + 2])

    def normalize(chunk):
        for i in chunk:
            if i:
                known = [res_ref[pl.ds(i * _LANES + r, _KNOWN), :]
                         for r in range(0, _LANES, 2 * seg)]
                normed_ref[(i - 1) * 2 * _KNOWN:i * 2 * _KNOWN, :] = _layernorm(_stack(known))

    _start(queue[0])
    _start(queue[1])
    for before, chunk in zip([()] + x_chunks, x_chunks):
        advance()
        normalize(before)
        for i in chunk:
            res_ref[i * _LANES:(i + 1) * _LANES, :] = tile_ref[i].astype(jnp.float32).T
    normalize(x_chunks[-1])
    pacer = _Pacer(zero)
    rows = early.rows // 2
    sums = _Tiles(weights[4].ref, 0, rows)
    fresh = _operands([normed_ref[:rows, :], normed_ref[rows:, :]], jnp.float32)
    slots = {}

    def lhs(key):
        if key not in slots:
            slots[key] = len(slots)
            sums.store(slots[key], fresh(key))
        return sums.load(slots[key])

    def raw(which, unit, x, hold=lambda words: words):
        words = hold(stages[which][x // 2, unit * _UNIT:(unit + 1) * _UNIT, :])
        words = words & jnp.uint32(0xFFFF0000) if x % 2 else words << 16
        return pltpu.bitcast(words, jnp.float32)

    def build(which, j, *hold):
        value = _gather(lambda u, x: raw(which, u, x, *hold))
        weights[which].store(j, _stack([value(key) for key in _HEADS.weights[j]]))

    def sweep(which, plan):
        def weight(j):
            build(which, j)
            return weights[which].load(j)

        return _expand(plan, lhs, weight, 2,
                       lambda x, halves: early.store(which * n_heads + x, _stack(halves)))

    def extra(which):
        return (build(which, j, pacer.hold)
                for j in range(len(_HEADS.double), len(_HEADS.weights)))

    def needs(product):
        last = max(x for key in _HEADS.weights[product[0]] for _, x in _leaves(key)) // 2
        return sum(cut <= last for cut in _Q_CUTS[1:])

    plan = sorted(_HEADS.double, key=needs)
    products = sweep(0, plan)
    for c in range(len(q_chunks) - 1):
        advance()
        _take(products, sum(needs(product) <= c for product in plan) // _MXUS * _MXUS
              - sum(needs(product) < c for product in plan) // _MXUS * _MXUS)
    advance()
    _weave(pacer.run(products, extra(0), 0.5))
    advance()
    _start(v_copies)
    products = pacer.run(sweep(1, _HEADS.double), extra(1), 0.25)
    _take(products, _WO_START)
    _start(wo_copies)
    _weave(products)
    _wait(v_copies)
    _start(later_copies[0])
    products = pacer.run(sweep(2, _HEADS.double), extra(2), 0.5)
    _take(products, _WO_AT)
    _wait(wo_copies)
    _start(later_copies[1])
    _weave(pacer.run(products, _build_output(weights[3], raw_ref, True, pacer),
                     len(_HEADS.single) / (len(_HEADS.double) - _WO_AT - 4)))


def _layers(outt_hbm, mem0_ref, ffn_copies, tile_ref, res_ref, early, weights, raw_refs,
            w2t_hbm, rawo_ref, zero, tile_sem, raw2_ref, act_ref, out_ref, q_ref, k_ref, v_ref,
            *, seg):
    n_mem = mem0_ref.shape[0]
    n_heads = len(_HEADS.blocks)
    n_io = tile_ref.shape[0]
    n_seg = res_ref.shape[0] // seg
    n_pairs = (n_seg - _LAG) // 2
    n_ffn = len(_HIDDEN.double)
    score_scale = _LANES ** -0.5 * _LOG2E
    qkv_tiles = [_Tiles(ref, 0, 2 * (n_mem + seg)) for ref in (q_ref, k_ref, v_ref)]

    kept = [tiles.shifted(zero, 0) if _PIN else tiles for tiles in qkv_tiles]

    w2_copy = pltpu.make_async_copy(w2t_hbm.bitcast(jnp.uint32), raw2_ref, tile_sem.at[0])

    def block(r, n=1):
        return pl.ds(pl.multiple_of(r * seg, seg), n * seg)

    def transpose_out(i):
        rows = pl.ds(pl.multiple_of(i * _LANES, _LANES), _LANES)
        tile_ref[i] = res_ref[rows, :].T.astype(tile_ref.dtype)

    def attention(plan, sets, dtype, keep, fetch, filler=None, lead=0, n_filler=0, spill=0,
                  pace=lambda which, products: products):
        n_layers = len(sets)
        lhs = _operands(sets, dtype)
        visible, fill = _attention_masks(n_layers, n_mem, seg)
        probs, heads, totals = [], [], [{} for _ in sets]

        def project(which):
            return pace(which, _expand(plan, lhs, weights[which].load, n_layers,
                                       functools.partial(keep, which)))

        def scores():
            for h in range(n_heads):
                s = jnp.where(visible, _dot_nt(fetch(0, h), fetch(1, h)) * score_scale, fill)
                p = jnp.exp2(s - jnp.max(s, axis=-1, keepdims=True))
                p = p * _reciprocal(jnp.sum(p, axis=-1, keepdims=True))
                probs.append(p.astype(keep.dtype))
                if len(probs) % _MXUS == 0:
                    yield

        def values():
            for h in range(n_heads):
                o = _dot(probs[h], fetch(2, h))
                tokens = n_layers * n_mem
                heads.append([_stack([o[i * n_mem:(i + 1) * n_mem],
                                      o[tokens + i * seg:tokens + (i + 1) * seg]])
                              for i in range(n_layers)])
                if len(heads) % _MXUS == 0:
                    yield

        def head(h, x):
            while x >= len(heads):
                next(mixed)
            return heads[x][h]

        n = len(plan)
        mixed = values()
        output = pace(3, _reduce(plan, head, weights[3].load, totals, jnp.float32))
        _weave(project(0))
        _weave(project(1))
        if filler:
            _weave(itertools.chain(itertools.islice(filler, lead), project(2)), scores(), _FIRST,
                   (n + lead) // n_heads * _MXUS)
            _weave(itertools.chain(itertools.islice(filler, n_filler - lead), output), mixed,
                   _FIRST, (n_filler - lead + spill) // n_heads * _MXUS)
        else:
            _weave(project(2), scores(), 15, (n - 16) // n_heads * _MXUS)
            _take(mixed, 3)
            _weave(output, mixed, 3, n // 16 // _MXUS * _MXUS)
        return [_fold(t) for t in totals]

    def gated(sets):
        lhs = _operands([_layernorm(x) for x in sets], jnp.bfloat16)
        gates = {}

        def gate(x, halves):
            gates[x] = [g * _reciprocal(1.0 + jnp.exp2(g * -_LOG2E)) for g in halves]

        def up(x, halves):
            for h in range(2):
                act_ref[x, h] = gates[x][h] * halves[h]

        yield from _expand(_HIDDEN.double, lhs, weights[4].load, 2, gate)
        yield from _expand(_HIDDEN.double, lhs, weights[5].load, 2, up)

    def down(ffn=None):
        totals = [{}, {}]
        gen = _reduce(_HIDDEN.double, lambda h, x: act_ref[x, h], weights[6].load, totals,
                      jnp.bfloat16)
        if ffn:
            _take(gen, _D0)
            _take(ffn, _F0)
        _weave(gen)
        return [_merge(_fold(t)) for t in totals]

    def single_step(r, mem, **options):
        x = res_ref[block(r), :]
        qkv = {}

        def keep(which, h, parts):
            qkv[which, h] = parts[0].astype(jnp.bfloat16) if which else parts[0]

        keep.dtype = jnp.float32
        out = _merge(*attention(_HEADS.single, [_stack([mem, _layernorm(x)])], jnp.float32,
                                keep, lambda which, h: qkv[which, h], **options))
        res_ref[block(r), :] = x + out[n_mem:]
        return out[:n_mem]

    def head_step(r, mem):
        _wait(ffn_copies(r))
        pl.when(r + 2 < _LAG)(lambda: _start(ffn_copies(r + 2)))
        pl.when(r + 2 == _LAG)(w2_copy.start)
        pacer = _Pacer(zero)
        chores = itertools.chain(*[
            _build_rows(tiles.shifted(r * 16, _UNIT - 16), _HIDDEN.weights[:n_ffn],
                        lambda u, x, raw=raw: pacer.hold(raw[r, u, :, x * _LANES:(x + 1) * _LANES]))
            for raw, tiles in zip(raw_refs, weights[4:])])
        _take(chores, _AHEAD)
        mem = single_step(
            r, mem, pace=lambda which, products: pacer.run(products, chores, _CHORES[which]))
        _weave(chores)
        return mem

    def double_step(mems, x1, x2, pair, *filler):
        h2 = _layernorm(x2)
        if pair is None:
            sets = [_stack([mems[0], _layernorm(x1)]), _stack([mems[1], h2])]
        else:
            moved = _KNOWN // 2
            known = early.shifted(pair * _KNOWN, early.rows - _KNOWN)
            sets = [_stack([mems[0], _layernorm(x1[_KNOWN:]), h2[:moved]]),
                    _stack([mems[1], h2[moved:]])]
        slot = int(pair is None)

        def keep(which, h, parts):
            tiles, i = qkv_tiles[which], slot * n_heads + h
            tokens = _stack([p[n_mem:] for p in parts])
            tiles.store(i, _stack([p[:n_mem] for p in parts]))
            tiles.store(i, tokens, tiles.rows - tokens.shape[0])
            if pair is not None:
                tiles.store_words(i, known.load_words(which * n_heads + h, _KNOWN), 2 * n_mem)

        keep.dtype = jnp.bfloat16
        return attention(_HEADS.double, sets, jnp.float32 if pair is None else jnp.bfloat16, keep,
                         lambda which, h: kept[which].load(slot * n_heads + h), *filler)

    folded = list(_fold(dict.fromkeys(_HEADS.places)))

    def pair_step(j, mems, x2, ffn=None):
        x1 = res_ref[block(2 * j + _LAG, 2), :]
        out = [_merge(t) for t in
               double_step(mems, x1[:seg], x2[:seg], j, ffn, _LEAD, _F2, _SPILL)]
        res_ref[block(2 * j + _LAG), :] = x1[:seg] + out[0][n_mem:]
        res_ref[block(2 * j), :] = x2[:seg] + out[1][n_mem:]
        res_ref[block(2 * j + 1), :] = x2[seg:]
        if ffn:
            _take(ffn, _F3)
        tiles = double_step([o[:n_mem] for o in out], x1[seg:], x2[seg:], None,
                            ffn, _LEAD_B, 2 * n_ffn - _F0 - _F1 - _F2 - _F3, _SPILL_B)
        for h in range(2):
            for i, key in enumerate(folded):
                out_ref[h, i] = tiles[h][key]

    def finish_pair(j):
        out = [_merge({key: out_ref[h, i] for i, key in enumerate(folded)}) for h in range(2)]
        xs = []
        for r, o in zip((2 * j + _LAG, 2 * j), out):
            x = res_ref[block(r, 2), :]
            xs.append(_stack([x[:seg], x[seg:] + o[n_mem:]]))
        for r, x in zip((2 * j + _LAG, 2 * j), xs):
            res_ref[block(r + 1), :] = x[seg:]
        return [o[:n_mem] for o in out], xs

    def steady(j):
        mems, xs = finish_pair(j - 1)
        ffn = gated(xs)
        y = down(ffn)
        x2 = res_ref[block(2 * j, 2), :] + y[0]
        old = block(2 * j - _LAG, 2)
        res_ref[old, :] = res_ref[old, :] + y[1]
        transpose_out(jnp.maximum(j - 3, 0) // 2)
        _take(ffn, _F1)
        pair_step(j, mems, x2, ffn)

    out_copies = [
        pltpu.make_async_copy(tile_ref.at[i],
                              outt_hbm.at[:, pl.ds(i * _LANES, _LANES)], tile_sem.at[i])
        for i in range(n_io)]

    if _ONLY == "pair":
        pl.loop(2, n_pairs)(steady)
        _start(out_copies)
        _wait(out_copies)
        return
    mem0 = mem0_ref[...].astype(jnp.float32)
    mem1 = jax.lax.fori_loop(0, _LAG, head_step, mem0)
    xs = [res_ref[block(2 * h, 2), :] for h in range(2)]
    _wait([w2_copy])
    pacer = _Pacer(zero)
    chores = _build_transposed(
        weights[6], _HIDDEN.weights, range(n_ffn), lambda u, x:
        raw2_ref[u * _UNIT // 2:(u + 1) * _UNIT // 2, x * _LANES:(x + 1) * _LANES], pacer)
    _weave(pacer.run(gated(xs), chores, _W2_RATE))
    pacer.after = None
    _weave(chores)
    xs = [x + y for x, y in zip(xs, down())]
    if _ONLY in ("head", "start"):
        tile_ref[n_io - 1] = _stack(xs).astype(tile_ref.dtype).T
        _start(out_copies)
        _wait(out_copies)
        return
    if _ONLY != "tail":
        _weave(_build_output(weights[3], rawo_ref, False, pacer))
        pair_step(0, [mem1, mem0], xs[0])
        mems, ready = finish_pair(0)
        ffn = gated(ready)
        _take(ffn, _F0 + _F1)
        pair_step(1, mems, xs[1], ffn)
        pl.loop(2, n_pairs)(steady)

    last = n_seg - _LAG
    n_done = (n_pairs - 4) // 2 + 1
    _start(out_copies[:n_done])
    mems, xs = finish_pair(n_pairs - 1)
    for r, y in zip((last, last - _LAG), down()):
        res_ref[block(r, 2), :] = res_ref[block(r, 2), :] + y
    _weave(gated(xs))
    for r, x, y in zip((last + 2, last + 2 - _LAG), xs, down()):
        res_ref[block(r, 2), :] = x + y
    jax.lax.fori_loop(last, n_seg, single_step, mems[1])
    for i in range(n_done, n_io - 1):
        transpose_out(i)
        out_copies[i].start()
    xs = [res_ref[block(last + 2 * h, 2), :] for h in range(2)]
    _weave(gated(xs))
    tile_ref[n_io - 1] = (_stack(xs) + _stack(down())).T.astype(tile_ref.dtype)
    out_copies[n_io - 1].start()
    _wait(out_copies)


def _kernel(xt_hbm, mem0_hbm, wq_hbm, wk_hbm, wv_hbm, wot_hbm, w1_hbm, w3_hbm, w2t_hbm,
            outt_hbm, mem0_ref, tile_ref, res_ref, early_ref, w_ref, ffn_ref,
            rawo_ref, raw1_ref, raw3_ref, zero_ref, tile_sem, raw_sem, *, seg):
    d_model, n_heads, _ = wq_hbm.shape
    n_mem = mem0_ref.shape[0]
    weights = [_Tiles(ref, i * ref.shape[0] // n) for ref, n in ((w_ref, 4), (ffn_ref, 3))
               for i in range(n)]
    early = _Tiles(early_ref, 0, early_ref.shape[0] // (3 * n_heads))
    raw_refs = (raw1_ref, raw3_ref)

    @pl.loop(0, 2)
    def _(i):
        zero_ref[i] = i

    zero = zero_ref[0]

    def ffn_copies(r):
        rows = pl.ds(pl.multiple_of(r * 8, 8), 8)
        return [pltpu.make_async_copy(src.bitcast(jnp.uint32).at[:, rows, :], dst.at[r],
                                      raw_sem.at[r])
                for src, dst in zip((w1_hbm, w3_hbm), raw_refs)]

    mem_copy = pltpu.make_async_copy(mem0_hbm, mem0_ref, raw_sem.at[_LAG])
    if _ONLY in (None, "prologue", "start"):
        pl.run_scoped(
            functools.partial(_prologue, xt_hbm, (wq_hbm, wk_hbm, wv_hbm), wot_hbm,
                              [[mem_copy] + ffn_copies(0), ffn_copies(1)], tile_ref, res_ref,
                              early, weights, zero, rawo_ref, seg=seg),
            pltpu.VMEM((early.rows, d_model), jnp.float32),
            pltpu.VMEM((n_heads // 2, d_model, _LANES), jnp.uint32),
            pltpu.VMEM((n_heads // 2, d_model, _LANES), jnp.uint32),
            pltpu.SemaphoreType.DMA((len(_X_CUTS) + len(_Q_CUTS) + 1,)))
        _wait([mem_copy])
    if _ONLY == "prologue":
        _wait(ffn_copies(0) + ffn_copies(1))

        @pl.loop(0, 8)
        def _(i):
            tile_ref[0, :_LANES, :] = weights[0].shifted(i * 16, 128).load(0) + early.shifted(i * 16, 128).load(0)[:_LANES] + res_ref[pl.ds(i * _LANES, _LANES), :_LANES].astype(jnp.bfloat16)
        pltpu.sync_copy(tile_ref.at[0], outt_hbm.at[:, pl.ds(0, _LANES)])
        return
    pl.run_scoped(
        functools.partial(_layers, outt_hbm, mem0_ref, ffn_copies, tile_ref, res_ref, early,
                          weights, raw_refs, w2t_hbm, rawo_ref, zero, tile_sem, seg=seg),
        pltpu.VMEM((d_model // 2, w2t_hbm.shape[1]), jnp.uint32),
        pltpu.VMEM((len(_HIDDEN.blocks), 2, 2 * seg, _LANES), jnp.float32),
        pltpu.VMEM((2, _UNITS + 1, n_mem + seg, _LANES), jnp.float32),
        *[pltpu.VMEM((4 * n_heads * (n_mem + seg), _LANES), jnp.bfloat16)] * 3)


@functools.partial(jax.jit, static_argnames=("A_seg_len",))
def pallas_interleave_layers__memory_aug_recurrent_mem_tr__glu_gated_swiglu__prompt_kernel(
    A_x: jax.Array,
    A_mem0: jax.Array,
    A_Wq: jax.Array,
    A_Wk: jax.Array,
    A_Wv: jax.Array,
    A_Wo: jax.Array,
    A_seg_len: int,
    B_x: jax.Array,
    B_w1: jax.Array,
    B_w3: jax.Array,
    B_w2: jax.Array,
):
    del B_x
    _, n_tok, d_model = A_x.shape
    n_mem = A_mem0.shape[1]
    _, n_heads, d_head = A_Wq.shape
    d_ff = B_w1.shape[1]
    seg = A_seg_len
    n_known = (n_tok // seg - _LAG) // 2 * _KNOWN
    hbm = pl.BlockSpec(memory_space=pltpu.HBM)
    out_t = pl.pallas_call(
        functools.partial(_kernel, seg=seg),
        out_shape=jax.ShapeDtypeStruct((d_model, n_tok), A_x.dtype),
        in_specs=[hbm] * 9,
        out_specs=hbm,
        scratch_shapes=[
            pltpu.VMEM((n_mem, d_model), A_mem0.dtype),
            pltpu.VMEM((n_tok // _LANES, d_model, _LANES), A_x.dtype),
            pltpu.VMEM((n_tok, d_model), jnp.float32),
            pltpu.VMEM((3 * n_heads * n_known, d_head), jnp.bfloat16),
            pltpu.VMEM((4 * len(_HEADS.weights) * _LANES, _LANES), jnp.bfloat16),
            pltpu.VMEM((3 * len(_HIDDEN.double) * _LANES, _LANES), jnp.bfloat16),
            pltpu.VMEM((n_heads, d_model // 2, d_head), jnp.uint32),
            *[pltpu.VMEM((_LAG, _UNITS, 8, d_ff), jnp.uint32)] * 2,
            pltpu.SMEM((2,), jnp.int32),
            pltpu.SemaphoreType.DMA((n_tok // _LANES,)),
            pltpu.SemaphoreType.DMA((_LAG + 1,)),
        ],
        compiler_params=pltpu.CompilerParams(vmem_limit_bytes=127 * 1024 * 1024, flags=_FLAGS),
    )(A_x.reshape(n_tok, d_model).T, A_mem0.reshape(n_mem, d_model), A_Wq, A_Wk, A_Wv,
      A_Wo.transpose(0, 2, 1), *[w.reshape(_UNITS, _UNIT, d_ff) for w in (B_w1, B_w3)], B_w2.T)
    return out_t.T.reshape(A_x.shape)
```

```python
import functools
import itertools
import math

import jax
import jax.numpy as jnp
import jax.experimental.pallas as pl
import jax.experimental.pallas.tpu as pltpu
import numpy as np

_EPS = 1e-05
_MASKED = -1000000000.0
_LOG2E = math.log2(math.e)
_LANES = 128
_UNIT = _LANES // 2
_UNITS = 9
_MXUS = 4
_LAG = 4
_KNOWN = 16
_ONLY = None
_FLAGS = None
_D0, _F0, _F1, _F2, _F3 = 100, 40, 71, 160, 72
_LEAD, _SPILL, _FIRST = 72, 40, 19
_LEAD_B, _SPILL_B = 72, 40
_CHORES, _AHEAD, _W2_RATE = (0.6, 1.4, 0.6, 0.8), 30, 0.5
_PLAIN = tuple((i, 0) for i in range(5))
_O_QKV, _O_OUT, _O_UP, _O_DOWN = (1, 0, _PLAIN), (1, 0, _PLAIN), (1, 2, _PLAIN), (1, 2, _PLAIN)
_MERGED = 0
_FIRST_B, _FIRSTV, _FIRSTV_B, _SQUEEZE, _SQUEEZE_B = 19, 19, 19, 0, 0
_PACE_A, _PACE_B = (1, 12), (1, 12)
_P_F32, _EARLY_F32 = 0, 0
_PIN = 1
_D1 = 0
_PRIORITY = 0
_X_CUTS = (1, 5)
_RING = 32
_Q_CUTS = (0, 4, 8, 12, 16)
_WO_START, _WO_AT = 80, 128

_D0 = 100
_D1 = 0
_F0 = 40
_F1 = 71
_F2 = 156
_F3 = 72
_LEAD = 72
_LEAD_B = 88
_SPILL = 40
_SPILL_B = 40
_FIRST = 19
_FIRST_B = 19
_FIRSTV = 51
_FIRSTV_B = 35
_SQUEEZE = 0
_SQUEEZE_B = 2
_PACE_A = (1, 10)
_PACE_B = (1, 12)
_P_F32 = 1
_MERGED = 1
_O_QKV = (1, 0, ((0, 0), (1, 0), (2, 0), (3, 0), (4, 0)))
_O_OUT = (3, 2, ((2, 5), (1, 1), (0, 1), (4, 0), (3, 0)))
_O_UP = (1, 2, ((0, 0), (1, 0), (2, 0), (3, 0), (4, 0)))
_O_DOWN = (5, 2, ((1, 8), (2, 8), (0, 3), (3, 6), (4, 0)))
_FLAGS = None

class _Scheme:
    def __init__(self, period, blocks, links, orient=tuple, late=True, first=()):
        self.period, self.n_links = period, len(links)
        links = [tuple((orbit, (s + shift) % period) for orbit, shift in link)
                 for s in range(period) for link in links]
        nodes = list(dict.fromkeys([*first] + [node for link in links for node in link]))
        self.nodes = nodes
        links = [tuple(nodes.index(node) for node in link) for link in links]
        kinds = [orbit // 2 for orbit, _ in nodes]
        self.blocks = [orient([u if u >= period else (u + s) % period for u in blocks[orbit]])
                       for orbit, s in nodes]
        cells, products = [], {}

        def form(side, v, p):
            if len(v) > (2 if p == 2 else 1):
                key = ((1, form(side, v[:-1], p)[1]), (1, form(side, v[-1:], p)[1]))
            elif p == 2:
                key = ((1, form(side, v, 0)[1]), (1 - 2 * side, form(side, v, 1)[1]))
            else:
                key = (p, self.blocks[v[0]]) if side == 0 else (1 - p, v[0])
            return (-1 if p == 2 * (1 - side) else 1), key

        def use(narrow, wide, sign):
            weight = products.setdefault((narrow[1], wide[1]), {})
            weight[len(cells) - 1] = sign * narrow[0] * wide[0]

        def square(v, p, q, sign):
            use(form(0, v, p), form(1, v, q), sign)

        def cross(u, v, both, p):
            q, r = (p + 1) % 3, (p + 2) % 3
            mixed = []
            for side in range(2):
                (s, a), (t, b) = form(side, u, q), form(side, v, p)
                mixed.append((s, ((1, a), (-s * t, b))))
            cells.append((u, v))
            square(both, p, q, 1), square(u, r, q, 1), square(v, p, r, 1), use(*mixed, 1)
            cells.append((v, u))
            square(both, q, p, -1), square(u, q, r, -1), square(v, r, p, -1), use(*mixed, -1)

        owner = {}
        for i, link in enumerate(links):
            for x in link:
                if ((x,), (x,)) not in cells:
                    cells.append(((x,), (x,)))
                    square((x,), (kinds[x] + 1) % 3, (kinds[x] + 2) % 3, 1)
                    square((x,), (kinds[x] + 2) % 3, (kinds[x] + 1) % 3, -1)
            before = len(cells)
            cross(link[:1], link[1:2], link[:2], 0)
            if len(link) == 3 and kinds[link[2]]:
                cross(link[2:], link[:2], link, 1)
            elif len(link) == 3:
                cross(link[:2], link[2:], link, 2)
            owner.update(dict.fromkeys(range(before, len(cells)), i))
        self.links = [sorted({owner[j] for j in weight if j in owner})
                      for weight in products.values()]
        self.double = [(j, narrow, wide) for j, (narrow, wide) in enumerate(products)]

        sums = list(products.values())
        own = [products[form(0, (x,), 1 - kinds[x])[1], form(1, (x,), 2)[1]]
               for x in range(len(nodes))]
        self.single = []
        for j, (rows, cols) in enumerate(cells):
            weight = own[rows[0]] if rows == cols else {j: -1} if {j: -1} in sums else {j: 1}
            if weight not in sums:
                sums.append(weight)
            if rows != cols:
                rows, cols = (rows + cols[:len(cols) == 1 and j in own[cols[0]]],
                              cols + rows[:len(rows) == 1 and j in own[rows[0]]])
            self.single.append((sums.index(weight), form(0, rows, 0)[1],
                                ((weight[j], form(1, cols, 1)[1]),)))

        basis = np.zeros((_UNITS, len(nodes), len(cells), 2))
        for j, (rows, cols) in enumerate(cells):
            for x, y, lane in itertools.product(rows, cols, range(2)):
                basis[self.blocks[x][lane], y, j, lane] += 1
        inverse = np.rint(np.linalg.inv(basis.reshape(2 * len(cells), -1))).reshape(
            len(cells), 2, _UNITS, -1)
        raw = [[_sum((int(lane[u, x]), (int(u), int(x))) for u, x in np.argwhere(lane))
                for lane in cell] for cell in inverse]
        self.weights = [[_sum((sign, raw[j][lane]) for j, sign in weight.items())
                         for lane in range(2)] for weight in sums]
        self.places = sorted({(u, lane) for b in self.blocks for lane, u in enumerate(b)})


    def ordered(self, step, pick, visits):
        rank = {(s * step + shift) % self.period * self.n_links + link: (s, i)
                for s in range(self.period) for i, (link, shift) in enumerate(visits)}

        def position(product):
            ranks = sorted(rank[i] for i in self.links[product[0]])
            return ranks[min(pick, len(ranks) - 1)], (len(ranks) > 1) == (pick > 0)

        return sorted(self.double, key=position)


def _sum(terms):
    terms = sorted(terms, key=lambda term: -term[0])
    return terms[0][1] if len(terms) == 1 and terms[0][0] == 1 else tuple(terms)


def _is_leaf(key):
    return isinstance(key[0], int)


def _leaves(key):
    return [key] if _is_leaf(key) else [leaf for _, term in key for leaf in _leaves(term)]


def _add(total, sign, value):
    if total is None:
        return value if sign > 0 else -value
    return total + value if sign > 0 else total - value


def _gather(leaf):
    @functools.lru_cache(maxsize=None)
    def value(key):
        if _is_leaf(key):
            return leaf(*key)
        total = None
        for sign, term in key:
            total = _add(total, sign, value(term))
        return total

    return value


def _scatter(keys, done):
    missing, totals = {}, {}

    def count(key):
        missing[key] = missing.get(key, 0) + 1
        if missing[key] == 1 and not _is_leaf(key):
            for _, term in key:
                count(term)

    def add(key, value, sign=1):
        if key in totals:
            old_sign, old = totals[key]
            if old_sign >= sign:
                sign, value = old_sign, _add(old, sign * old_sign, value)
            else:
                value = value - old
        totals[key] = sign, value
        missing[key] -= 1
        if missing[key]:
            return
        if _is_leaf(key):
            done(*key, _add(None, sign, value))
        else:
            for factor, term in key:
                add(term, value, sign * factor)

    for key in keys:
        count(key)
    return add


def _by_parity(block):
    low, high = sorted(block)
    if high == _UNITS - 1:
        return (high, low) if low % 2 else (low, high)
    return (low, high) if high % 2 else (high, low)


_H8 = (8, ((7, 0), (7, 3), (8, 6), (5, 6)),
                 (((0, 6), (2, 6), (0, 3)), ((0, 6), (3, 4)), ((1, 1), (3, 4)),
                  ((1, 1), (3, 1), (2, 5)), ((1, 1), (2, 7))))
_H9 = (9, ((0, 3), (3, 2), (6, 5), (5, 8)),
                  (((0, 3), (2, 3), (0, 4)), ((0, 3), (3, 2)), ((1, 3), (3, 3), (3, 2)),
                   ((1, 3), (2, 4)), ((1, 0), (2, 4))), _by_parity)
_HEADS = _Scheme(*_H8, late=False)
_HIDDEN = _Scheme(*_H9)


def _stack(parts):
    return parts[0] if len(parts) == 1 else jnp.concatenate(parts, axis=0)


def _join(low, high):
    return low if low is high else jnp.concatenate([low[:, :_UNIT], high[:, _UNIT:]], axis=1)


def _swap(x):
    return jnp.concatenate([x[:, _UNIT:], x[:, :_UNIT]], axis=1)


def _operands(sets, dtype):
    @functools.lru_cache(maxsize=None)
    def tile(h, i, swapped):
        if i == _UNITS // 2:
            return jnp.concatenate([sets[h][:, -_UNIT:]] * 2, axis=1)
        return _swap(tile(h, i, 0)) if swapped else sets[h][:, i * _LANES:(i + 1) * _LANES]

    value = _gather(lambda h, block: _join(
        *[tile(h, unit // 2, (unit + lane) % 2) for lane, unit in enumerate(block)]))
    return functools.lru_cache(maxsize=None)(lambda key: value(key).astype(dtype))


def _expand(plan, lhs, weight, n_sets, done):
    parts = {}

    def finished(h, x, value):
        parts[h, x] = value
        if all((i, x) in parts for i in range(n_sets)):
            done(x, [parts[i, x] for i in range(n_sets)])

    add = _scatter([wide for _, _, wide in plan], finished)
    for j, narrow, wide in plan:
        product = _dot(lhs(narrow), weight(j))
        add(wide, product)
        yield product


def _reduce(plan, tile, weight, totals, dtype):
    def finished(h, block, value):
        for lane, unit in enumerate(block):
            totals[h][unit, lane] = _add(totals[h].get((unit, lane)), 1, value)

    lhs = _gather(tile)
    add = _scatter([narrow for _, narrow, _ in plan], finished)
    for j, narrow, wide in plan:
        product = _dot(lhs(wide).astype(dtype), weight(j))
        add(narrow, product)
        yield product


def _fold(totals):
    return {(u // 2, u % 2): _join(x, totals.get((u ^ 1, 1), x))
            for (u, lane), x in sorted(totals.items()) if lane == 0} | {
                (u // 2, 1 - u % 2): x
                for (u, lane), x in sorted(totals.items()) if lane and (u ^ 1, 0) not in totals}


def _merge(tiles):
    out = [tiles[i, 0] + _swap(tiles[i, 1]) if (i, 1) in tiles else tiles[i, 0]
           for i in range(_UNITS // 2 + 1)]
    return jnp.concatenate(out[:-1] + [out[-1][:, :_UNIT]], axis=1)


def _weave(main, side=(), first=0, every=1):
    side = iter(side)
    for i, _ in enumerate(main):
        if i >= first and (i - first) % every == 0:
            next(side, None)
    for _ in side:
        pass


def _take(gen, n):
    _weave(itertools.islice(gen, n))


def _layernorm(x):
    m = jnp.mean(x, axis=-1, keepdims=True)
    d = x - m
    v = jnp.mean(d * d, axis=-1, keepdims=True)
    return d * jax.lax.rsqrt(v + _EPS)


def _reciprocal(x):
    return pltpu.reciprocal(x, approx=True)


def _dot(a, b):
    return jax.lax.dot_general(a, b, (((1,), (0,)), ((), ())),
                               preferred_element_type=jnp.float32)


def _dot_nt(a, b):
    return jax.lax.dot_general(a, b, (((1,), (1,)), ((), ())),
                               preferred_element_type=jnp.float32)


def _unpack(words):
    return pltpu.bitcast(words, jnp.bfloat16)


class _Tiles:
    def __init__(self, ref, first=0, rows=_LANES):
        self.ref, self.first, self.rows = ref, first, rows

    def shifted(self, by, limit):
        rows = pl.ds(pl.multiple_of(by, 16), self.ref.shape[0] - limit)
        return _Tiles(self.ref.at[rows], self.first, self.rows)

    def load_words(self, j, rows=None):
        start = (self.first + j * self.rows) // 2
        return self.ref.bitcast(jnp.uint32)[pl.ds(start, (rows or self.rows) // 2), :]

    def store_words(self, j, words, at=0):
        start = (self.first + j * self.rows + at) // 2
        self.ref.bitcast(jnp.uint32)[pl.ds(start, words.shape[0]), :] = words

    def load(self, j):
        return _unpack(self.load_words(j))

    def store(self, j, value, at=0):
        start = self.first + j * self.rows + at
        self.ref[pl.ds(start, value.shape[0]), :] = value.astype(jnp.bfloat16)


def _attention_masks(n_layers, n_mem, seg):
    rows = n_layers * (n_mem + seg)
    i = jax.lax.broadcasted_iota(jnp.int32, (rows, rows), 0)
    j = jax.lax.broadcasted_iota(jnp.int32, (rows, rows), 1)
    visible = (i < n_layers * n_mem) | (i >= j)
    if n_layers == 1:
        return visible, _MASKED * _LOG2E

    def second_layer(r):
        return ((r >= n_mem) & (r < 2 * n_mem)) | (r >= 2 * n_mem + seg)

    same = second_layer(i) == second_layer(j)
    fill = jnp.where(same, _MASKED * _LOG2E, -jnp.inf).astype(jnp.float32)
    return same & visible, fill


def _start(copies):
    for c in copies:
        c.start(priority=_PRIORITY)


_SCOPES = False
_WAITS = itertools.count()


def _wait(copies):
    if _SCOPES:
        with jax.named_scope(f"wait{next(_WAITS):02d}"):
            for c in copies:
                c.wait()
        return
    for c in copies:
        c.wait()


class _Pacer:
    def __init__(self, zero):
        self.zero, self.after = zero.astype(jnp.uint32), None

    def hold(self, words):
        if self.after is None:
            return words
        return words | _stack([self.after] * (words.shape[0] // 8))

    def hold_rows(self, x):
        zeros = _stack([pltpu.bitcast(self.after, jnp.float32)] * (x.shape[0] // 8))
        return x + jnp.concatenate([zeros] * (_UNITS // 2) + [zeros[:, :_UNIT]], axis=1)

    def run(self, products, chores, rate):
        for i, product in enumerate(products):
            count = int((i + 1) * rate) - int(i * rate)
            if count:
                self.after = pltpu.bitcast(product[:8], jnp.uint32) & self.zero
                _take(chores, count)
            yield product


def _build_rows(tiles, weights, words):
    value = _gather(lambda u, x: _unpack(words(u, x)).astype(jnp.float32))
    for j, _, _ in _HIDDEN.ordered(1, 2, _PLAIN):
        for lane, key in enumerate(weights[j]):
            if _is_leaf(key):
                tiles.store_words(j, words(*key), lane * _UNIT)
            else:
                tiles.store(j, value(key), lane * _UNIT)
        yield


def _build_transposed(tiles, weights, chosen, words, pacer):
    for j in chosen:
        first = _leaves(weights[j][0])[0]

        def rows(*key):
            return pacer.hold(words(*key)) if key == first else words(*key)

        if all(_is_leaf(key) for key in weights[j]):
            tile = _unpack(_stack([rows(*key) for key in weights[j]]))
        else:
            value = _gather(lambda u, x: _unpack(rows(u, x)).astype(jnp.float32))
            tile = _stack([value(key) for key in weights[j]]).astype(jnp.bfloat16)
        tiles.store_words(j, pltpu.bitcast(tile.T, jnp.uint32))
        yield


def _build_output(tiles, raw_ref, for_single, pacer):
    single = [j for j, _, _ in _HEADS.single]
    chosen = single if for_single else [
        j for j, _, _ in _HEADS.ordered(*_O_OUT) if j not in single]
    return _build_transposed(
        tiles, _HEADS.weights, chosen,
        lambda u, x: raw_ref[x, u * _UNIT // 2:(u + 1) * _UNIT // 2, :], pacer)


def _prologue(xt_hbm, w_hbms, wot_hbm, later_copies, tile_ref, res_ref, early, weights, zero,
              raw_ref, normed_ref, stage0_ref, stage1_ref, sems, *, seg):
    n_heads = raw_ref.shape[0]
    stages = (stage0_ref, stage1_ref, stage0_ref)
    next_sem = itertools.count()

    def copies(pairs):
        sem = sems.at[next(next_sem)]
        return [pltpu.make_async_copy(src, dst, sem) for src, dst in pairs]

    def head_copies(which, pairs):
        return copies((w_hbms[which].bitcast(jnp.uint32).at[:, p, :], stages[which].at[p])
                      for p in pairs)

    x_chunks = [range(a, b) for a, b in zip(_X_CUTS, _X_CUTS[1:])]
    q_chunks = [range(a, b) for a, b in zip(_Q_CUTS, _Q_CUTS[1:])]
    queue = [copies((xt_hbm.at[:, pl.ds(i * _LANES, _LANES)], tile_ref.at[i]) for i in chunk)
             for chunk in x_chunks]
    queue += [head_copies(0, chunk) for chunk in q_chunks]
    queue += [head_copies(1, range(n_heads // 2))]
    v_sem = sems.at[next(next_sem)]
    wo_copies = copies([(wot_hbm.bitcast(jnp.uint32), raw_ref),
                        (xt_hbm.at[:, pl.ds(0, _LANES)], tile_ref.at[0])])
    arrived = itertools.count()

    def advance():
        i = next(arrived)
        _wait(queue[i])
        if i + 2 < len(queue):
            _start(queue[i + 2])

    n_early = (res_ref.shape[0] // seg - _LAG) // 2
    sums = _Tiles(weights[4].ref, 0, n_early // 2 * _KNOWN)
    _start(queue[0])
    _start(queue[1])
    advance()
    x = _stack([tile_ref[i].astype(jnp.float32).T for i in x_chunks[0]])
    res_ref[pl.ds(_LAG * seg, x.shape[0]), :] = x
    normed_ref[...] = _layernorm(x[:2 * sums.rows])
    fresh = _operands([normed_ref[:sums.rows, :], normed_ref[sums.rows:, :]], jnp.float32)
    slots = {}
    pacer = _Pacer(zero)

    def lhs(key):
        if key not in slots:
            slots[key] = len(slots)
            sums.store(slots[key], fresh(key))
        return sums.load(slots[key])

    def raw(which, unit, x, hold=lambda words: words):
        words = hold(stages[which][x // 2, unit * _UNIT:(unit + 1) * _UNIT, :])
        words = words & jnp.uint32(0xFFFF0000) if x % 2 else words << 16
        return pltpu.bitcast(words, jnp.float32)

    def build(which, j, *hold):
        value = _gather(lambda u, x: raw(which, u, x, *hold))
        weights[which].store(j, _stack([value(key) for key in _HEADS.weights[j]]))

    def sweep(which, plan):
        def weight(j):
            build(which, j)
            return weights[which].load(j)

        return _expand(plan, lhs, weight, 2,
                       lambda x, halves: early[which].store(x, _stack(halves)))

    def extra(which):
        return (build(which, j, pacer.hold)
                for j in range(len(_HEADS.double), len(_HEADS.weights)))

    def needs(product):
        last = max(x for key in _HEADS.weights[product[0]] for _, x in _leaves(key)) // 2
        return sum(cut <= last for cut in _Q_CUTS[1:])

    plan = sorted(_HEADS.ordered(1, 2, _PLAIN), key=needs)
    products = sweep(0, plan)
    for c in range(len(q_chunks) - 1):
        advance()
        _take(products, sum(needs(product) <= c for product in plan) // _MXUS * _MXUS
              - sum(needs(product) < c for product in plan) // _MXUS * _MXUS)
    advance()
    _weave(pacer.run(products, extra(0), 0.5))
    advance()
    pl.loop(0, n_heads // 2)(lambda p: pltpu.make_async_copy(
        w_hbms[2].bitcast(jnp.uint32).at[:, p, :], stages[2].at[p], v_sem).start())
    products = pacer.run(sweep(1, _HEADS.ordered(1, 2, _PLAIN)), extra(1), 0.25)
    _take(products, _WO_START)
    _start(wo_copies)
    _weave(products)
    _wait([pltpu.make_async_copy(stages[2], stages[2], v_sem)])
    _start(later_copies[0])
    products = pacer.run(sweep(2, _HEADS.ordered(1, 2, _PLAIN)), extra(2), 0.5)
    _take(products, _WO_AT)
    _wait(wo_copies)
    _start(later_copies[1])
    res_ref[:_LANES, :] = tile_ref[0].astype(jnp.float32).T
    _weave(pacer.run(products, _build_output(weights[3], raw_ref, True, pacer),
                     len(_HEADS.single) / (len(_HEADS.double) - _WO_AT - 4)))


def _layers(xt_hbm, outt_hbm, mem0_ref, ffn_copies, tile_ref, res_ref, early, weights, raw_refs,
            w2t_hbm, rawo_ref, zero, tile_sem, raw2_ref, act_ref, out_ref, q_ref, k_ref, v_ref, pair_ref, old_ref, normed_ref, final_ref,
            *, seg):
    n_mem = mem0_ref.shape[0]
    n_heads = len(_HEADS.blocks)
    n_io = tile_ref.shape[0]
    n_seg = res_ref.shape[0] // seg
    n_pairs = (n_seg - _LAG) // 2
    n_ffn = len(_HIDDEN.double)
    score_scale = _LANES ** -0.5 * _LOG2E
    qkv_tiles = [_Tiles(ref, 0, 2 * n_mem + seg) for ref in (q_ref, k_ref, v_ref)]

    kept = [tiles.shifted(zero, 0) if _PIN else tiles for tiles in qkv_tiles]

    def w2_copy(r):
        rows = raw2_ref.shape[0] // _LAG
        rows = pl.ds(pl.multiple_of(r * rows, 8), rows)
        return pltpu.make_async_copy(w2t_hbm.bitcast(jnp.uint32).at[rows], raw2_ref.at[rows],
                                     tile_sem.at[0])

    x_copies = [pltpu.make_async_copy(xt_hbm.at[:, pl.ds(i * _LANES, _LANES)], tile_ref.at[i],
                                      tile_sem.at[1]) for i in range(_X_CUTS[-1], n_io)]

    def block(r, n=1):
        return pl.ds(pl.multiple_of(r * seg, seg), n * seg)

    def attention(plan, out_plan, sets, dtype, keep, fetch, filler=None, lead=0, n_filler=0, spill=0,
                  first=0, firstv=0, squeeze=0,
                  pace=lambda which, products: products):
        n_layers = len(sets)
        lhs = _operands(sets, dtype)
        visible, fill = _attention_masks(n_layers, n_mem, seg)
        probs, heads, totals = {}, {}, [{} for _ in sets]
        order = list(dict.fromkeys(x for _, _, wide in out_plan for _, x in _leaves(wide)))

        def split(x):
            tokens = n_layers * n_mem
            return [_stack([x[i * n_mem:(i + 1) * n_mem],
                            x[tokens + i * seg:tokens + (i + 1) * seg]]) for i in range(n_layers)]


        def project(which):
            return pace(which, _expand(plan, lhs, weights[which].load, n_layers,
                                       functools.partial(keep, which)))

        def softmax(s):
            if n_layers == 1 or not _MERGED:
                s = jnp.where(visible, s * score_scale, fill)
                p = jnp.exp2(s - jnp.max(s, axis=-1, keepdims=True))
                return p * _reciprocal(jnp.sum(p, axis=-1, keepdims=True))
            shape = (n_mem + seg, s.shape[1])
            i = jax.lax.broadcasted_iota(jnp.int32, shape, 0)
            j = jax.lax.broadcasted_iota(jnp.int32, shape, 1)
            second = ((j >= n_mem) & (j < 2 * n_mem)) | (j >= 2 * n_mem + seg)
            seen = (i < n_mem) | (i + n_mem >= jnp.where(second, j - seg, j))

            def per_layer(reduce, x, neutral):
                return jnp.where(
                    second, reduce(jnp.where(second, x, neutral), axis=-1, keepdims=True),
                    reduce(jnp.where(second, neutral, x), axis=-1, keepdims=True))

            s1, s2 = split(s)
            s = jnp.where(seen, jnp.where(second, s2, s1) * score_scale, _MASKED * _LOG2E)
            p = jnp.exp2(s - per_layer(jnp.max, s, -jnp.inf))
            p = p * _reciprocal(per_layer(jnp.sum, p, 0.0))
            p1, p2 = jnp.where(second, 0.0, p), jnp.where(second, p, 0.0)
            return _stack([p1[:n_mem], p2[:n_mem], p1[n_mem:], p2[n_mem:]])

        def scores():
            for h in order:
                probs[h] = softmax(_dot_nt(fetch(0, h), fetch(1, h))).astype(keep.dtype)
                if len(probs) % _MXUS == 0:
                    yield

        def values():
            for h in order:
                heads[h] = split(_dot(probs[h], fetch(2, h)))
                if len(heads) % _MXUS == 0:
                    yield

        def head(h, x):
            while x not in heads:
                next(mixed)
            return heads[x][h]

        n = len(plan)
        mixed = values()
        output = pace(3, _reduce(out_plan, head, weights[3].load, totals, jnp.float32))
        _weave(project(0))
        _weave(project(1))
        if filler:
            _weave(itertools.chain(itertools.islice(filler, lead), project(2)), scores(), first,
                   ((n + lead) // n_heads - squeeze) * _MXUS)
            _weave(itertools.chain(itertools.islice(filler, n_filler - lead), output), mixed,
                   firstv, (n_filler - lead + spill) // n_heads * _MXUS)
        else:
            _weave(project(2), scores(), 15, (n - 16) // n_heads * _MXUS)
            _take(mixed, 3)
            _weave(output, mixed, 3, n // 16 // _MXUS * _MXUS)
        return [_fold(t) for t in totals]

    def gated(sets):
        lhs = _operands(sets, jnp.bfloat16)
        gates = {}

        def gate(x, halves):
            gates[x] = [g * _reciprocal(1.0 + jnp.exp2(g * -_LOG2E)) for g in halves]

        def up(x, halves):
            for h in range(2):
                act_ref[x, h] = gates[x][h] * halves[h]

        yield from _expand(_HIDDEN.ordered(*_O_UP), lhs, weights[4].load, 2, gate)
        yield from _expand(_HIDDEN.ordered(*_O_UP), lhs, weights[5].load, 2, up)

    def down(ffn=None):
        totals = [{}, {}]
        gen = _reduce(_HIDDEN.ordered(*_O_DOWN), lambda h, x: act_ref[x, h], weights[6].load, totals,
                      jnp.bfloat16)
        if ffn:
            _take(gen, _D0)
            for _ in range(_F0 // _MXUS):
                _take(ffn, _MXUS)
                _take(gen, _D1)
        _weave(gen)
        return [_merge(_fold(t)) for t in totals]

    def single_step(x, mem, *filler, **options):
        qkv = {}

        def keep(which, h, parts):
            qkv[which, h] = parts[0].astype(jnp.bfloat16) if which else parts[0]

        keep.dtype = jnp.float32
        out = _merge(*attention(_HEADS.single, _HEADS.single, [_stack([mem, _layernorm(x)])], jnp.float32,
                                keep, lambda which, h: qkv[which, h], *filler, **options))
        return x + out[n_mem:], out[:n_mem]

    def head_step(r, mem):
        _wait(ffn_copies(r))
        pl.when((r > 0) & (r + 1 < _LAG))(lambda: _start(ffn_copies(r + 1)))
        w2_copy(r).start()
        pl.when(r == 0)(lambda: _start(x_copies))
        pacer = _Pacer(zero)
        chores = itertools.chain(*[
            _build_rows(tiles.shifted(r * 16, _UNIT - 16), _HIDDEN.weights[:n_ffn],
                        lambda u, x, raw=raw: pacer.hold(raw[r % 2, u, :, x * _LANES:(x + 1) * _LANES]))
            for raw, tiles in zip(raw_refs, weights[4:])])
        _take(chores, _AHEAD)
        res_ref[block(r), :], mem = single_step(
            res_ref[block(r), :], mem, pace=lambda which, products: pacer.run(products, chores, _CHORES[which]))
        _weave(chores)
        return mem

    def double_step(j, slot, mems, x2, chores, *filler):
        ahead = n_pairs + 3 * j + slot
        x1 = res_ref[pl.ds(pl.multiple_of(_LAG * seg + ahead * _KNOWN, _KNOWN),
                           (1 + slot) * _KNOWN), :]
        h = _stack([_layernorm(x1), _layernorm(x2)])
        sets = [_stack([mems[0], h[:h.shape[0] // 2]]), _stack([mems[1], h[h.shape[0] // 2:]])]
        later = [[ring.shifted((ahead + i) % _RING * _KNOWN, ring.rows - _KNOWN) for ring in early]
                 for i in range(1 + slot)]
        now = [ring.shifted((2 * j + slot) * seg % ring.rows, ring.rows - seg) for ring in early]

        def keep(which, x, parts):
            tokens = _stack([p[n_mem:] for p in parts])
            qkv_tiles[which].store(slot * n_heads + x,
                                   _stack([p[:n_mem] for p in parts] + [tokens[-seg:]]))
            for i, rings in enumerate(later):
                rings[which].store(x, tokens[i * _KNOWN:(i + 1) * _KNOWN])

        def fetch(which, x):
            words = kept[which].load_words(slot * n_heads + x)
            return _unpack(_stack([words[:n_mem], now[which].load_words(x, seg), words[n_mem:]]))

        keep.dtype = jnp.float32 if _P_F32 else jnp.bfloat16
        when, gap = _PACE_B if slot else _PACE_A
        return attention(_HEADS.ordered(*_O_QKV), _HEADS.ordered(*_O_OUT), sets, jnp.float32 if slot else jnp.bfloat16, keep,
                         fetch, *filler,
                         pace=lambda which, products:
                         pacer.run(products, chores, 1 / gap) if which == when else products)

    folded = list(_fold(dict.fromkeys(_HEADS.places)))

    pacer = _Pacer(zero)
    pieces = [slice(r, r + 8) for r in range(0, seg, 8)]

    def pair_step(j, mems, x2, chores=iter(()), ffn=None):
        x1 = res_ref[block(2 * j + _LAG, 2), :]
        out = [_merge(t) for t in
               double_step(j, 0, mems, x2[:seg], chores, ffn, _LEAD, _F2, _SPILL, _FIRST, _FIRSTV, _SQUEEZE)]

        def park():
            for h, x in enumerate((x1, x2)):
                for rows in pieces:
                    first = pacer.hold_rows(x[rows]) + out[h][n_mem:][rows]
                    pair_ref[h, rows, :] = first
                    normed_ref[h, rows, :] = _layernorm(first)
                    yield
                    pair_ref[h, seg + rows.start:seg + rows.stop, :] = pacer.hold_rows(x[seg:][rows])
                    yield

        if ffn:
            _take(ffn, _F3)
        tiles = double_step(j, 1, [o[:n_mem] for o in out], x2[seg:], park(),
                            ffn, _LEAD_B, 2 * n_ffn - _F0 - _F1 - _F2 - _F3, _SPILL_B, _FIRST_B, _FIRSTV_B, _SQUEEZE_B)
        for h in range(2):
            for i, key in enumerate(folded):
                out_ref[h, i] = tiles[h][key]

    def finish_pair():
        out = [_merge({key: out_ref[h, i] for i, key in enumerate(folded)}) for h in range(2)]
        second = [pair_ref[h, seg:, :] + out[h][n_mem:] for h in range(2)]
        return ([o[:n_mem] for o in out],
                [_stack([pair_ref[h, :seg, :], second[h]]) for h in range(2)],
                [_stack([normed_ref[h], _layernorm(second[h])]) for h in range(2)])

    def hand_over(xs, j=None, y=None):
        for r in range(0, 2 * seg, 8):
            if j is not None:
                at = pl.ds(pl.multiple_of(j % 2 * 2 * seg + r, 8), 8)
                final_ref[at, :] = pacer.hold_rows(old_ref[1, r:r + 8, :]) + y[r:r + 8]
            old_ref[1, r:r + 8, :] = pacer.hold_rows(xs[1][r:r + 8])
            yield
            old_ref[0, r:r + 8, :] = pacer.hold_rows(xs[0][r:r + 8])
            yield
        if j is not None:
            tile_ref[j // 2 - 1] = final_ref[...].T.astype(tile_ref.dtype)

    def steady(j):
        mems, xs, normed = finish_pair()
        ffn = gated(normed)
        y = down(ffn)
        _take(ffn, _F1)
        pair_step(j, mems, old_ref[0] + y[0], hand_over(xs, j, y[1]), ffn)

    out_copies = [
        pltpu.make_async_copy(tile_ref.at[i],
                              outt_hbm.at[:, pl.ds(i * _LANES, _LANES)], tile_sem.at[i])
        for i in range(n_io)]

    if _ONLY == "pair":
        pl.loop(2, n_pairs)(steady)
        _start(out_copies)
        _wait(out_copies)
        return
    if _ONLY != "tail":
        mem0 = mem0_ref[...].astype(jnp.float32)
        mem1 = jax.lax.fori_loop(0, _LAG, head_step, mem0)
        xs = [res_ref[block(2 * h, 2), :] for h in range(2)]
        _wait([w2_copy(r) for r in range(_LAG)] + x_copies)

        def transpose_in():
            for i in range(_X_CUTS[-1], n_io):
                x = _unpack(pacer.hold(tile_ref.bitcast(jnp.uint32)[i]))
                res_ref[i * _LANES:(i + 1) * _LANES, :] = x.astype(jnp.float32).T
                yield

        chores = _build_transposed(
            weights[6], _HIDDEN.weights, [j for j, _, _ in _HIDDEN.ordered(*_O_DOWN)], lambda u, x:
            raw2_ref[u * _UNIT // 2:(u + 1) * _UNIT // 2, x * _LANES:(x + 1) * _LANES], pacer)
        _weave(pacer.run(gated([_layernorm(x) for x in xs]), chores, _W2_RATE))
        pacer.after = None
        _weave(chores)
        xs = [x + y for x, y in zip(xs, down())]
        if _ONLY in ("head", "start"):
            tile_ref[n_io - 1] = _stack(xs).astype(tile_ref.dtype).T
            _start(out_copies)
            _wait(out_copies)
            return
        _weave(_build_output(weights[3], rawo_ref, False, pacer))
        pair_step(0, [mem1, mem0], xs[0], transpose_in())
        mems, ready, normed = finish_pair()
        ffn = gated(normed)
        _take(ffn, _F0 + _F1)
        final_ref[...] = jnp.zeros(final_ref.shape, final_ref.dtype)
        pair_step(1, mems, xs[1], hand_over(ready), ffn)
        if _ONLY == "ramp":
            tile_ref[0, :40] = out_ref[zero, zero].astype(tile_ref.dtype) + (act_ref[zero, 0, :40] + old_ref[zero, :40, :128] + pair_ref[zero, :40, :128]).astype(tile_ref.dtype)
            _start(out_copies)
            _wait(out_copies)
            return
        pl.loop(2, n_pairs)(steady)

    _start(out_copies[:n_io - 2])
    mems, xs, normed = finish_pair()
    ffn = gated(normed)
    older = [old_ref[h] + y for h, y in enumerate(down(ffn))]
    _take(ffn, _F1)
    x0, mem = single_step(older[0][:seg], mems[1], ffn, 48, 128, 0, 15, 15, 1)
    _weave(ffn)
    totals = [{}, {}]
    ffn = _reduce(_HIDDEN.ordered(*_O_DOWN), lambda h, x: act_ref[x, h], weights[6].load, totals,
                  jnp.bfloat16)
    x1, mem = single_step(older[0][seg:], mem, ffn, 128, n_ffn, 0, 15, 15, 1)
    newer = [x + _merge(_fold(t)) for x, t in zip(xs, totals)]
    tile_ref[n_io - 2] = _stack([older[1], newer[1]]).T.astype(tile_ref.dtype)
    x2, mem = single_step(newer[0][:seg], mem)
    out_copies[n_io - 2].start()
    x3, mem = single_step(newer[0][seg:], mem)
    xs = [_stack([x0, x1]), _stack([x2, x3])]
    _weave(gated([_layernorm(x) for x in xs]))
    tile_ref[n_io - 1] = (_stack(xs) + _stack(down())).T.astype(tile_ref.dtype)
    out_copies[n_io - 1].start()
    _wait(out_copies)


def _kernel(xt_hbm, mem0_hbm, wq_hbm, wk_hbm, wv_hbm, wot_hbm, w1_hbm, w3_hbm, w2t_hbm,
            outt_hbm, mem0_ref, tile_ref, res_ref, eq_ref, ek_ref, ev_ref, w_ref, ffn_ref,
            rawo_ref, raw1_ref, raw3_ref, zero_ref, tile_sem, raw_sem, *, seg):
    d_model, n_heads, _ = wq_hbm.shape
    n_mem = mem0_ref.shape[0]
    weights = [_Tiles(ref, i * ref.shape[0] // n) for ref, n in ((w_ref, 4), (ffn_ref, 3))
               for i in range(n)]
    early = [_Tiles(ref, 0, _RING * _KNOWN) for ref in (eq_ref, ek_ref, ev_ref)]
    raw_refs = (raw1_ref, raw3_ref)

    @pl.loop(0, 2)
    def _(i):
        zero_ref[i] = i

    zero = zero_ref[0]

    def ffn_copies(r):
        rows = pl.ds(pl.multiple_of(r * 8, 8), 8)
        return [pltpu.make_async_copy(src.bitcast(jnp.uint32).at[:, rows, :], dst.at[r % 2],
                                      raw_sem.at[r])
                for src, dst in zip((w1_hbm, w3_hbm), raw_refs)]

    mem_copy = pltpu.make_async_copy(mem0_hbm, mem0_ref, raw_sem.at[_LAG])
    if _ONLY in (None, "prologue", "start"):
        pl.run_scoped(
            functools.partial(_prologue, xt_hbm, (wq_hbm, wk_hbm, wv_hbm), wot_hbm,
                              [[mem_copy] + ffn_copies(0), ffn_copies(1)], tile_ref, res_ref,
                              early, weights, zero, rawo_ref, seg=seg),
            pltpu.VMEM(((res_ref.shape[0] // seg - _LAG) // 2 * _KNOWN, d_model), jnp.float32),
            pltpu.VMEM((n_heads // 2, d_model, _LANES), jnp.uint32),
            pltpu.VMEM((n_heads // 2, d_model, _LANES), jnp.uint32),
            pltpu.SemaphoreType.DMA((len(_X_CUTS) + len(_Q_CUTS) + 1,)))
        _wait([mem_copy])
    if _ONLY == "prologue":
        _wait(ffn_copies(0) + ffn_copies(1))

        @pl.loop(0, 8)
        def _(i):
            tile_ref[0, :_LANES, :] = weights[0].shifted(i * 16, 128).load(0) + sum(e.shifted(i * 16, 128).load(0)[:_LANES] for e in early) + res_ref[pl.ds(i * _LANES, _LANES), :_LANES].astype(jnp.bfloat16)
        pltpu.sync_copy(tile_ref.at[0], outt_hbm.at[:, pl.ds(0, _LANES)])
        return
    pl.run_scoped(
        functools.partial(_layers, xt_hbm, outt_hbm, mem0_ref, ffn_copies, tile_ref, res_ref, early,
                          weights, raw_refs, w2t_hbm, rawo_ref, zero, tile_sem, seg=seg),
        pltpu.VMEM((d_model // 2, w2t_hbm.shape[1]), jnp.uint32),
        pltpu.VMEM((len(_HIDDEN.blocks), 2, 2 * seg, _LANES), jnp.float32),
        pltpu.VMEM((2, _UNITS + 1, n_mem + seg, _LANES), jnp.float32),
        *[pltpu.VMEM((2 * n_heads * (2 * n_mem + seg), _LANES), jnp.bfloat16)] * 3,
        *[pltpu.VMEM((2, 2 * seg, d_model), jnp.float32)] * 2,
        pltpu.VMEM((2, seg, d_model), jnp.float32),
        pltpu.VMEM((_LANES, d_model), jnp.float32))


@functools.partial(jax.jit, static_argnames=("A_seg_len",))
def pallas_interleave_layers__memory_aug_recurrent_mem_tr__glu_gated_swiglu__prompt_kernel(
    A_x: jax.Array,
    A_mem0: jax.Array,
    A_Wq: jax.Array,
    A_Wk: jax.Array,
    A_Wv: jax.Array,
    A_Wo: jax.Array,
    A_seg_len: int,
    B_x: jax.Array,
    B_w1: jax.Array,
    B_w3: jax.Array,
    B_w2: jax.Array,
):
    del B_x
    _, n_tok, d_model = A_x.shape
    n_mem = A_mem0.shape[1]
    _, n_heads, d_head = A_Wq.shape
    d_ff = B_w1.shape[1]
    seg = A_seg_len
    n_known = (n_tok // seg - _LAG) // 2 * _KNOWN
    hbm = pl.BlockSpec(memory_space=pltpu.HBM)
    out_t = pl.pallas_call(
        functools.partial(_kernel, seg=seg),
        out_shape=jax.ShapeDtypeStruct((d_model, n_tok), A_x.dtype),
        in_specs=[hbm] * 9,
        out_specs=hbm,
        scratch_shapes=[
            pltpu.VMEM((n_mem, d_model), A_mem0.dtype),
            pltpu.VMEM((n_tok // _LANES, d_model, _LANES), A_x.dtype),
            pltpu.VMEM((n_tok, d_model), jnp.float32),
            *[pltpu.VMEM((n_heads * _RING * _KNOWN, d_head), jnp.bfloat16)] * 3,
            pltpu.VMEM((4 * len(_HEADS.weights) * _LANES, _LANES), jnp.bfloat16),
            pltpu.VMEM((3 * len(_HIDDEN.double) * _LANES, _LANES), jnp.bfloat16),
            pltpu.VMEM((n_heads, d_model // 2, d_head), jnp.uint32),
            *[pltpu.VMEM((2, _UNITS, 8, d_ff), jnp.uint32)] * 2,
            pltpu.SMEM((2,), jnp.int32),
            pltpu.SemaphoreType.DMA((n_tok // _LANES,)),
            pltpu.SemaphoreType.DMA((_LAG + 1,)),
        ],
        compiler_params=pltpu.CompilerParams(vmem_limit_bytes=127 * 1024 * 1024, flags=_FLAGS),
    )(A_x.reshape(n_tok, d_model).T, A_mem0.reshape(n_mem, d_model), A_Wq, A_Wk, A_Wv,
      A_Wo.transpose(0, 2, 1), *[w.reshape(_UNITS, _UNIT, d_ff) for w in (B_w1, B_w3)], B_w2.T)
    return out_t.T.reshape(A_x.shape)
```

```python
import collections
import functools
import itertools
import math

import jax
import jax.numpy as jnp
import jax.experimental.pallas as pl
import jax.experimental.pallas.tpu as pltpu
import numpy as np

_EPS = 1e-05
_MASKED = -1000000000.0
_LOG2E = math.log2(math.e)
_LANES = 128
_MXUS = 4
_PACKED = 16
_UNIT = _LANES // 2
_UNITS = 9
_LAG = 4
_SCORE_SCALE = _LANES ** -0.5 * _LOG2E

_Timing = collections.namedtuple(
    "_Timing", "scores_at scores_gap filler rounds_at rounds_gap chores_gap")
_FIRST_STEP = _Timing(71, 72, 156, 15, 40, 13)
_SECOND_STEP = _Timing(79, 40, 183, 31, 68, 13)
_BARE_STEP = _Timing(79, 24, 0, 3, 24, 12)
_GATES_AT = 148
_GATES_INSIDE = 40
_GATES_AFTER = 71
_QUERY_CUTS = (0, 4, 8, 12, 16)
_OUTPUT_COPY_AT = 60
_OUTPUT_BUILD_AT = 140
_HELD_BACK = 32
_HEAD_CHORES = (0.6, 1.4, 0.6, 0.8)


def _sum(terms):
    terms = sorted(terms, key=lambda term: -term[0])
    return terms[0][1] if len(terms) == 1 and terms[0][0] == 1 else tuple(terms)


def _is_leaf(key):
    return isinstance(key[0], int)


def _leaves(key):
    return [key] if _is_leaf(key) else [leaf for _, term in key for leaf in _leaves(term)]


class _Scheme:
    def __init__(self, period, blocks, links, orient=tuple):
        self.period, self.n_links = period, len(links)
        links = [tuple((orbit, (s + shift) % period) for orbit, shift in link)
                 for s in range(period) for link in links]
        nodes = list(dict.fromkeys(node for link in links for node in link))
        links = [tuple(nodes.index(node) for node in link) for link in links]
        ways = [orbit // 2 for orbit, _ in nodes]
        blocks = [orient([u if u >= period else (u + s) % period for u in blocks[orbit]])
                  for orbit, s in nodes]
        cells, products, owner = [], {}, {}

        def form(side, tiles, p):
            if len(tiles) > (2 if p == 2 else 1):
                key = ((1, form(side, tiles[:-1], p)[1]), (1, form(side, tiles[-1:], p)[1]))
            elif p == 2:
                key = ((1, form(side, tiles, 0)[1]), (1 - 2 * side, form(side, tiles, 1)[1]))
            else:
                key = (p, blocks[tiles[0]]) if side == 0 else (1 - p, tiles[0])
            return (-1 if p == 2 * (1 - side) else 1), key

        def use(narrow, wide, sign):
            weight = products.setdefault((narrow[1], wide[1]), {})
            weight[len(cells) - 1] = sign * narrow[0] * wide[0]

        def cross(u, v, both, p):
            q, r = (p + 1) % 3, (p + 2) % 3
            mixed = []
            for side in range(2):
                (s, a), (t, b) = form(side, u, q), form(side, v, p)
                mixed.append((s, ((1, a), (-s * t, b))))
            for cell, sign in (((u, v), 1), ((v, u), -1)):
                cells.append(cell)
                for tiles, pair in ((both, (p, q)), (u, (r, q)), (v, (p, r))):
                    i, j = pair[::sign]
                    use(form(0, tiles, i), form(1, tiles, j), sign)
                use(*mixed, sign)

        for i, link in enumerate(links):
            for x in link:
                if ((x,), (x,)) not in cells:
                    cells.append(((x,), (x,)))
                    for sign in (1, -1):
                        use(form(0, (x,), (ways[x] + sign) % 3),
                            form(1, (x,), (ways[x] - sign) % 3), sign)
            before = len(cells)
            cross(link[:1], link[1:2], link[:2], 0)
            if len(link) == 3 and ways[link[2]]:
                cross(link[2:], link[:2], link, 1)
            elif len(link) == 3:
                cross(link[:2], link[2:], link, 2)
            owner.update(dict.fromkeys(range(before, len(cells)), i))
        self.products = [(j, narrow, wide) for j, (narrow, wide) in enumerate(products)]
        self.links = [[owner[j] for j in weight if j in owner] for weight in products.values()]

        sums = list(products.values())
        own = [products[form(0, (x,), 1 - ways[x])[1], form(1, (x,), 2)[1]]
               for x in range(len(nodes))]
        self.single = []
        for j, (rows, cols) in enumerate(cells):
            weight = own[rows[0]] if rows == cols else {j: -1} if {j: -1} in sums else {j: 1}
            if weight not in sums:
                sums.append(weight)
            if rows != cols:
                rows, cols = (rows + cols[:len(cols) == 1 and j in own[cols[0]]],
                              cols + rows[:len(rows) == 1 and j in own[rows[0]]])
            self.single.append((sums.index(weight), form(0, rows, 0)[1],
                                ((weight[j], form(1, cols, 1)[1]),)))

        basis = np.zeros((_UNITS, len(nodes), len(cells), 2))
        for j, (rows, cols) in enumerate(cells):
            for x, y, lane in itertools.product(rows, cols, range(2)):
                basis[blocks[x][lane], y, j, lane] += 1
        basis = basis.reshape(2 * len(cells), -1)
        inverse = np.clip(np.rint(np.linalg.inv(basis)), -1, 1)
        assert (inverse @ basis == np.eye(len(basis))).all()
        raw = [[_sum((int(half[u, x]), (int(u), int(x))) for u, x in np.argwhere(half))
                for half in cell] for cell in inverse.reshape(len(cells), 2, _UNITS, -1)]
        self.weights = [[_sum((sign, raw[j][lane]) for j, sign in weight.items())
                         for lane in range(2)] for weight in sums]
        self.n_tiles = len(nodes)
        self.places = sorted({(u, lane) for block in blocks for lane, u in enumerate(block)})

    def last_tile(self, j):
        return max(x for key in self.weights[j] for _, x in _leaves(key))

    def plan(self, step, pick, visits):
        rank = {(s * step + shift) % self.period * self.n_links + link: (s, i)
                for s in range(self.period) for i, (link, shift) in enumerate(visits)}

        def position(product):
            ranks = sorted(rank[i] for i in dict.fromkeys(self.links[product[0]]))
            return ranks[min(pick, len(ranks) - 1)], (len(ranks) > 1) == (pick > 0)

        return sorted(self.products, key=position)


def _by_parity(block):
    low, high = sorted(block)
    if high == _UNITS - 1:
        return (high, low) if low % 2 else (low, high)
    return (low, high) if high % 2 else (high, low)


_HEADS = _Scheme(8, ((7, 0), (7, 3), (8, 6), (5, 6)),
                 (((0, 6), (2, 6), (0, 3)), ((0, 6), (3, 4)), ((1, 1), (3, 4)),
                  ((1, 1), (3, 1), (2, 5)), ((1, 1), (2, 7))))
_HIDDEN = _Scheme(9, ((0, 3), (3, 2), (6, 5), (5, 8)),
                  (((0, 3), (2, 3), (0, 4)), ((0, 3), (3, 2)), ((1, 3), (3, 3), (3, 2)),
                   ((1, 3), (2, 4)), ((1, 0), (2, 4))), _by_parity)
_IN_ORDER = tuple((link, 0) for link in range(5))
_SWEEP_PLAN = _HEADS.plan(1, 2, _IN_ORDER)
_QKV_PLAN = _HEADS.plan(1, 0, _IN_ORDER)
_OUTPUT_PLAN = _HEADS.plan(5, 1, ((3, 0), (4, 0), (0, 1), (1, 1), (2, 5)))
_UP_PLAN = _HIDDEN.plan(1, 2, _IN_ORDER)
_DOWN_PLAN = _HIDDEN.plan(5, 2, ((1, 8), (2, 8), (0, 3), (3, 6), (4, 0)))


def _add(total, sign, value):
    if total is None:
        return value if sign > 0 else -value
    return total + value if sign > 0 else total - value


def _gather(leaf):
    @functools.lru_cache(maxsize=None)
    def value(key):
        if _is_leaf(key):
            return leaf(*key)
        total = None
        for sign, term in key:
            total = _add(total, sign, value(term))
        return total

    return value


def _scatter(keys, done):
    missing, totals = {}, {}

    def count(key):
        missing[key] = missing.get(key, 0) + 1
        if missing[key] == 1 and not _is_leaf(key):
            for _, term in key:
                count(term)

    def add(key, value, sign=1):
        if key in totals:
            old_sign, old = totals[key]
            if old_sign >= sign:
                sign, value = old_sign, _add(old, sign * old_sign, value)
            else:
                value = value - old
        totals[key] = sign, value
        missing[key] -= 1
        if missing[key]:
            return
        if _is_leaf(key):
            done(*key, _add(None, sign, value))
        else:
            for factor, term in key:
                add(term, value, sign * factor)

    for key in keys:
        count(key)
    return add


def _stack(parts):
    return parts[0] if len(parts) == 1 else jnp.concatenate(parts, axis=0)


def _join(low, high):
    return low if low is high else jnp.concatenate([low[:, :_UNIT], high[:, _UNIT:]], axis=1)


def _swap(x):
    return jnp.concatenate([x[:, _UNIT:], x[:, :_UNIT]], axis=1)


def _dot(a, b):
    return jax.lax.dot_general(a, b, (((1,), (0,)), ((), ())),
                               preferred_element_type=jnp.float32)


def _operands(sets, dtype):
    @functools.lru_cache(maxsize=None)
    def tile(h, i, swapped):
        if i == _UNITS // 2:
            return jnp.concatenate([sets[h][:, -_UNIT:]] * 2, axis=1)
        return _swap(tile(h, i, 0)) if swapped else sets[h][:, i * _LANES:(i + 1) * _LANES]

    value = _gather(lambda h, block: _join(
        *[tile(h, unit // 2, (unit + lane) % 2) for lane, unit in enumerate(block)]))
    return functools.lru_cache(maxsize=None)(lambda key: value(key).astype(dtype))


def _expand(plan, lhs, weight, n_sets, done):
    parts = {}

    def finished(h, x, value):
        parts[h, x] = value
        if all((i, x) in parts for i in range(n_sets)):
            done(x, [parts[i, x] for i in range(n_sets)])

    add = _scatter([wide for _, _, wide in plan], finished)
    for j, narrow, wide in plan:
        product = _dot(lhs(narrow), weight(j))
        add(wide, product)
        yield product


def _reduce(plan, tile, weight, totals, dtype):
    def finished(h, block, value):
        for lane, unit in enumerate(block):
            totals[h][unit, lane] = _add(totals[h].get((unit, lane)), 1, value)

    lhs = _gather(tile)
    add = _scatter([narrow for _, narrow, _ in plan], finished)
    for j, narrow, wide in plan:
        product = _dot(lhs(wide).astype(dtype), weight(j))
        add(narrow, product)
        yield product


def _fold(totals):
    tiles = {}
    for unit, lane in sorted(totals):
        x = totals[unit, lane]
        if lane == 0:
            tiles[unit // 2, unit % 2] = _join(x, totals[unit ^ 1, 1] if unit < _UNITS - 1 else x)
        elif unit == _UNITS - 1:
            tiles[unit // 2, 1] = x
        else:
            assert (unit ^ 1, 0) in totals
    return tiles


def _merge(tiles):
    out = [tiles[i, 0] + _swap(tiles[i, 1]) if (i, 1) in tiles else tiles[i, 0]
           for i in range(_UNITS // 2 + 1)]
    return jnp.concatenate(out[:-1] + [out[-1][:, :_UNIT]], axis=1)


def _run(main, side=(), first=0, every=1):
    side = iter(side)
    for i, _ in enumerate(main):
        if i >= first and (i - first) % every == 0:
            next(side, None)
    for _ in side:
        pass


def _take(items, n):
    _run(itertools.islice(items, n))


def _layernorm(x):
    m = jnp.mean(x, axis=-1, keepdims=True)
    d = x - m
    v = jnp.mean(d * d, axis=-1, keepdims=True)
    return d * jax.lax.rsqrt(v + _EPS)


def _reciprocal(x):
    return pltpu.reciprocal(x, approx=True)


def _unpack(words):
    return pltpu.bitcast(words, jnp.bfloat16)


class _Tiles:
    def __init__(self, ref, rows=_LANES, first=0):
        self.ref, self.rows, self.first = ref, rows, first

    def shifted(self, by, limit, step):
        view = pl.ds(pl.multiple_of(by * step, step), self.ref.shape[0] - limit * step)
        return _Tiles(self.ref.at[view], self.rows, self.first)

    def load_words(self, j, rows=None, at=0):
        start = (self.first + j * self.rows + at) // 2
        return self.ref.bitcast(jnp.uint32)[pl.ds(start, (rows or self.rows) // 2), :]

    def store_words(self, j, words, at=0):
        start = (self.first + j * self.rows + at) // 2
        self.ref.bitcast(jnp.uint32)[pl.ds(start, words.shape[0]), :] = words

    def load(self, j, rows=None):
        return _unpack(self.load_words(j, rows))

    def store(self, j, value, at=0):
        start = self.first + j * self.rows + at
        self.ref[pl.ds(start, value.shape[0]), :] = value.astype(jnp.bfloat16)


class _Pacer:
    def __init__(self, zero):
        self.zero, self.after = zero.astype(jnp.uint32), None

    def hold(self, words):
        if self.after is None:
            return words
        return words | _stack([self.after] * (words.shape[0] // 8))

    def hold_rows(self, x):
        zeros = pltpu.bitcast(self.after, jnp.float32)
        return x + jnp.concatenate([zeros] * (_UNITS // 2) + [zeros[:, :_UNIT]], axis=1)

    def spread(self, passes, chores, rate):
        for i, product in enumerate(passes):
            count = int((i + 1) * rate) - int(i * rate)
            if count:
                self.after = pltpu.bitcast(product[:8], jnp.uint32) & self.zero
                _take(chores, count)
            yield product


def _build_rows(tiles, scheme, chosen, words):
    value = _gather(lambda u, x: _unpack(words(u, x)).astype(jnp.float32))
    for j in chosen:
        for lane, key in enumerate(scheme.weights[j]):
            if _is_leaf(key):
                tiles.store_words(j, words(*key), lane * _UNIT)
            else:
                tiles.store(j, value(key), lane * _UNIT)
        yield


def _build_transposed(tiles, scheme, chosen, words, pacer):
    for j in chosen:
        halves = scheme.weights[j]

        def rows(*key):
            return pacer.hold(words(*key)) if key == _leaves(halves[0])[0] else words(*key)

        if all(_is_leaf(key) for key in halves):
            tile = _unpack(_stack([rows(*key) for key in halves]))
        else:
            value = _gather(lambda u, x: _unpack(rows(u, x)).astype(jnp.float32))
            tile = _stack([value(key) for key in halves]).astype(jnp.bfloat16)
        tiles.store_words(j, pltpu.bitcast(tile.T, jnp.uint32))
        yield


def _unit_words(u):
    return slice(u * _UNIT // 2, (u + 1) * _UNIT // 2)


def _lane_tile(i):
    return pl.ds(i * _LANES, _LANES)


def _used(plan):
    return list(dict.fromkeys(x for _, _, wide in plan for _, x in _leaves(wide)))


def _start(copies):
    for c in copies:
        c.start()


def _wait(copies):
    for c in copies:
        c.wait()


def _attention_rounds(tokens, memories, n_mem, seg, shared, out):
    rows = n_mem + seg
    lane = jax.lax.broadcasted_iota(jnp.int32, (rows, _LANES), 1)
    row = jax.lax.broadcasted_iota(jnp.int32, (rows, _LANES), 0)
    visible = (row < n_mem) | (lane >= 3 * seg) | (row - n_mem >= lane % seg)

    @functools.lru_cache(maxsize=None)
    def window(i, slot, n=rows):
        j = jax.lax.broadcasted_iota(jnp.int32, (n, _LANES), 1)
        at = 3 * seg + slot * n_mem
        return ((j >= i * seg) & (j < (i + 1) * seg)) | ((j >= at) & (j < at + n_mem))

    def windows(triple):
        slots = (0, 1, 2 + triple[2][1])
        return slots, [window(i, slot) for i, slot in enumerate(slots)]

    def stacked(which, triple):
        return _stack([tokens(which, *problem) for problem in triple]
                      + [memories(which, triple[0][0]), memories(which, triple[2][0])])

    def query(x, layer):
        mem = _unpack(memories(0, x)).astype(jnp.float32)[layer * n_mem:(layer + 1) * n_mem]
        return _stack([mem, _unpack(tokens(0, x, layer)).astype(jnp.float32)])

    def by_rows(slots, piece):
        upper = jax.lax.broadcasted_iota(jnp.int32, (n_mem, _LANES), 0) < n_mem // 2
        parts = [piece(i, slice(i * seg // 2, (i + 1) * seg // 2)) for i in range(3)]
        for pair in range(2):
            at = slice(3 * seg // 2 + pair * n_mem, 3 * seg // 2 + (pair + 1) * n_mem)
            parts.append(jnp.where(upper, *[
                piece(slots.index(slot) if slot in slots else None, at)
                for slot in (2 * pair, 2 * pair + 1)]))
        return _unpack(_stack(parts))

    def pick(inside, parts):
        return jnp.where(inside[0], parts[0], jnp.where(inside[1], parts[1], parts[2]))

    def softmax(inside, s):
        s = jnp.where(visible, s * _SCORE_SCALE, _MASKED * _LOG2E)
        p = jnp.exp2(s - pick(inside, [
            jnp.max(jnp.where(k, s, -jnp.inf), axis=-1, keepdims=True) for k in inside]))
        return p * _reciprocal(pick(inside, [
            jnp.sum(jnp.where(k, p, 0.0), axis=-1, keepdims=True) for k in inside]))

    def keys(triple):
        return pltpu.bitcast(_unpack(stacked(1, triple)).T, jnp.uint32)

    def scores(triple, n=3):
        kt = _unpack(keys(triple))
        parts = [_dot(query(*problem), kt) for problem in triple[:n]]
        inside = windows(triple)[1]
        return softmax(inside, pick(inside, parts + parts[:3 - n]))

    def values(triple, p, n=3):
        v = _unpack(stacked(2, triple))
        for problem, k in zip(triple[:n], windows(triple)[1]):
            out[problem] = _dot(jnp.where(k, p, 0.0), v)

    def both(triple, earlier, p):
        slots, inside = windows(triple)
        assert slots == windows(earlier)[0]
        kt, v, q = keys(triple), stacked(2, earlier), [query(*problem) for problem in triple]

        def columns(i, words, keep=True):
            if i is None:
                return jnp.zeros_like(words)
            k = window(i, slots[i], words.shape[0])
            return jnp.where(k, words, 0) if keep else jnp.where(k, 0, words)

        s = _dot(pick(inside, q), by_rows(slots, lambda i, at: columns(i, kt[at])))
        o = _dot(jnp.where(inside[0] | inside[1] | inside[2], p, 0.0),
                 by_rows(slots, lambda i, at: columns(i, v[at])))
        mixed = [_dot(jnp.where(inside[i], p, q[i]), by_rows(
            slots, lambda j, at: columns(i, v[at], False) if j == i else columns(i, kt[at])))
                 for i in range(3)]
        for problem, k, x in zip(earlier, inside, mixed):
            out[problem] = jnp.where(k, o, x)
        return softmax(inside, s + pick(inside, mixed))

    order = _used(_OUTPUT_PLAN)
    pairs = [((x, 0), (x, 1), (x, 0)) for x in order[:2]]
    triples = [((order[i + 2 * layer], 0), (order[i + 2 * layer], 1), (order[i + 1], layer))
               for i in range(2, len(order), 3) for layer in range(2)]
    rounds = [triples[i:i + _MXUS] for i in range(0, len(triples), _MXUS)]
    first = [scores(pair, 2) for pair in pairs]
    yield
    waiting = []
    for group in rounds[:1] if shared else rounds:
        waiting.append([(triple, scores(triple)) for triple in group])
        yield
    for pair, p in zip(pairs, first):
        values(pair, p, 2)
    for group in rounds[len(waiting):]:
        waiting = [[(triple, both(triple, *done)) for triple, done in zip(group, waiting[0])]]
        yield
    for group in waiting:
        for done in group:
            values(*done)
        yield


class _Kernel:
    def __init__(self, seg, xt_hbm, mem0_hbm, wq_hbm, wk_hbm, wv_hbm, wot_hbm, w1_hbm, w3_hbm,
                 w2t_hbm, outt_hbm, mem0_ref, tile_ref, x_ref, attention_ref, ffn_ref, wo_ref,
                 w1_ref, w3_ref, q_ref, k_ref, v_ref, count_ref, sems):
        self.seg, self.n_mem = seg, mem0_ref.shape[0]
        self.n_pairs = (x_ref.shape[0] // seg - _LAG) // 2
        self.n_first = 1 + pl.cdiv(self.n_pairs * _PACKED, _LANES)
        self.xt_hbm, self.outt_hbm, self.wot_hbm, self.w2t_hbm = xt_hbm, outt_hbm, wot_hbm, w2t_hbm
        self.qkv_hbm, self.up_hbm = (wq_hbm, wk_hbm, wv_hbm), (w1_hbm, w3_hbm)
        self.mem0_ref, self.tile_ref, self.x_ref = mem0_ref, tile_ref, x_ref
        self.wo_ref, self.up_refs, self.sems = wo_ref, (w1_ref, w3_ref), sems
        self.attention, self.ffn = [
            [_Tiles(ref, _LANES, i * ref.shape[0] // n) for i in range(n)]
            for ref, n in ((attention_ref, 4), (ffn_ref, 3))]
        ring = (self.n_pairs + 2) * _PACKED
        self.ahead = [_Tiles(ref, _PACKED) for ref in (q_ref, k_ref, v_ref)]
        self.current = [_Tiles(ref, _PACKED + seg, _HEADS.n_tiles * ring)
                        for ref in (q_ref, k_ref, v_ref)]
        self.mem_copy = pltpu.make_async_copy(mem0_hbm, mem0_ref, sems.at[_LAG])

        @pl.loop(0, count_ref.shape[0])
        def _(i):
            count_ref[i] = i

        self.zero = count_ref[0]

    def x_copy(self, i, sem):
        return pltpu.make_async_copy(self.xt_hbm.at[:, _lane_tile(i)], self.tile_ref.at[i], sem)

    def up_copies(self, r):
        rows = pl.ds(pl.multiple_of(r * 8, 8), 8)
        return [pltpu.make_async_copy(src.bitcast(jnp.uint32).at[:, rows, :], dst.at[r % 2],
                                      self.sems.at[r])
                for src, dst in zip(self.up_hbm, self.up_refs)]

    def put_ahead(self, which, x, value, at):
        for r in range(0, value.shape[0], _PACKED):
            self.ahead[which].store((at + r) // _PACKED * _HEADS.n_tiles + x, value[r:r + _PACKED])

    def build_output(self, chosen, pacer):
        return _build_transposed(self.attention[3], _HEADS, chosen,
                                 lambda u, x: self.wo_ref[x, _unit_words(u), :], pacer)

    def start_up(self, even_ref, odd_ref, sems):
        stages = (even_ref, odd_ref, even_ref)
        rows = self.n_pairs * _PACKED // 2
        pacer = _Pacer(self.zero)

        def pair_copy(which, p, sem):
            return pltpu.make_async_copy(self.qkv_hbm[which].bitcast(jnp.uint32).at[:, p, :],
                                         stages[which].at[p], sems.at[sem])

        def build(which, j, hold=lambda words: words):
            def raw(u, x):
                words = hold(stages[which][x // 2, u * _UNIT:(u + 1) * _UNIT, :])
                return pltpu.bitcast(words & jnp.uint32(0xFFFF0000) if x % 2 else words << 16,
                                     jnp.float32)

            self.attention[which].store(j, _stack(list(map(_gather(raw), _HEADS.weights[j]))))

        def sweep(which, plan, n=rows):
            def lhs(key):
                if key not in slots:
                    slots[key] = len(slots)
                    sums.store(slots[key], fresh(key))
                return sums.load(slots[key], n)

            def weight(j):
                build(which, j)
                return self.attention[which].load(j)

            def done(x, sets):
                for h, value in enumerate(sets):
                    self.put_ahead(which, x, value, h * rows)

            chores = (build(which, j, pacer.hold)
                      for j in range(len(plan), len(_HEADS.weights)))
            return _expand(plan, lhs, weight, 2, done), chores

        def chunk(product):
            return sum(cut <= _HEADS.last_tile(product[0]) // 2 for cut in _QUERY_CUTS[1:])

        queue = [[self.x_copy(i, sems.at[0]) for i in range(1, self.n_first)]]
        queue += [[pair_copy(0, p, 4 + c) for p in range(a, b)]
                  for c, (a, b) in enumerate(zip(_QUERY_CUTS, _QUERY_CUTS[1:]))]
        queue += [[pair_copy(1, p, 1) for p in range(odd_ref.shape[0])]]

        def advance():
            _wait(queue.pop(0))
            for copies in queue[1:2]:
                _start(copies)

        _start(queue[0] + queue[1])
        advance()
        x = _stack([self.tile_ref[i].astype(jnp.float32).T for i in range(1, self.n_first)])
        self.x_ref[pl.ds(_LANES, x.shape[0]), :] = x
        normed = _layernorm(x[:2 * rows])
        fresh, slots = _operands([normed[:rows], normed[rows:]], jnp.float32), {}
        sums = _Tiles(self.ffn[0].ref, rows)

        plan = sorted(_SWEEP_PLAN, key=chunk)
        passes, chores = sweep(0, plan)
        for c in range(len(_QUERY_CUTS) - 2):
            advance()
            _take(passes, sum(chunk(product) <= c for product in plan) // _MXUS * _MXUS
                  - sum(chunk(product) < c for product in plan) // _MXUS * _MXUS)
        advance()
        _run(pacer.spread(passes, chores, 0.5))
        _run(chores)

        advance()
        pl.loop(0, even_ref.shape[0])(lambda p: pair_copy(2, p, 2).start())
        output_copies = [
            pltpu.make_async_copy(self.wot_hbm.bitcast(jnp.uint32), self.wo_ref, sems.at[3]),
            self.x_copy(0, sems.at[3])]
        passes, chores = sweep(1, _SWEEP_PLAN)
        passes = pacer.spread(passes, chores, 0.25)
        _take(passes, _OUTPUT_COPY_AT)
        _start(output_copies)
        _run(passes)
        _run(chores)

        pl.loop(0, even_ref.shape[0])(lambda p: pair_copy(2, p, 2).wait())
        passes, chores = sweep(2, _SWEEP_PLAN, rows - _HELD_BACK)
        _take(pacer.spread(passes, chores, 0.5), _OUTPUT_BUILD_AT)
        _run(chores)
        _wait(output_copies)
        _start([self.mem_copy] + self.up_copies(0) + self.up_copies(1))
        self.x_ref[:_LANES, :] = self.tile_ref[0].astype(jnp.float32).T
        chores = self.build_output([j for j, _, _ in _HEADS.single], pacer)
        _run(pacer.spread(passes, chores,
                          len(_HEADS.single) / (len(plan) - _OUTPUT_BUILD_AT - _MXUS)))
        _run(chores)
        self.mem_copy.wait()


class _Layers:
    def __init__(self, kernel, w2_ref, act_ref, out_ref, pair_ref, old_ref,
                 normed_ref, rows_ref, sems):
        self.k = kernel
        self.w2_ref, self.act_ref, self.out_ref, self.sems = w2_ref, act_ref, out_ref, sems
        self.pair_ref, self.old_ref = pair_ref, old_ref
        self.normed_ref, self.rows_ref = normed_ref, rows_ref
        self.folded = list(_fold(dict.fromkeys(_HEADS.places)))
        self.pacer = _Pacer(kernel.zero)

    def gated(self, sets):
        lhs = _operands(sets, jnp.bfloat16)
        gates = {}

        def gate(x, parts):
            gates[x] = parts

        def up(x, parts):
            for h, g in enumerate(gates[x]):
                self.act_ref[x, h] = g * _reciprocal(1.0 + jnp.exp2(g * -_LOG2E)) * parts[h]

        yield from _expand(_UP_PLAN, lhs, self.k.ffn[0].load, 2, gate)
        yield from _expand(_UP_PLAN, lhs, self.k.ffn[1].load, 2, up)

    def down(self):
        totals = [{}, {}]
        passes = _reduce(_DOWN_PLAN, lambda h, x: self.act_ref[x, h], self.k.ffn[2].load,
                         totals, jnp.bfloat16)
        return passes, lambda: [_merge(_fold(t)) for t in totals]

    def single_step(self, normed, mem, filler=(), lead=0, skip=0, pace=lambda which, p: p):
        plan, weights = _HEADS.single, self.k.attention
        lhs = _operands([_stack([mem, normed])], jnp.float32)
        shape = (mem.shape[0] + normed.shape[0] - skip, mem.shape[0] + normed.shape[0])
        i = jax.lax.broadcasted_iota(jnp.int32, shape, 0) + skip
        visible = (i < mem.shape[0]) | (i >= jax.lax.broadcasted_iota(jnp.int32, shape, 1))
        qkv, probs, heads, totals = {}, {}, {}, {}

        def project(which):
            def keep(x, parts):
                qkv[which, x] = parts[0].astype(jnp.bfloat16) if which else parts[0]

            rows = (lambda key: lhs(key)[skip:]) if skip and not which else lhs
            return pace(which, _expand(plan, rows, weights[which].load, 1, keep))

        def scores():
            for x in _used(plan):
                s = jax.lax.dot_general(qkv[0, x], qkv[1, x], (((1,), (1,)), ((), ())),
                                        preferred_element_type=jnp.float32)
                s = jnp.where(visible, s * _SCORE_SCALE, _MASKED * _LOG2E)
                p = jnp.exp2(s - jnp.max(s, axis=-1, keepdims=True))
                probs[x] = p * _reciprocal(jnp.sum(p, axis=-1, keepdims=True))
                if len(probs) % _MXUS == 0:
                    yield

        def values():
            for x in _used(plan):
                heads[x] = _dot(probs[x], qkv[2, x])
                if len(heads) % _MXUS == 0:
                    yield

        def head(h, x):
            while x not in heads:
                next(rounds)
            return heads[x]

        rounds = values()
        output = pace(3, _reduce(plan, head, weights[3].load, [totals], jnp.float32))
        _run(project(0))
        _run(project(1))
        _run(itertools.chain(itertools.islice(filler, lead), project(2)), scores(), 15,
             (len(plan) + lead - 16) // _HEADS.n_tiles * _MXUS)
        if lead:
            _run(itertools.chain(filler, output), rounds, 15, 8)
        else:
            _take(rounds, 3)
            _run(output, rounds, 3, 8)
        return _merge(_fold(totals))

    def double_step(self, j, second, mems, x2, timing, filler, pace):
        k, seg, n_mem = self.k, self.k.seg, self.k.n_mem
        put = k.n_pairs + 3 * j + second
        x1 = k.x_ref[pl.ds(pl.multiple_of(_LANES + put * _PACKED, _PACKED), (1 + second) * _PACKED), :]
        normed = _stack([_layernorm(x1), _layernorm(x2)])
        half = normed.shape[0] // 2
        lhs = _operands([_stack([mems[0], normed[:half]]), _stack([mems[1], normed[half:]])],
                        jnp.float32 if (n_mem + half) % _PACKED else jnp.bfloat16)
        size, step = k.n_pairs + 2, _HEADS.n_tiles * _PACKED
        later = [[ring.shifted((put + i) % size, size - 1, step) for ring in k.ahead]
                 for i in range(1 + second)]
        now = [ring.shifted((4 * j + 2 * second) % size, size - 2, step) for ring in k.ahead]
        base = second * _HEADS.n_tiles
        heads, totals = {}, [{}, {}]

        def project(which):
            def keep(x, parts):
                rows = _stack([p[n_mem:] for p in parts])
                k.current[which].store(base + x, _stack([p[:n_mem] for p in parts] + [rows[-seg:]]))
                for i, rings in enumerate(later):
                    rings[which].store(x, rows[i * _PACKED:(i + 1) * _PACKED])

            return pace(which, _expand(_QKV_PLAN, lhs, k.attention[which].load, 2, keep))

        def tokens(which, x, layer):
            if layer:
                return k.current[which].load_words(base + x, seg, _PACKED)
            return _stack([now[which].load_words(i * _HEADS.n_tiles + x) for i in range(2)])

        def head(layer, x):
            while (x, layer) not in heads:
                next(rounds)
            return heads[x, layer]

        rounds = _attention_rounds(
            tokens, lambda which, x: k.current[which].load_words(base + x, _PACKED),
            n_mem, seg, timing.filler > 0, heads)
        _run(project(0))
        _run(project(1))
        _run(project(2), itertools.islice(rounds, 2 if timing.filler else 6),
             timing.scores_at, timing.scores_gap)
        output = _reduce(_OUTPUT_PLAN, head, k.attention[3].load, totals, jnp.float32)
        _run(itertools.chain(itertools.islice(filler, timing.filler), output), rounds,
             timing.rounds_at, timing.rounds_gap)
        return [_fold(t) for t in totals]

    def under_keys(self, chores, gap):
        def pace(which, passes):
            yield from self.pacer.spread(passes, chores, (which == 1) / gap)
            if which == 1:
                _run(chores)

        return pace

    def pair(self, j, mems, x2, filler, between, timings, pace):
        seg, n_mem = self.k.seg, self.k.n_mem
        x1 = self.k.x_ref[pl.ds(pl.multiple_of((2 * j + _LAG) * seg, seg), 2 * seg), :]
        out = [_merge(t) for t in self.double_step(j, 0, mems, x2[:seg], timings[0], filler, pace)]

        def park():
            for h, x in enumerate((x1, x2)):
                for r in range(0, seg, 8):
                    first = self.pacer.hold_rows(x[r:r + 8]) + out[h][n_mem + r:n_mem + r + 8]
                    self.pair_ref[h, r:r + 8, :] = first
                    self.normed_ref[h, r:r + 8, :] = _layernorm(first)
                    yield
                    rows = slice(seg + r, seg + r + 8)
                    self.pair_ref[h, rows, :] = self.pacer.hold_rows(x[rows])
                    yield

        _take(filler, between)
        tiles = self.double_step(j, 1, [o[:n_mem] for o in out], x2[seg:], timings[1], filler,
                                 self.under_keys(park(), timings[1].chores_gap))
        for h in range(2):
            for i, key in enumerate(self.folded):
                self.out_ref[h, i] = tiles[h][key]

    def finish_pair(self):
        seg, n_mem = self.k.seg, self.k.n_mem
        out = [_merge({key: self.out_ref[h, i] for i, key in enumerate(self.folded)})
               for h in range(2)]
        second = [self.pair_ref[h, seg:, :] + out[h][n_mem:] for h in range(2)]
        return ([o[:n_mem] for o in out],
                [_stack([self.pair_ref[h, :seg, :], second[h]]) for h in range(2)],
                self.gated([_stack([self.normed_ref[h], _layernorm(second[h])])
                            for h in range(2)]))

    def gated_pair(self, j, mems, x2, xs, filler, taken, first, final=None):
        def hand_over():
            for r in range(0, xs[0].shape[0], 8):
                if final is not None:
                    at = pl.ds(pl.multiple_of(j % 2 * xs[0].shape[0] + r, 8), 8)
                    self.rows_ref[at, :] = (self.pacer.hold_rows(self.old_ref[1, r:r + 8, :])
                                            + final[r:r + 8])
                for h in (1, 0):
                    self.old_ref[h, r:r + 8, :] = self.pacer.hold_rows(xs[h][r:r + 8])
                    yield
            if final is not None:
                self.k.tile_ref[j // 2 - 1] = self.rows_ref[...].T.astype(self.k.tile_ref.dtype)

        between = 2 * len(_UP_PLAN) - taken - first.filler - _SECOND_STEP.filler
        assert between >= 0
        self.pair(j, mems, x2, filler, between, (first, _SECOND_STEP),
                  self.under_keys(hand_over(), first.chores_gap))

    def close_ffn(self):
        mems, xs, filler = self.finish_pair()
        passes, result = self.down()
        _take(passes, _GATES_AT)
        _take(filler, _GATES_INSIDE)
        _run(passes)
        y = result()
        _take(filler, _GATES_AFTER)
        return mems, xs, filler, y

    def steady(self, j):
        mems, xs, filler, y = self.close_ffn()
        self.gated_pair(j, mems, self.old_ref[0] + y[0], xs, filler,
                        _GATES_INSIDE + _GATES_AFTER, _FIRST_STEP, y[1])

    def ramp_up(self):
        k, seg, pacer = self.k, self.k.seg, self.pacer
        rest = range(k.n_first, k.tile_ref.shape[0])
        x_copies = [k.x_copy(i, self.sems.at[1]) for i in rest]
        half = self.w2_ref.shape[1] // 2
        w2_copies = [
            pltpu.make_async_copy(k.w2t_hbm.bitcast(jnp.uint32).at[:, pl.ds(i * half, half)],
                                  self.w2_ref.at[:, pl.ds(i * half, half)], self.sems.at[i])
            for i in range(2)]

        def head_step(r, mem):
            _wait(k.up_copies(r))
            pl.when((r > 0) & (r + 1 < _LAG))(lambda: _start(k.up_copies(r + 1)))
            pl.when(r + 2 == _LAG)(w2_copies[0].start)
            pl.when(r + 1 == _LAG)(lambda: _start(w2_copies[1:] + x_copies))
            local = _Pacer(k.zero)
            chores = itertools.chain(*[
                _build_rows(tiles.shifted(r, _LAG - 1, _PACKED), _HIDDEN,
                            [j for j, _, _ in _UP_PLAN],
                            lambda u, x, ref=ref: local.hold(ref[r % 2, u, :, _lane_tile(x)]))
                for ref, tiles in zip(k.up_refs, k.ffn)])
            _take(chores, 30)
            rows = pl.ds(pl.multiple_of(r * seg, seg), seg)
            out = self.single_step(
                self.rows_ref[rows, :], mem,
                pace=lambda which, passes: local.spread(passes, chores, _HEAD_CHORES[which]))
            _run(chores)
            k.x_ref[rows, :] = k.x_ref[rows, :] + out[k.n_mem:]
            return out[:k.n_mem]

        def held_back():
            ends = [(h + 1) * k.n_pairs * _PACKED // 2 - _HELD_BACK for h in range(2)]
            assert ends[0] >= 4 * seg

            def done(x, sets):
                for at, value in zip(ends, sets):
                    k.put_ahead(2, x, value, at)

            return _expand(_QKV_PLAN, _operands([self.normed_ref[h] for h in range(2)],
                                                jnp.bfloat16), k.attention[2].load, 2, done)

        def transpose_in():
            for i in rest:
                x = _unpack(pacer.hold(k.tile_ref.bitcast(jnp.uint32)[i]))
                k.x_ref[_lane_tile(i), :] = x.astype(jnp.float32).T
                yield

        mem0 = k.mem0_ref[...].astype(jnp.float32)
        self.rows_ref[...] = _layernorm(k.x_ref[:_LANES, :])
        for h in range(2):
            at = _LANES + (h + 1) * k.n_pairs * _PACKED // 2 - _HELD_BACK
            self.normed_ref[h] = _layernorm(k.x_ref[pl.ds(at, _HELD_BACK), :])
        mem1 = jax.lax.fori_loop(0, _LAG, head_step, mem0)

        def build_down(late):
            chosen = [j for j, _, _ in _DOWN_PLAN
                      if (_HIDDEN.last_tile(j) * _LANES >= half) == late]
            return _build_transposed(
                k.ffn[2], _HIDDEN, chosen,
                lambda u, x: self.w2_ref[_unit_words(u), _lane_tile(x)], pacer)

        _wait(w2_copies[:1])
        spare = held_back()
        xs = [k.x_ref[pl.ds(h * 2 * seg, 2 * seg), :] for h in range(2)]
        _take(spare, 56)
        passes, chores = self.gated([_layernorm(x) for x in xs]), build_down(False)
        _take(pacer.spread(passes, chores, 0.4), 260)
        _run(chores)
        _wait(w2_copies[1:] + x_copies)
        chores = build_down(True)
        _run(pacer.spread(passes, chores, 0.45))
        passes, result = self.down()
        _run(pacer.spread(passes, chores, 0.25))
        xs = [x + y for x, y in zip(xs, result())]

        _take(spare, 72)
        single = [j for j, _, _ in _HEADS.single]
        _run(k.build_output([j for j, _, _ in _OUTPUT_PLAN if j not in single], pacer))
        self.pair(0, [mem1, mem0], xs[0], spare, 52, (_BARE_STEP, _BARE_STEP),
                  self.under_keys(transpose_in(), 20))
        _run(spare)
        mems, ready, filler = self.finish_pair()
        extra = _GATES_INSIDE + _GATES_AFTER
        self.gated_pair(1, mems, xs[1], ready, filler, 0,
                        _FIRST_STEP._replace(filler=_FIRST_STEP.filler + extra))

    def wind_down(self):
        k, seg, n_mem = self.k, self.k.seg, self.k.n_mem
        last = k.tile_ref.shape[0] - 1
        copies = [pltpu.make_async_copy(k.tile_ref.at[i], k.outt_hbm.at[:, _lane_tile(i)],
                                        self.sems.at[0]) for i in range(last + 1)]

        def step(x, mem, **options):
            out = self.single_step(_layernorm(x), mem, **options)
            return x + out[-seg:], out[:n_mem]

        _start(copies[:last - 1])
        mems, xs, filler, y = self.close_ffn()
        older = [self.old_ref[h] + y[h] for h in range(2)]
        x0, mem = step(older[0][:seg], mems[1], filler=itertools.islice(filler, 128), lead=48)
        _run(filler)
        passes, result = self.down()
        x1, mem = step(older[0][seg:], mem, filler=passes, lead=128)
        newer = [x + y for x, y in zip(xs, result())]
        k.tile_ref[last - 1] = _stack([older[1], newer[1]]).T.astype(k.tile_ref.dtype)
        x2, mem = step(newer[0][:seg], mem)
        copies[last - 1].start()
        x3, _ = step(newer[0][seg:], mem, skip=n_mem)
        xs = [_stack([x0, x1]), _stack([x2, x3])]
        _run(self.gated([_layernorm(x) for x in xs]))
        passes, result = self.down()
        _run(passes)
        k.tile_ref[last] = (_stack(xs) + _stack(result())).T.astype(k.tile_ref.dtype)
        copies[last].start()
        _wait(copies)


def _kernel(*refs, seg):
    kernel = _Kernel(seg, *refs)
    d_model, rows = _UNITS * _UNIT, kernel.n_mem + seg

    def run_layers(*scratch):
        layers = _Layers(kernel, *scratch)
        layers.ramp_up()
        pl.loop(2, kernel.n_pairs)(layers.steady)
        layers.wind_down()

    pl.run_scoped(
        kernel.start_up,
        *[pltpu.VMEM((_HEADS.n_tiles // 2, d_model, _LANES), jnp.uint32)] * 2,
        pltpu.SemaphoreType.DMA((3 + len(_QUERY_CUTS),)))
    pl.run_scoped(
        run_layers,
        pltpu.VMEM((d_model // 2, _HIDDEN.n_tiles * _LANES), jnp.uint32),
        pltpu.VMEM((_HIDDEN.n_tiles, 2, 2 * seg, _LANES), jnp.float32),
        pltpu.VMEM((2, _UNITS, rows, _LANES), jnp.float32),
        *[pltpu.VMEM((2, 2 * seg, d_model), jnp.float32)] * 2,
        pltpu.VMEM((2, seg, d_model), jnp.float32),
        pltpu.VMEM((_LANES, d_model), jnp.float32),
        pltpu.SemaphoreType.DMA((2,)))


@functools.partial(jax.jit, static_argnames=("A_seg_len",))
def pallas_interleave_layers__memory_aug_recurrent_mem_tr__glu_gated_swiglu__prompt_kernel(
    A_x: jax.Array,
    A_mem0: jax.Array,
    A_Wq: jax.Array,
    A_Wk: jax.Array,
    A_Wv: jax.Array,
    A_Wo: jax.Array,
    A_seg_len: int,
    B_x: jax.Array,
    B_w1: jax.Array,
    B_w3: jax.Array,
    B_w2: jax.Array,
):
    del B_x
    _, n_tok, d_model = A_x.shape
    n_mem, d_ff = A_mem0.shape[1], B_w1.shape[1]
    assert A_x.shape[0] == 1 and _LAG * A_seg_len == _LANES and 2 * n_mem == _PACKED
    assert A_Wq.shape == (_UNITS * _UNIT, _HEADS.n_tiles, _LANES) and n_tok % _LANES == 0
    assert d_ff == _HIDDEN.n_tiles * _LANES
    hbm = pl.BlockSpec(memory_space=pltpu.HBM)
    out_t = pl.pallas_call(
        functools.partial(_kernel, seg=A_seg_len),
        out_shape=jax.ShapeDtypeStruct((d_model, n_tok), A_x.dtype),
        in_specs=[hbm] * 9,
        out_specs=hbm,
        scratch_shapes=[
            pltpu.VMEM((n_mem, d_model), A_mem0.dtype),
            pltpu.VMEM((n_tok // _LANES, d_model, _LANES), A_x.dtype),
            pltpu.VMEM((n_tok, d_model), jnp.float32),
            pltpu.VMEM((4 * len(_HEADS.weights) * _LANES, _LANES), jnp.bfloat16),
            pltpu.VMEM((3 * len(_UP_PLAN) * _LANES, _LANES), jnp.bfloat16),
            pltpu.VMEM((_HEADS.n_tiles, d_model // 2, _LANES), jnp.uint32),
            *[pltpu.VMEM((2, _UNITS, 8, d_ff), jnp.uint32)] * 2,
            *[pltpu.VMEM((_HEADS.n_tiles * (n_tok // 4 + 2 * (_PACKED + A_seg_len)), _LANES),
                         jnp.bfloat16)] * 3,
            pltpu.SMEM((2,), jnp.int32),
            pltpu.SemaphoreType.DMA((_LAG + 1,)),
        ],
        compiler_params=pltpu.CompilerParams(vmem_limit_bytes=127 * 1024 * 1024),
    )(A_x.reshape(n_tok, d_model).T, A_mem0.reshape(n_mem, d_model), A_Wq, A_Wk, A_Wv,
      A_Wo.transpose(0, 2, 1), B_w1.reshape(_UNITS, _UNIT, d_ff),
      B_w3.reshape(_UNITS, _UNIT, d_ff), B_w2.T)
    return out_t.T.reshape(A_x.shape)
```

```python
import collections
import functools
import itertools
import math

import jax
import jax.numpy as jnp
import jax.experimental.pallas as pl
import jax.experimental.pallas.tpu as pltpu
import numpy as np

_EPS = 1e-05
_MASKED = -1000000000.0
_LOG2E = math.log2(math.e)
_LANES = 128
_MXUS = 4
_PACKED = 16
_UNIT = _LANES // 2
_UNITS = 9
_LAG = 4
_SCORE_SCALE = _LANES ** -0.5 * _LOG2E

_Timing = collections.namedtuple(
    "_Timing", "scores_at scores_gap filler rounds_at rounds_gap chores_gap")
_FIRST_STEP = _Timing(71, 72, 156, 15, 40, 13)
_SECOND_STEP = _Timing(79, 40, 183, 31, 68, 13)
_BARE_STEP = _Timing(79, 24, 0, 3, 24, 12)
_GATES_AT = 148
_GATES_INSIDE = 40
_GATES_AFTER = 71
_QUERY_CUTS = (0, 4, 8, 12, 16)
_OUTPUT_COPY_AT = 60
_OUTPUT_BUILD_AT = 140
_HELD_BACK = 32
_HEAD_CHORES = (0.6, 1.4, 0.6, 0.8)


def _sum(terms):
    terms = sorted(terms, key=lambda term: -term[0])
    return terms[0][1] if len(terms) == 1 and terms[0][0] == 1 else tuple(terms)


def _is_leaf(key):
    return isinstance(key[0], int)


def _leaves(key):
    return [key] if _is_leaf(key) else [leaf for _, term in key for leaf in _leaves(term)]


class _Scheme:
    def __init__(self, period, blocks, links, orient=tuple):
        self.period, self.n_links = period, len(links)
        links = [tuple((orbit, (s + shift) % period) for orbit, shift in link)
                 for s in range(period) for link in links]
        nodes = list(dict.fromkeys(node for link in links for node in link))
        links = [tuple(nodes.index(node) for node in link) for link in links]
        ways = [orbit // 2 for orbit, _ in nodes]
        blocks = [orient([u if u >= period else (u + s) % period for u in blocks[orbit]])
                  for orbit, s in nodes]
        cells, products, owner = [], {}, {}

        def form(side, tiles, p):
            if len(tiles) > (2 if p == 2 else 1):
                key = ((1, form(side, tiles[:-1], p)[1]), (1, form(side, tiles[-1:], p)[1]))
            elif p == 2:
                key = ((1, form(side, tiles, 0)[1]), (1 - 2 * side, form(side, tiles, 1)[1]))
            else:
                key = (p, blocks[tiles[0]]) if side == 0 else (1 - p, tiles[0])
            return (-1 if p == 2 * (1 - side) else 1), key

        def use(narrow, wide, sign):
            weight = products.setdefault((narrow[1], wide[1]), {})
            weight[len(cells) - 1] = sign * narrow[0] * wide[0]

        def cross(u, v, both, p):
            q, r = (p + 1) % 3, (p + 2) % 3
            mixed = []
            for side in range(2):
                (s, a), (t, b) = form(side, u, q), form(side, v, p)
                mixed.append((s, ((1, a), (-s * t, b))))
            for cell, sign in (((u, v), 1), ((v, u), -1)):
                cells.append(cell)
                for tiles, pair in ((both, (p, q)), (u, (r, q)), (v, (p, r))):
                    i, j = pair[::sign]
                    use(form(0, tiles, i), form(1, tiles, j), sign)
                use(*mixed, sign)

        for i, link in enumerate(links):
            for x in link:
                if ((x,), (x,)) not in cells:
                    cells.append(((x,), (x,)))
                    for sign in (1, -1):
                        use(form(0, (x,), (ways[x] + sign) % 3),
                            form(1, (x,), (ways[x] - sign) % 3), sign)
            before = len(cells)
            cross(link[:1], link[1:2], link[:2], 0)
            if len(link) == 3 and ways[link[2]]:
                cross(link[2:], link[:2], link, 1)
            elif len(link) == 3:
                cross(link[:2], link[2:], link, 2)
            owner.update(dict.fromkeys(range(before, len(cells)), i))
        self.products = [(j, narrow, wide) for j, (narrow, wide) in enumerate(products)]
        self.links = [[owner[j] for j in weight if j in owner] for weight in products.values()]

        sums = list(products.values())
        own = [products[form(0, (x,), 1 - ways[x])[1], form(1, (x,), 2)[1]]
               for x in range(len(nodes))]
        self.single = []
        for j, (rows, cols) in enumerate(cells):
            weight = own[rows[0]] if rows == cols else {j: -1} if {j: -1} in sums else {j: 1}
            if weight not in sums:
                sums.append(weight)
            if rows != cols:
                rows, cols = (rows + cols[:len(cols) == 1 and j in own[cols[0]]],
                              cols + rows[:len(rows) == 1 and j in own[rows[0]]])
            self.single.append((sums.index(weight), form(0, rows, 0)[1],
                                ((weight[j], form(1, cols, 1)[1]),)))

        basis = np.zeros((_UNITS, len(nodes), len(cells), 2))
        for j, (rows, cols) in enumerate(cells):
            for x, y, lane in itertools.product(rows, cols, range(2)):
                basis[blocks[x][lane], y, j, lane] += 1
        basis = basis.reshape(2 * len(cells), -1)
        inverse = np.clip(np.rint(np.linalg.inv(basis)), -1, 1)
        assert (inverse @ basis == np.eye(len(basis))).all()
        raw = [[_sum((int(half[u, x]), (int(u), int(x))) for u, x in np.argwhere(half))
                for half in cell] for cell in inverse.reshape(len(cells), 2, _UNITS, -1)]
        self.weights = [[_sum((sign, raw[j][lane]) for j, sign in weight.items())
                         for lane in range(2)] for weight in sums]
        self.n_tiles = len(nodes)
        self.places = sorted({(u, lane) for block in blocks for lane, u in enumerate(block)})

    def last_tile(self, j):
        return max(x for key in self.weights[j] for _, x in _leaves(key))

    def plan(self, step, pick, visits):
        rank = {(s * step + shift) % self.period * self.n_links + link: (s, i)
                for s in range(self.period) for i, (link, shift) in enumerate(visits)}

        def position(product):
            ranks = sorted(rank[i] for i in dict.fromkeys(self.links[product[0]]))
            return ranks[min(pick, len(ranks) - 1)], (len(ranks) > 1) == (pick > 0)

        return sorted(self.products, key=position)


def _by_parity(block):
    low, high = sorted(block)
    if high == _UNITS - 1:
        return (high, low) if low % 2 else (low, high)
    return (low, high) if high % 2 else (high, low)


_HEADS = _Scheme(8, ((7, 0), (7, 3), (8, 6), (5, 6)),
                 (((0, 6), (2, 6), (0, 3)), ((0, 6), (3, 4)), ((1, 1), (3, 4)),
                  ((1, 1), (3, 1), (2, 5)), ((1, 1), (2, 7))))
_HIDDEN = _Scheme(9, ((0, 3), (3, 2), (6, 5), (5, 8)),
                  (((0, 3), (2, 3), (0, 4)), ((0, 3), (3, 2)), ((1, 3), (3, 3), (3, 2)),
                   ((1, 3), (2, 4)), ((1, 0), (2, 4))), _by_parity)
_IN_ORDER = tuple((link, 0) for link in range(5))
_SWEEP_PLAN = _HEADS.plan(1, 2, _IN_ORDER)
_QKV_PLAN = _HEADS.plan(1, 0, _IN_ORDER)
_OUTPUT_PLAN = _HEADS.plan(5, 1, ((3, 0), (4, 0), (0, 1), (1, 1), (2, 5)))
_UP_PLAN = _HIDDEN.plan(1, 2, _IN_ORDER)
_DOWN_PLAN = _HIDDEN.plan(5, 2, ((1, 8), (2, 8), (0, 3), (3, 6), (4, 0)))


def _add(total, sign, value):
    if total is None:
        return value if sign > 0 else -value
    return total + value if sign > 0 else total - value


def _gather(leaf):
    @functools.lru_cache(maxsize=None)
    def value(key):
        if _is_leaf(key):
            return leaf(*key)
        total = None
        for sign, term in key:
            total = _add(total, sign, value(term))
        return total

    return value


def _scatter(keys, done):
    missing, totals = {}, {}

    def count(key):
        missing[key] = missing.get(key, 0) + 1
        if missing[key] == 1 and not _is_leaf(key):
            for _, term in key:
                count(term)

    def add(key, value, sign=1):
        if key in totals:
            old_sign, old = totals[key]
            if old_sign >= sign:
                sign, value = old_sign, _add(old, sign * old_sign, value)
            else:
                value = value - old
        totals[key] = sign, value
        missing[key] -= 1
        if missing[key]:
            return
        if _is_leaf(key):
            done(*key, _add(None, sign, value))
        else:
            for factor, term in key:
                add(term, value, sign * factor)

    for key in keys:
        count(key)
    return add


def _stack(parts):
    return parts[0] if len(parts) == 1 else jnp.concatenate(parts, axis=0)


def _join(low, high):
    return low if low is high else jnp.concatenate([low[:, :_UNIT], high[:, _UNIT:]], axis=1)


def _swap(x):
    return jnp.concatenate([x[:, _UNIT:], x[:, :_UNIT]], axis=1)


def _dot(a, b):
    return jax.lax.dot_general(a, b, (((1,), (0,)), ((), ())),
                               preferred_element_type=jnp.float32)


def _operands(sets, dtype):
    @functools.lru_cache(maxsize=None)
    def tile(h, i, swapped):
        if i == _UNITS // 2:
            return jnp.concatenate([sets[h][:, -_UNIT:]] * 2, axis=1)
        return _swap(tile(h, i, 0)) if swapped else sets[h][:, i * _LANES:(i + 1) * _LANES]

    value = _gather(lambda h, block: _join(
        *[tile(h, unit // 2, (unit + lane) % 2) for lane, unit in enumerate(block)]))
    return functools.lru_cache(maxsize=None)(lambda key: value(key).astype(dtype))


def _expand(plan, lhs, weight, n_sets, done):
    parts = {}

    def finished(h, x, value):
        parts[h, x] = value
        if all((i, x) in parts for i in range(n_sets)):
            done(x, [parts[i, x] for i in range(n_sets)])

    add = _scatter([wide for _, _, wide in plan], finished)
    for j, narrow, wide in plan:
        product = _dot(lhs(narrow), weight(j))
        add(wide, product)
        yield product


def _reduce(plan, tile, weight, totals, dtype):
    def finished(h, block, value):
        for lane, unit in enumerate(block):
            totals[h][unit, lane] = _add(totals[h].get((unit, lane)), 1, value)

    lhs = _gather(tile)
    add = _scatter([narrow for _, narrow, _ in plan], finished)
    for j, narrow, wide in plan:
        product = _dot(lhs(wide).astype(dtype), weight(j))
        add(narrow, product)
        yield product


def _fold(totals):
    tiles = {}
    for unit, lane in sorted(totals):
        x = totals[unit, lane]
        if lane == 0:
            tiles[unit // 2, unit % 2] = _join(x, totals[unit ^ 1, 1] if unit < _UNITS - 1 else x)
        elif unit == _UNITS - 1:
            tiles[unit // 2, 1] = x
        else:
            assert (unit ^ 1, 0) in totals
    return tiles


def _merge(tiles):
    out = [tiles[i, 0] + _swap(tiles[i, 1]) if (i, 1) in tiles else tiles[i, 0]
           for i in range(_UNITS // 2 + 1)]
    return jnp.concatenate(out[:-1] + [out[-1][:, :_UNIT]], axis=1)


def _run(main, side=(), first=0, every=1):
    side = iter(side)
    for i, _ in enumerate(main):
        if i >= first and (i - first) % every == 0:
            next(side, None)
    for _ in side:
        pass


def _take(items, n):
    _run(itertools.islice(items, n))


def _layernorm(x):
    m = jnp.mean(x, axis=-1, keepdims=True)
    d = x - m
    v = jnp.mean(d * d, axis=-1, keepdims=True)
    return d * jax.lax.rsqrt(v + _EPS)


def _reciprocal(x):
    return pltpu.reciprocal(x, approx=True)


def _unpack(words):
    return pltpu.bitcast(words, jnp.bfloat16)


class _Tiles:
    def __init__(self, ref, rows=_LANES, first=0):
        self.ref, self.rows, self.first = ref, rows, first

    def shifted(self, by, limit, step):
        view = pl.ds(pl.multiple_of(by * step, step), self.ref.shape[0] - limit * step)
        return _Tiles(self.ref.at[view], self.rows, self.first)

    def load_words(self, j, rows=None, at=0):
        start = (self.first + j * self.rows + at) // 2
        return self.ref.bitcast(jnp.uint32)[pl.ds(start, (rows or self.rows) // 2), :]

    def store_words(self, j, words, at=0):
        start = (self.first + j * self.rows + at) // 2
        self.ref.bitcast(jnp.uint32)[pl.ds(start, words.shape[0]), :] = words

    def load(self, j, rows=None):
        return _unpack(self.load_words(j, rows))

    def store(self, j, value, at=0):
        start = self.first + j * self.rows + at
        self.ref[pl.ds(start, value.shape[0]), :] = value.astype(jnp.bfloat16)


class _Pacer:
    def __init__(self, zero):
        self.zero, self.after = zero.astype(jnp.uint32), None

    def hold(self, words):
        if self.after is None:
            return words
        return words | _stack([self.after] * (words.shape[0] // 8))

    def hold_rows(self, x):
        zeros = pltpu.bitcast(self.after, jnp.float32)
        return x + jnp.concatenate([zeros] * (_UNITS // 2) + [zeros[:, :_UNIT]], axis=1)

    def spread(self, passes, chores, rate):
        for i, product in enumerate(passes):
            count = int((i + 1) * rate) - int(i * rate)
            if count:
                self.after = pltpu.bitcast(product[:8], jnp.uint32) & self.zero
                _take(chores, count)
            yield product


def _build_rows(tiles, scheme, chosen, words):
    value = _gather(lambda u, x: _unpack(words(u, x)).astype(jnp.float32))
    for j in chosen:
        for lane, key in enumerate(scheme.weights[j]):
            if _is_leaf(key):
                tiles.store_words(j, words(*key), lane * _UNIT)
            else:
                tiles.store(j, value(key), lane * _UNIT)
        yield


def _build_transposed(tiles, scheme, chosen, words, pacer):
    for j in chosen:
        halves = scheme.weights[j]

        def rows(*key):
            return pacer.hold(words(*key)) if key == _leaves(halves[0])[0] else words(*key)

        if all(_is_leaf(key) for key in halves):
            tile = _unpack(_stack([rows(*key) for key in halves]))
        else:
            value = _gather(lambda u, x: _unpack(rows(u, x)).astype(jnp.float32))
            tile = _stack([value(key) for key in halves]).astype(jnp.bfloat16)
        tiles.store_words(j, pltpu.bitcast(tile.T, jnp.uint32))
        yield


def _unit_words(u):
    return slice(u * _UNIT // 2, (u + 1) * _UNIT // 2)


def _lane_tile(i):
    return pl.ds(i * _LANES, _LANES)


def _used(plan):
    return list(dict.fromkeys(x for _, _, wide in plan for _, x in _leaves(wide)))


def _start(copies):
    for c in copies:
        c.start()


def _wait(copies):
    for c in copies:
        c.wait()


def _attention_rounds(tokens, memories, n_mem, seg, shared, out):
    rows = n_mem + seg
    lane = jax.lax.broadcasted_iota(jnp.int32, (rows, _LANES), 1)
    row = jax.lax.broadcasted_iota(jnp.int32, (rows, _LANES), 0)
    visible = (row < n_mem) | (lane >= 3 * seg) | (row - n_mem >= lane % seg)
    upper = jax.lax.broadcasted_iota(jnp.int32, (n_mem, _LANES), 0) < n_mem // 2
    zeros, lowest, masked = [jnp.full((rows, _LANES), value, jnp.float32)
                             for value in (0.0, -jnp.inf, _MASKED * _LOG2E)]
    select = jax.lax.select

    @functools.lru_cache(maxsize=None)
    def window(i, slot, n=rows):
        j = jax.lax.broadcasted_iota(jnp.int32, (n, _LANES), 1)
        at = 3 * seg + slot * n_mem
        return ((j >= i * seg) & (j < (i + 1) * seg)) | ((j >= at) & (j < at + n_mem))

    def windows(triple):
        slots = (0, 1, 2 + triple[2][1])
        return slots, [window(i, slot) for i, slot in enumerate(slots)]

    def stacked(which, triple):
        return ([tokens(which, *problem) for problem in triple]
                + [memories(which, triple[0][0]), memories(which, triple[2][0])])

    def query(x, layer):
        mem = _unpack(memories(0, x)).astype(jnp.float32)[layer * n_mem:(layer + 1) * n_mem]
        return _stack([mem, _unpack(tokens(0, x, layer)).astype(jnp.float32)])

    def by_rows(slots, piece):
        parts = [piece(i, i) for i in range(3)]
        for pair in range(2):
            a, b = [piece(slots.index(slot) if slot in slots else None, 3 + pair)
                    for slot in (2 * pair, 2 * pair + 1)]
            parts.append(a if a is b else select(upper, a, b))
        return _unpack(_stack(parts))

    def pick(inside, parts):
        a, b, c = [jnp.broadcast_to(part, zeros.shape) for part in parts]
        return select(inside[0], a, select(inside[1], b, c))

    def softmax(inside, s):
        s = select(visible, s * _SCORE_SCALE, masked)
        p = jnp.exp2(s - pick(inside, [
            jnp.max(select(k, s, lowest), axis=-1, keepdims=True) for k in inside]))
        return p * _reciprocal(pick(inside, [
            jnp.sum(select(k, p, zeros), axis=-1, keepdims=True) for k in inside]))

    def keys(triple):
        return pltpu.bitcast(_unpack(_stack(stacked(1, triple))).T, jnp.uint32)

    def scores(triple, n=3):
        kt = _unpack(keys(triple))
        parts = [_dot(query(*problem), kt) for problem in triple[:n]]
        inside = windows(triple)[1]
        return softmax(inside, pick(inside, parts + parts[:3 - n]))

    def values(triple, p, n=3):
        v = _unpack(_stack(stacked(2, triple)))
        for problem, k in zip(triple[:n], windows(triple)[1]):
            out[problem] = _dot(select(k, p, zeros), v)

    def both(triple, earlier, p):
        slots, inside = windows(triple)
        assert slots == windows(earlier)[0]
        kt, v, q = keys(triple), stacked(2, earlier), [query(*problem) for problem in triple]

        ends = list(itertools.accumulate([0] + [part.shape[0] for part in v]))
        parts = ([kt[a:b] for a, b in zip(ends, ends[1:])], v)
        blank = {part.shape: jnp.zeros_like(part) for part in (v[0], v[-1])}

        @functools.lru_cache(maxsize=None)
        def columns(which, part, i, keep=True):
            words = parts[which][part]
            if i is None:
                return blank[words.shape]
            pair = (words, blank[words.shape])
            return select(window(i, slots[i], words.shape[0]), *pair[::1 if keep else -1])

        s = _dot(pick(inside, q), by_rows(slots, lambda i, part: columns(0, part, i)))
        o = _dot(select(inside[0] | inside[1] | inside[2], p, zeros),
                 by_rows(slots, lambda i, part: columns(1, part, i)))
        mixed = [_dot(select(inside[i], p, q[i]), by_rows(
            slots, lambda j, part: columns(1, part, i, False) if j == i else columns(0, part, i)))
                 for i in range(3)]
        for problem, k, x in zip(earlier, inside, mixed):
            out[problem] = select(k, o, x)
        return softmax(inside, s + pick(inside, mixed))

    order = _used(_OUTPUT_PLAN)
    pairs = [((x, 0), (x, 1), (x, 0)) for x in order[:2]]
    triples = [((order[i + 2 * layer], 0), (order[i + 2 * layer], 1), (order[i + 1], layer))
               for i in range(2, len(order), 3) for layer in range(2)]
    rounds = [triples[i:i + _MXUS] for i in range(0, len(triples), _MXUS)]
    first = [scores(pair, 2) for pair in pairs]
    yield
    waiting = []
    for group in rounds[:1] if shared else rounds:
        waiting.append([(triple, scores(triple)) for triple in group])
        yield
    for pair, p in zip(pairs, first):
        values(pair, p, 2)
    for group in rounds[len(waiting):]:
        waiting = [[(triple, both(triple, *done)) for triple, done in zip(group, waiting[0])]]
        yield
    for group in waiting:
        for done in group:
            values(*done)
        yield


class _Kernel:
    def __init__(self, seg, xt_hbm, mem0_hbm, wq_hbm, wk_hbm, wv_hbm, wot_hbm, w1_hbm, w3_hbm,
                 w2t_hbm, outt_hbm, mem0_ref, tile_ref, x_ref, attention_ref, ffn_ref, wo_ref,
                 w1_ref, w3_ref, q_ref, k_ref, v_ref, count_ref, sems):
        self.seg, self.n_mem = seg, mem0_hbm.shape[0]
        self.n_pairs = (x_ref.shape[0] // seg - _LAG) // 2
        self.n_first = 1 + pl.cdiv(self.n_pairs * _PACKED, _LANES)
        self.xt_hbm, self.outt_hbm, self.wot_hbm, self.w2t_hbm = xt_hbm, outt_hbm, wot_hbm, w2t_hbm
        self.qkv_hbm, self.up_hbm = (wq_hbm, wk_hbm, wv_hbm), (w1_hbm, w3_hbm)
        self.mem0_ref, self.tile_ref, self.x_ref = mem0_ref, tile_ref, x_ref
        self.wo_ref, self.up_refs, self.sems = wo_ref, (w1_ref, w3_ref), sems
        self.attention, self.ffn = [
            [_Tiles(ref, _LANES, i * ref.shape[0] // n) for i in range(n)]
            for ref, n in ((attention_ref, 4), (ffn_ref, 3))]
        ring = (self.n_pairs + 2) * _PACKED
        self.ahead = [_Tiles(ref, _PACKED) for ref in (q_ref, k_ref, v_ref)]
        self.current = [_Tiles(ref, _PACKED + seg, _HEADS.n_tiles * ring)
                        for ref in (q_ref, k_ref, v_ref)]
        self.mem_copy = pltpu.make_async_copy(mem0_hbm, mem0_ref.at[0], sems.at[_LAG])

        @pl.loop(0, count_ref.shape[0])
        def _(i):
            count_ref[i] = i

        self.zero = count_ref[0]

    def x_copy(self, i, sem):
        return pltpu.make_async_copy(self.xt_hbm.at[:, _lane_tile(i)], self.tile_ref.at[i], sem)

    def up_copies(self, r):
        rows = pl.ds(pl.multiple_of(r * 8, 8), 8)
        return [pltpu.make_async_copy(src.bitcast(jnp.uint32).at[:, rows, :], dst.at[r % 2],
                                      self.sems.at[r])
                for src, dst in zip(self.up_hbm, self.up_refs)]

    def put_ahead(self, which, x, value, at):
        for r in range(0, value.shape[0], _PACKED):
            self.ahead[which].store((at + r) // _PACKED * _HEADS.n_tiles + x, value[r:r + _PACKED])

    def build_output(self, chosen, pacer):
        return _build_transposed(self.attention[3], _HEADS, chosen,
                                 lambda u, x: self.wo_ref[x, _unit_words(u), :], pacer)

    def start_up(self, even_ref, odd_ref, sems):
        stages = (even_ref, odd_ref, even_ref)
        rows = self.n_pairs * _PACKED // 2
        pacer = _Pacer(self.zero)

        def pair_copy(which, p, sem):
            return pltpu.make_async_copy(self.qkv_hbm[which].bitcast(jnp.uint32).at[:, p, :],
                                         stages[which].at[p], sems.at[sem])

        def build(which, j, hold=lambda words: words):
            def raw(u, x):
                words = hold(stages[which][x // 2, u * _UNIT:(u + 1) * _UNIT, :])
                return pltpu.bitcast(words & jnp.uint32(0xFFFF0000) if x % 2 else words << 16,
                                     jnp.float32)

            self.attention[which].store(j, _stack(list(map(_gather(raw), _HEADS.weights[j]))))

        def sweep(which, plan, n=rows):
            def lhs(key):
                if key not in slots:
                    slots[key] = len(slots)
                    sums.store(slots[key], fresh(key))
                return sums.load(slots[key], n)

            def weight(j):
                build(which, j)
                return self.attention[which].load(j)

            def done(x, sets):
                for h, value in enumerate(sets):
                    self.put_ahead(which, x, value, h * rows)

            chores = (build(which, j, pacer.hold)
                      for j in range(len(plan), len(_HEADS.weights)))
            return _expand(plan, lhs, weight, 2, done), chores

        def chunk(product):
            return sum(cut <= _HEADS.last_tile(product[0]) // 2 for cut in _QUERY_CUTS[1:])

        queue = [[self.x_copy(i, sems.at[0]) for i in range(1, self.n_first)]]
        queue += [[pair_copy(0, p, 4 + c) for p in range(a, b)]
                  for c, (a, b) in enumerate(zip(_QUERY_CUTS, _QUERY_CUTS[1:]))]
        queue += [[pair_copy(1, p, 1) for p in range(odd_ref.shape[0])]]

        def advance():
            _wait(queue.pop(0))
            for copies in queue[1:2]:
                _start(copies)

        _start(queue[0] + queue[1])
        advance()
        x = _stack([self.tile_ref[i].astype(jnp.float32).T for i in range(1, self.n_first)])
        self.x_ref[pl.ds(_LANES, x.shape[0]), :] = x
        normed = _layernorm(x[:2 * rows])
        fresh, slots = _operands([normed[:rows], normed[rows:]], jnp.float32), {}
        sums = _Tiles(self.ffn[0].ref, rows)

        plan = sorted(_SWEEP_PLAN, key=chunk)
        passes, chores = sweep(0, plan)
        for c in range(len(_QUERY_CUTS) - 2):
            advance()
            _take(passes, sum(chunk(product) <= c for product in plan) // _MXUS * _MXUS
                  - sum(chunk(product) < c for product in plan) // _MXUS * _MXUS)
        advance()
        _run(pacer.spread(passes, chores, 0.5))
        _run(chores)

        advance()
        pl.loop(0, even_ref.shape[0])(lambda p: pair_copy(2, p, 2).start())
        output_copies = [
            pltpu.make_async_copy(self.wot_hbm.bitcast(jnp.uint32), self.wo_ref, sems.at[3]),
            self.x_copy(0, sems.at[3])]
        passes, chores = sweep(1, _SWEEP_PLAN)
        passes = pacer.spread(passes, chores, 0.25)
        _take(passes, _OUTPUT_COPY_AT)
        _start(output_copies)
        _run(passes)
        _run(chores)

        pl.loop(0, even_ref.shape[0])(lambda p: pair_copy(2, p, 2).wait())
        passes, chores = sweep(2, _SWEEP_PLAN, rows - _HELD_BACK)
        _take(pacer.spread(passes, chores, 0.5), _OUTPUT_BUILD_AT)
        _run(chores)
        _wait(output_copies)
        _start([self.mem_copy] + self.up_copies(0) + self.up_copies(1))
        self.x_ref[:_LANES, :] = self.tile_ref[0].astype(jnp.float32).T
        chores = self.build_output([j for j, _, _ in _HEADS.single], pacer)
        _run(pacer.spread(passes, chores,
                          len(_HEADS.single) / (len(plan) - _OUTPUT_BUILD_AT - _MXUS)))
        _run(chores)
        self.mem_copy.wait()


class _Layers:
    def __init__(self, kernel, w2_ref, act_ref, out_ref, pair_ref, old_ref,
                 normed_ref, rows_ref, sems):
        self.k = kernel
        self.w2_ref, self.act_ref, self.out_ref, self.sems = w2_ref, act_ref, out_ref, sems
        self.pair_ref, self.old_ref = pair_ref, old_ref
        self.normed_ref, self.rows_ref = normed_ref, rows_ref
        self.folded = list(_fold(dict.fromkeys(_HEADS.places)))
        self.pacer = _Pacer(kernel.zero)

    def gated(self, sets):
        lhs = _operands(sets, jnp.bfloat16)
        gates = {}

        def gate(x, parts):
            gates[x] = parts

        def up(x, parts):
            for h, g in enumerate(gates[x]):
                self.act_ref[x, h] = g * _reciprocal(1.0 + jnp.exp2(g * -_LOG2E)) * parts[h]

        yield from _expand(_UP_PLAN, lhs, self.k.ffn[0].load, 2, gate)
        yield from _expand(_UP_PLAN, lhs, self.k.ffn[1].load, 2, up)

    def down(self):
        totals = [{}, {}]
        passes = _reduce(_DOWN_PLAN, lambda h, x: self.act_ref[x, h], self.k.ffn[2].load,
                         totals, jnp.bfloat16)
        return passes, lambda: [_merge(_fold(t)) for t in totals]

    def single_step(self, normed, mem, filler=(), lead=0, skip=0, pace=lambda which, p: p):
        plan, weights = _HEADS.single, self.k.attention
        lhs = _operands([_stack([mem, normed])], jnp.float32)
        shape = (mem.shape[0] + normed.shape[0] - skip, mem.shape[0] + normed.shape[0])
        i = jax.lax.broadcasted_iota(jnp.int32, shape, 0) + skip
        visible = (i < mem.shape[0]) | (i >= jax.lax.broadcasted_iota(jnp.int32, shape, 1))
        qkv, probs, heads, totals = {}, {}, {}, {}

        def project(which):
            def keep(x, parts):
                qkv[which, x] = parts[0].astype(jnp.bfloat16) if which else parts[0]

            rows = (lambda key: lhs(key)[skip:]) if skip and not which else lhs
            return pace(which, _expand(plan, rows, weights[which].load, 1, keep))

        def scores():
            for x in _used(plan):
                s = jax.lax.dot_general(qkv[0, x], qkv[1, x], (((1,), (1,)), ((), ())),
                                        preferred_element_type=jnp.float32)
                s = jnp.where(visible, s * _SCORE_SCALE, _MASKED * _LOG2E)
                p = jnp.exp2(s - jnp.max(s, axis=-1, keepdims=True))
                probs[x] = p * _reciprocal(jnp.sum(p, axis=-1, keepdims=True))
                if len(probs) % _MXUS == 0:
                    yield

        def values():
            for x in _used(plan):
                heads[x] = _dot(probs[x], qkv[2, x])
                if len(heads) % _MXUS == 0:
                    yield

        def head(h, x):
            while x not in heads:
                next(rounds)
            return heads[x]

        rounds = values()
        output = pace(3, _reduce(plan, head, weights[3].load, [totals], jnp.float32))
        _run(project(0))
        _run(project(1))
        _run(itertools.chain(itertools.islice(filler, lead), project(2)), scores(), 15,
             (len(plan) + lead - 16) // _HEADS.n_tiles * _MXUS)
        if lead:
            _run(itertools.chain(filler, output), rounds, 15, 8)
        else:
            _take(rounds, 3)
            _run(output, rounds, 3, 8)
        return _merge(_fold(totals))

    def double_step(self, j, second, mems, x2, timing, filler, pace):
        k, seg, n_mem = self.k, self.k.seg, self.k.n_mem
        put = k.n_pairs + 3 * j + second
        x1 = k.x_ref[pl.ds(pl.multiple_of(_LANES + put * _PACKED, _PACKED), (1 + second) * _PACKED), :]
        normed = _stack([_layernorm(x1), _layernorm(x2)])
        half = normed.shape[0] // 2
        lhs = _operands([_stack([mems[0], normed[:half]]), _stack([mems[1], normed[half:]])],
                        jnp.float32 if (n_mem + half) % _PACKED else jnp.bfloat16)
        size, step = k.n_pairs + 2, _HEADS.n_tiles * _PACKED
        later = [[ring.shifted((put + i) % size, size - 1, step) for ring in k.ahead]
                 for i in range(1 + second)]
        now = [ring.shifted((4 * j + 2 * second) % size, size - 2, step) for ring in k.ahead]
        base = second * _HEADS.n_tiles
        heads, totals = {}, [{}, {}]

        def project(which):
            def keep(x, parts):
                rows = _stack([p[n_mem:] for p in parts])
                k.current[which].store(base + x, _stack([p[:n_mem] for p in parts] + [rows[-seg:]]))
                for i, rings in enumerate(later):
                    rings[which].store(x, rows[i * _PACKED:(i + 1) * _PACKED])

            return pace(which, _expand(_QKV_PLAN, lhs, k.attention[which].load, 2, keep))

        def tokens(which, x, layer):
            if layer:
                return k.current[which].load_words(base + x, seg, _PACKED)
            return _stack([now[which].load_words(i * _HEADS.n_tiles + x) for i in range(2)])

        def head(layer, x):
            while (x, layer) not in heads:
                next(rounds)
            return heads[x, layer]

        rounds = _attention_rounds(
            tokens, lambda which, x: k.current[which].load_words(base + x, _PACKED),
            n_mem, seg, timing.filler > 0, heads)
        _run(project(0))
        _run(project(1))
        _run(project(2), itertools.islice(rounds, 2 if timing.filler else 6),
             timing.scores_at, timing.scores_gap)
        output = _reduce(_OUTPUT_PLAN, head, k.attention[3].load, totals, jnp.float32)
        _run(itertools.chain(itertools.islice(filler, timing.filler), output), rounds,
             timing.rounds_at, timing.rounds_gap)
        return [_fold(t) for t in totals]

    def under_keys(self, chores, gap):
        def pace(which, passes):
            yield from self.pacer.spread(passes, chores, (which == 1) / gap)
            if which == 1:
                _run(chores)

        return pace

    def pair(self, j, mems, x2, filler, between, timings, pace):
        seg, n_mem = self.k.seg, self.k.n_mem
        x1 = self.k.x_ref[pl.ds(pl.multiple_of((2 * j + _LAG) * seg, seg), 2 * seg), :]
        out = [_merge(t) for t in self.double_step(j, 0, mems, x2[:seg], timings[0], filler, pace)]

        def park():
            for h, x in enumerate((x1, x2)):
                for r in range(0, seg, 8):
                    first = self.pacer.hold_rows(x[r:r + 8]) + out[h][n_mem + r:n_mem + r + 8]
                    self.pair_ref[h, r:r + 8, :] = first
                    self.normed_ref[h, r:r + 8, :] = _layernorm(first)
                    yield
                    rows = slice(seg + r, seg + r + 8)
                    self.pair_ref[h, rows, :] = self.pacer.hold_rows(x[rows])
                    yield

        _take(filler, between)
        tiles = self.double_step(j, 1, [o[:n_mem] for o in out], x2[seg:], timings[1], filler,
                                 self.under_keys(park(), timings[1].chores_gap))
        for h in range(2):
            for i, key in enumerate(self.folded):
                self.out_ref[h, i] = tiles[h][key]

    def finish_pair(self):
        seg, n_mem = self.k.seg, self.k.n_mem
        out = [_merge({key: self.out_ref[h, i] for i, key in enumerate(self.folded)})
               for h in range(2)]
        second = [self.pair_ref[h, seg:, :] + out[h][n_mem:] for h in range(2)]
        return ([o[:n_mem] for o in out],
                [_stack([self.pair_ref[h, :seg, :], second[h]]) for h in range(2)],
                self.gated([_stack([self.normed_ref[h], _layernorm(second[h])])
                            for h in range(2)]))

    def gated_pair(self, j, mems, x2, xs, filler, taken, first, final=None):
        def hand_over():
            for r in range(0, xs[0].shape[0], 8):
                if final is not None:
                    i, at = divmod(r, self.k.seg)
                    self.rows_ref[j % 2 * 2 + i, at:at + 8, :] = (
                        self.pacer.hold_rows(self.old_ref[1, r:r + 8, :]) + final[r:r + 8])
                for h in (1, 0):
                    self.old_ref[h, r:r + 8, :] = self.pacer.hold_rows(xs[h][r:r + 8])
                    yield
            if final is not None:
                rows = _stack([self.rows_ref[i] for i in range(_LAG)])
                self.k.tile_ref[j // 2 - 1] = rows.T.astype(self.k.tile_ref.dtype)

        between = 2 * len(_UP_PLAN) - taken - first.filler - _SECOND_STEP.filler
        assert between >= 0
        self.pair(j, mems, x2, filler, between, (first, _SECOND_STEP),
                  self.under_keys(hand_over(), first.chores_gap))

    def close_ffn(self):
        mems, xs, filler = self.finish_pair()
        passes, result = self.down()
        _take(passes, _GATES_AT)
        _take(filler, _GATES_INSIDE)
        _run(passes)
        y = result()
        _take(filler, _GATES_AFTER)
        return mems, xs, filler, y

    def steady(self, j):
        mems, xs, filler, y = self.close_ffn()
        self.gated_pair(j, mems, self.old_ref[0] + y[0], xs, filler,
                        _GATES_INSIDE + _GATES_AFTER, _FIRST_STEP, y[1])

    def ramp_up(self):
        k, seg, pacer = self.k, self.k.seg, self.pacer
        rest = range(k.n_first, k.tile_ref.shape[0])
        x_copies = [k.x_copy(i, self.sems.at[1]) for i in rest]
        half = self.w2_ref.shape[1] // 2
        w2_copies = [
            pltpu.make_async_copy(k.w2t_hbm.bitcast(jnp.uint32).at[:, pl.ds(i * half, half)],
                                  self.w2_ref.at[:, pl.ds(i * half, half)], self.sems.at[i])
            for i in range(2)]

        def head_step(r, mem):
            _wait(k.up_copies(r))
            pl.when((r > 0) & (r + 1 < _LAG))(lambda: _start(k.up_copies(r + 1)))
            pl.when(r + 2 == _LAG)(w2_copies[0].start)
            pl.when(r + 1 == _LAG)(lambda: _start(w2_copies[1:] + x_copies))
            local, slot = _Pacer(k.zero), r % 2
            chores = itertools.chain(*[
                _build_rows(tiles.shifted(r, _LAG - 1, _PACKED), _HIDDEN,
                            [j for j, _, _ in _UP_PLAN],
                            lambda u, x, ref=ref: local.hold(ref[slot, u, :, _lane_tile(x)]))
                for ref, tiles in zip(k.up_refs, k.ffn)])
            _take(chores, 30)
            rows = pl.ds(pl.multiple_of(r * seg, seg), seg)
            out = self.single_step(
                self.rows_ref[r], mem,
                pace=lambda which, passes: local.spread(passes, chores, _HEAD_CHORES[which]))
            _run(chores)
            k.x_ref[rows, :] = k.x_ref[rows, :] + out[k.n_mem:]
            return out[:k.n_mem]

        def held_back():
            ends = [(h + 1) * k.n_pairs * _PACKED // 2 - _HELD_BACK for h in range(2)]
            assert ends[0] >= 4 * seg

            def done(x, sets):
                for at, value in zip(ends, sets):
                    k.put_ahead(2, x, value, at)

            return _expand(_QKV_PLAN, _operands([self.normed_ref[h] for h in range(2)],
                                                jnp.bfloat16), k.attention[2].load, 2, done)

        def transpose_in():
            for i in rest:
                x = _unpack(pacer.hold(k.tile_ref.bitcast(jnp.uint32)[i]))
                k.x_ref[_lane_tile(i), :] = x.astype(jnp.float32).T
                yield

        mem0 = k.mem0_ref[0].astype(jnp.float32)
        for r in range(_LAG):
            self.rows_ref[r] = _layernorm(k.x_ref[pl.ds(r * seg, seg), :])
        for h in range(2):
            at = _LANES + (h + 1) * k.n_pairs * _PACKED // 2 - _HELD_BACK
            self.normed_ref[h] = _layernorm(k.x_ref[pl.ds(at, _HELD_BACK), :])
        mem1 = jax.lax.fori_loop(0, _LAG, head_step, mem0)

        def build_down(late):
            chosen = [j for j, _, _ in _DOWN_PLAN
                      if (_HIDDEN.last_tile(j) * _LANES >= half) == late]
            return _build_transposed(
                k.ffn[2], _HIDDEN, chosen,
                lambda u, x: self.w2_ref[_unit_words(u), _lane_tile(x)], pacer)

        _wait(w2_copies[:1])
        spare = held_back()
        xs = [k.x_ref[pl.ds(h * 2 * seg, 2 * seg), :] for h in range(2)]
        _take(spare, 56)
        passes, chores = self.gated([_layernorm(x) for x in xs]), build_down(False)
        _take(pacer.spread(passes, chores, 0.4), 260)
        _run(chores)
        _wait(w2_copies[1:] + x_copies)
        chores = build_down(True)
        _run(pacer.spread(passes, chores, 0.45))
        passes, result = self.down()
        _run(pacer.spread(passes, chores, 0.25))
        xs = [x + y for x, y in zip(xs, result())]

        _take(spare, 72)
        single = [j for j, _, _ in _HEADS.single]
        _run(k.build_output([j for j, _, _ in _OUTPUT_PLAN if j not in single], pacer))
        self.pair(0, [mem1, mem0], xs[0], spare, 52, (_BARE_STEP, _BARE_STEP),
                  self.under_keys(transpose_in(), 20))
        _run(spare)
        mems, ready, filler = self.finish_pair()
        extra = _GATES_INSIDE + _GATES_AFTER
        self.gated_pair(1, mems, xs[1], ready, filler, 0,
                        _FIRST_STEP._replace(filler=_FIRST_STEP.filler + extra))

    def wind_down(self):
        k, seg, n_mem = self.k, self.k.seg, self.k.n_mem
        last = k.tile_ref.shape[0] - 1
        copies = [pltpu.make_async_copy(k.tile_ref.at[i], k.outt_hbm.at[:, _lane_tile(i)],
                                        self.sems.at[0]) for i in range(last + 1)]

        def step(x, mem, **options):
            out = self.single_step(_layernorm(x), mem, **options)
            return x + out[-seg:], out[:n_mem]

        _start(copies[:last - 1])
        mems, xs, filler, y = self.close_ffn()
        older = [self.old_ref[h] + y[h] for h in range(2)]
        x0, mem = step(older[0][:seg], mems[1], filler=itertools.islice(filler, 128), lead=48)
        _run(filler)
        passes, result = self.down()
        x1, mem = step(older[0][seg:], mem, filler=passes, lead=128)
        newer = [x + y for x, y in zip(xs, result())]
        k.tile_ref[last - 1] = _stack([older[1], newer[1]]).T.astype(k.tile_ref.dtype)
        x2, mem = step(newer[0][:seg], mem)
        copies[last - 1].start()
        x3, _ = step(newer[0][seg:], mem, skip=n_mem)
        xs = [_stack([x0, x1]), _stack([x2, x3])]
        _run(self.gated([_layernorm(x) for x in xs]))
        passes, result = self.down()
        _run(passes)
        k.tile_ref[last] = (_stack(xs) + _stack(result())).T.astype(k.tile_ref.dtype)
        copies[last].start()
        _wait(copies)


def _kernel(*refs, seg):
    kernel = _Kernel(seg, *refs)
    d_model, rows = _UNITS * _UNIT, kernel.n_mem + seg

    def run_layers(*scratch):
        layers = _Layers(kernel, *scratch)
        layers.ramp_up()
        pl.loop(2, kernel.n_pairs)(layers.steady)
        layers.wind_down()

    pl.run_scoped(
        kernel.start_up,
        *[pltpu.VMEM((_HEADS.n_tiles // 2, d_model, _LANES), jnp.uint32)] * 2,
        pltpu.SemaphoreType.DMA((3 + len(_QUERY_CUTS),)))
    pl.run_scoped(
        run_layers,
        pltpu.VMEM((d_model // 2, _HIDDEN.n_tiles * _LANES), jnp.uint32),
        pltpu.VMEM((_HIDDEN.n_tiles, 2, 2 * seg, _LANES), jnp.float32),
        pltpu.VMEM((2, _UNITS + 1, rows, _LANES), jnp.float32),
        *[pltpu.VMEM((2, 2 * seg, d_model), jnp.float32)] * 2,
        pltpu.VMEM((2, seg, d_model), jnp.float32),
        pltpu.VMEM((_LAG, seg, d_model), jnp.float32),
        pltpu.SemaphoreType.DMA((2,)))


@functools.partial(jax.jit, static_argnames=("A_seg_len",))
def pallas_interleave_layers__memory_aug_recurrent_mem_tr__glu_gated_swiglu__prompt_kernel(
    A_x: jax.Array,
    A_mem0: jax.Array,
    A_Wq: jax.Array,
    A_Wk: jax.Array,
    A_Wv: jax.Array,
    A_Wo: jax.Array,
    A_seg_len: int,
    B_x: jax.Array,
    B_w1: jax.Array,
    B_w3: jax.Array,
    B_w2: jax.Array,
):
    del B_x
    _, n_tok, d_model = A_x.shape
    n_mem, d_ff = A_mem0.shape[1], B_w1.shape[1]
    assert A_x.shape[0] == 1 and _LAG * A_seg_len == _LANES and 2 * n_mem == _PACKED
    assert A_Wq.shape == (_UNITS * _UNIT, _HEADS.n_tiles, _LANES) and n_tok % _LANES == 0
    assert d_ff == _HIDDEN.n_tiles * _LANES
    hbm = pl.BlockSpec(memory_space=pltpu.HBM)
    out_t = pl.pallas_call(
        functools.partial(_kernel, seg=A_seg_len),
        out_shape=jax.ShapeDtypeStruct((d_model, n_tok), A_x.dtype),
        in_specs=[hbm] * 9,
        out_specs=hbm,
        scratch_shapes=[
            pltpu.VMEM((8, n_mem, d_model), A_mem0.dtype),
            pltpu.VMEM((n_tok // _LANES, d_model, _LANES), A_x.dtype),
            pltpu.VMEM((n_tok, d_model), jnp.float32),
            pltpu.VMEM((4 * len(_HEADS.weights) * _LANES, _LANES), jnp.bfloat16),
            pltpu.VMEM((3 * len(_UP_PLAN) * _LANES, _LANES), jnp.bfloat16),
            pltpu.VMEM((_HEADS.n_tiles, d_model // 2, _LANES), jnp.uint32),
            *[pltpu.VMEM((2, _UNITS, 8, d_ff), jnp.uint32)] * 2,
            *[pltpu.VMEM((_HEADS.n_tiles * (n_tok // 4 + 2 * (_PACKED + A_seg_len)), _LANES),
                         jnp.bfloat16)] * 3,
            pltpu.SMEM((2,), jnp.int32),
            pltpu.SemaphoreType.DMA((_LAG + 1,)),
        ],
        compiler_params=pltpu.CompilerParams(vmem_limit_bytes=127 * 1024 * 1024),
    )(A_x.reshape(n_tok, d_model).T, A_mem0.reshape(n_mem, d_model), A_Wq, A_Wk, A_Wv,
      A_Wo.transpose(0, 2, 1), B_w1.reshape(_UNITS, _UNIT, d_ff),
      B_w3.reshape(_UNITS, _UNIT, d_ff), B_w2.T)
    return out_t.T.reshape(A_x.shape)
```

```python
import collections
import functools
import itertools
import math

import jax
import jax.numpy as jnp
import jax.experimental.pallas as pl
import jax.experimental.pallas.tpu as pltpu
import numpy as np

_EPS = 1e-05
_MASKED = -1000000000.0
_LOG2E = math.log2(math.e)
_LANES = 128
_MXUS = 4
_PACKED = 16
_UNIT = _LANES // 2
_UNITS = 9
_LAG = 4
_SCORE_SCALE = _LANES ** -0.5 * _LOG2E

_Timing = collections.namedtuple(
    "_Timing", "scores_at scores_gap filler rounds_at rounds_gap chores_gap")
_FIRST_STEP = _Timing(71, 72, 156, 19, 44, 10)
_SECOND_STEP = _Timing(75, 64, 183, 47, 64, 11)
_BARE_STEP = _Timing(71, 20, 0, 3, 16, 12)
_GATES_AT = 148
_GATES_INSIDE = 40
_GATES_AFTER = 71
_QUERY_CUTS = (0, 4, 8, 12, 16)
_OUTPUT_COPY_AT = 60
_OUTPUT_BUILD_AT = 140
_HELD_BACK = 32
_HEAD_CHORES = (0.6, 1.4, 0.6, 0.8)


def _sum(terms):
    terms = sorted(terms, key=lambda term: -term[0])
    return terms[0][1] if len(terms) == 1 and terms[0][0] == 1 else tuple(terms)


def _is_leaf(key):
    return isinstance(key[0], int)


def _leaves(key):
    return [key] if _is_leaf(key) else [leaf for _, term in key for leaf in _leaves(term)]


class _Scheme:
    def __init__(self, period, blocks, links, orient=tuple):
        self.period, self.n_links = period, len(links)
        links = [tuple((orbit, (s + shift) % period) for orbit, shift in link)
                 for s in range(period) for link in links]
        nodes = list(dict.fromkeys(node for link in links for node in link))
        links = [tuple(nodes.index(node) for node in link) for link in links]
        ways = [orbit // 2 for orbit, _ in nodes]
        blocks = [orient([u if u >= period else (u + s) % period for u in blocks[orbit]])
                  for orbit, s in nodes]
        cells, products, owner = [], {}, {}

        def form(side, tiles, p):
            if len(tiles) > (2 if p == 2 else 1):
                key = ((1, form(side, tiles[:-1], p)[1]), (1, form(side, tiles[-1:], p)[1]))
            elif p == 2:
                key = ((1, form(side, tiles, 0)[1]), (1 - 2 * side, form(side, tiles, 1)[1]))
            else:
                key = (p, blocks[tiles[0]]) if side == 0 else (1 - p, tiles[0])
            return (-1 if p == 2 * (1 - side) else 1), key

        def use(narrow, wide, sign):
            weight = products.setdefault((narrow[1], wide[1]), {})
            weight[len(cells) - 1] = sign * narrow[0] * wide[0]

        def cross(u, v, both, p):
            q, r = (p + 1) % 3, (p + 2) % 3
            mixed = []
            for side in range(2):
                (s, a), (t, b) = form(side, u, q), form(side, v, p)
                mixed.append((s, ((1, a), (-s * t, b))))
            for cell, sign in (((u, v), 1), ((v, u), -1)):
                cells.append(cell)
                for tiles, pair in ((both, (p, q)), (u, (r, q)), (v, (p, r))):
                    i, j = pair[::sign]
                    use(form(0, tiles, i), form(1, tiles, j), sign)
                use(*mixed, sign)

        for i, link in enumerate(links):
            for x in link:
                if ((x,), (x,)) not in cells:
                    cells.append(((x,), (x,)))
                    for sign in (1, -1):
                        use(form(0, (x,), (ways[x] + sign) % 3),
                            form(1, (x,), (ways[x] - sign) % 3), sign)
            before = len(cells)
            cross(link[:1], link[1:2], link[:2], 0)
            if len(link) == 3 and ways[link[2]]:
                cross(link[2:], link[:2], link, 1)
            elif len(link) == 3:
                cross(link[:2], link[2:], link, 2)
            owner.update(dict.fromkeys(range(before, len(cells)), i))
        self.products = [(j, narrow, wide) for j, (narrow, wide) in enumerate(products)]
        self.links = [[owner[j] for j in weight if j in owner] for weight in products.values()]

        sums = list(products.values())
        own = [products[form(0, (x,), 1 - ways[x])[1], form(1, (x,), 2)[1]]
               for x in range(len(nodes))]
        self.single = []
        for j, (rows, cols) in enumerate(cells):
            weight = own[rows[0]] if rows == cols else {j: -1} if {j: -1} in sums else {j: 1}
            if weight not in sums:
                sums.append(weight)
            if rows != cols:
                rows, cols = (rows + cols[:len(cols) == 1 and j in own[cols[0]]],
                              cols + rows[:len(rows) == 1 and j in own[rows[0]]])
            self.single.append((sums.index(weight), form(0, rows, 0)[1],
                                ((weight[j], form(1, cols, 1)[1]),)))

        basis = np.zeros((_UNITS, len(nodes), len(cells), 2))
        for j, (rows, cols) in enumerate(cells):
            for x, y, lane in itertools.product(rows, cols, range(2)):
                basis[blocks[x][lane], y, j, lane] += 1
        basis = basis.reshape(2 * len(cells), -1)
        inverse = np.clip(np.rint(np.linalg.inv(basis)), -1, 1)
        assert (inverse @ basis == np.eye(len(basis))).all()
        raw = [[_sum((int(half[u, x]), (int(u), int(x))) for u, x in np.argwhere(half))
                for half in cell] for cell in inverse.reshape(len(cells), 2, _UNITS, -1)]
        self.weights = [[_sum((sign, raw[j][lane]) for j, sign in weight.items())
                         for lane in range(2)] for weight in sums]
        self.n_tiles = len(nodes)
        self.places = sorted({(u, lane) for block in blocks for lane, u in enumerate(block)})

    def last_tile(self, j):
        return max(x for key in self.weights[j] for _, x in _leaves(key))

    def plan(self, step, pick, visits):
        rank = {(s * step + shift) % self.period * self.n_links + link: (s, i)
                for s in range(self.period) for i, (link, shift) in enumerate(visits)}

        def position(product):
            ranks = sorted(rank[i] for i in dict.fromkeys(self.links[product[0]]))
            return ranks[min(pick, len(ranks) - 1)], (len(ranks) > 1) == (pick > 0)

        return sorted(self.products, key=position)


def _by_parity(block):
    low, high = sorted(block)
    if high == _UNITS - 1:
        return (high, low) if low % 2 else (low, high)
    return (low, high) if high % 2 else (high, low)


_HEADS = _Scheme(8, ((7, 0), (7, 3), (8, 6), (5, 6)),
                 (((0, 6), (2, 6), (0, 3)), ((0, 6), (3, 4)), ((1, 1), (3, 4)),
                  ((1, 1), (3, 1), (2, 5)), ((1, 1), (2, 7))))
_HIDDEN = _Scheme(9, ((0, 3), (3, 2), (6, 5), (5, 8)),
                  (((0, 3), (2, 3), (0, 4)), ((0, 3), (3, 2)), ((1, 3), (3, 3), (3, 2)),
                   ((1, 3), (2, 4)), ((1, 0), (2, 4))), _by_parity)
_IN_ORDER = tuple((link, 0) for link in range(5))
_SWEEP_PLAN = _HEADS.plan(1, 2, _IN_ORDER)
_QKV_PLAN = _HEADS.plan(1, 0, ((1, 0), (2, 0), (3, 0), (4, 0), (0, 1)))
_OUTPUT_PLAN = _HEADS.plan(1, 2, ((1, 4), (2, 4), (3, 4), (4, 4), (0, 5)))
_UP_PLAN = _HIDDEN.plan(1, 2, _IN_ORDER)
_DOWN_PLAN = _HIDDEN.plan(5, 2, ((1, 8), (2, 8), (0, 3), (3, 6), (4, 0)))


def _add(total, sign, value):
    if total is None:
        return value if sign > 0 else -value
    return total + value if sign > 0 else total - value


def _gather(leaf):
    @functools.lru_cache(maxsize=None)
    def value(key):
        if _is_leaf(key):
            return leaf(*key)
        total = None
        for sign, term in key:
            total = _add(total, sign, value(term))
        return total

    return value


def _scatter(keys, done):
    missing, totals = {}, {}

    def count(key):
        missing[key] = missing.get(key, 0) + 1
        if missing[key] == 1 and not _is_leaf(key):
            for _, term in key:
                count(term)

    def add(key, value, sign=1):
        if key in totals:
            old_sign, old = totals[key]
            if old_sign >= sign:
                sign, value = old_sign, _add(old, sign * old_sign, value)
            else:
                value = value - old
        totals[key] = sign, value
        missing[key] -= 1
        if missing[key]:
            return
        if _is_leaf(key):
            done(*key, _add(None, sign, value))
        else:
            for factor, term in key:
                add(term, value, sign * factor)

    for key in keys:
        count(key)
    return add


def _stack(parts):
    return parts[0] if len(parts) == 1 else jnp.concatenate(parts, axis=0)


def _join(low, high):
    return low if low is high else jnp.concatenate([low[:, :_UNIT], high[:, _UNIT:]], axis=1)


def _swap(x):
    return jnp.concatenate([x[:, _UNIT:], x[:, :_UNIT]], axis=1)


def _dot(a, b):
    return jax.lax.dot_general(a, b, (((1,), (0,)), ((), ())),
                               preferred_element_type=jnp.float32)


def _operands(sets, dtype):
    @functools.lru_cache(maxsize=None)
    def tile(h, i, swapped):
        if i == _UNITS // 2:
            return jnp.concatenate([sets[h][:, -_UNIT:]] * 2, axis=1)
        return _swap(tile(h, i, 0)) if swapped else sets[h][:, i * _LANES:(i + 1) * _LANES]

    value = _gather(lambda h, block: _join(
        *[tile(h, unit // 2, (unit + lane) % 2) for lane, unit in enumerate(block)]))
    return functools.lru_cache(maxsize=None)(lambda key: value(key).astype(dtype))


def _expand(plan, lhs, weight, n_sets, done):
    parts = {}

    def finished(h, x, value):
        parts[h, x] = value
        if all((i, x) in parts for i in range(n_sets)):
            done(x, [parts[i, x] for i in range(n_sets)])

    add = _scatter([wide for _, _, wide in plan], finished)
    for j, narrow, wide in plan:
        product = _dot(lhs(narrow), weight(j))
        add(wide, product)
        yield product


def _reduce(plan, tile, weight, totals, dtype):
    def finished(h, block, value):
        for lane, unit in enumerate(block):
            totals[h][unit, lane] = _add(totals[h].get((unit, lane)), 1, value)

    lhs = _gather(tile)
    add = _scatter([narrow for _, narrow, _ in plan], finished)
    for j, narrow, wide in plan:
        product = _dot(lhs(wide).astype(dtype), weight(j))
        add(narrow, product)
        yield product


def _fold(totals):
    tiles = {}
    for unit, lane in sorted(totals):
        x = totals[unit, lane]
        if lane == 0:
            tiles[unit // 2, unit % 2] = _join(x, totals[unit ^ 1, 1] if unit < _UNITS - 1 else x)
        elif unit == _UNITS - 1:
            tiles[unit // 2, 1] = x
        else:
            assert (unit ^ 1, 0) in totals
    return tiles


def _merge(tiles):
    out = [tiles[i, 0] + _swap(tiles[i, 1]) if (i, 1) in tiles else tiles[i, 0]
           for i in range(_UNITS // 2 + 1)]
    return jnp.concatenate(out[:-1] + [out[-1][:, :_UNIT]], axis=1)


def _run(main, side=(), first=0, every=1):
    side = iter(side)
    for i, _ in enumerate(main):
        if i >= first and (i - first) % every == 0:
            next(side, None)
    for _ in side:
        pass


def _take(items, n):
    _run(itertools.islice(items, n))


def _layernorm(x):
    m = jnp.mean(x, axis=-1, keepdims=True)
    d = x - m
    v = jnp.mean(d * d, axis=-1, keepdims=True)
    return d * jax.lax.rsqrt(v + _EPS)


def _reciprocal(x):
    return pltpu.reciprocal(x, approx=True)


def _unpack(words):
    return pltpu.bitcast(words, jnp.bfloat16)


class _Tiles:
    def __init__(self, ref, rows=_LANES, first=0):
        self.ref, self.rows, self.first = ref, rows, first

    def shifted(self, by, limit, step):
        view = pl.ds(pl.multiple_of(by * step, step), self.ref.shape[0] - limit * step)
        return _Tiles(self.ref.at[view], self.rows, self.first)

    def load_words(self, j, rows=None, at=0):
        start = (self.first + j * self.rows + at) // 2
        return self.ref.bitcast(jnp.uint32)[pl.ds(start, (rows or self.rows) // 2), :]

    def store_words(self, j, words, at=0):
        start = (self.first + j * self.rows + at) // 2
        self.ref.bitcast(jnp.uint32)[pl.ds(start, words.shape[0]), :] = words

    def load(self, j, rows=None):
        return _unpack(self.load_words(j, rows))

    def store(self, j, value, at=0):
        start = self.first + j * self.rows + at
        self.ref[pl.ds(start, value.shape[0]), :] = value.astype(jnp.bfloat16)


class _Pacer:
    def __init__(self, zero):
        self.zero, self.after = zero.astype(jnp.uint32), None

    def hold(self, words):
        if self.after is None:
            return words
        return words | _stack([self.after] * (words.shape[0] // 8))

    def hold_rows(self, x):
        zeros = pltpu.bitcast(self.after, jnp.float32)
        return x + jnp.concatenate([zeros] * (_UNITS // 2) + [zeros[:, :_UNIT]], axis=1)

    def spread(self, passes, chores, rate):
        for i, product in enumerate(passes):
            count = int((i + 1) * rate) - int(i * rate)
            if count:
                self.after = pltpu.bitcast(product[:8], jnp.uint32) & self.zero
                _take(chores, count)
            yield product


def _build_rows(tiles, scheme, chosen, words):
    value = _gather(lambda u, x: _unpack(words(u, x)).astype(jnp.float32))
    for j in chosen:
        for lane, key in enumerate(scheme.weights[j]):
            if _is_leaf(key):
                tiles.store_words(j, words(*key), lane * _UNIT)
            else:
                tiles.store(j, value(key), lane * _UNIT)
        yield


def _build_transposed(tiles, scheme, chosen, words, pacer):
    for j in chosen:
        halves = scheme.weights[j]

        def rows(*key):
            return pacer.hold(words(*key)) if key == _leaves(halves[0])[0] else words(*key)

        if all(_is_leaf(key) for key in halves):
            tile = _unpack(_stack([rows(*key) for key in halves]))
        else:
            value = _gather(lambda u, x: _unpack(rows(u, x)).astype(jnp.float32))
            tile = _stack([value(key) for key in halves]).astype(jnp.bfloat16)
        tiles.store_words(j, pltpu.bitcast(tile.T, jnp.uint32))
        yield


def _unit_words(u):
    return slice(u * _UNIT // 2, (u + 1) * _UNIT // 2)


def _lane_tile(i):
    return pl.ds(i * _LANES, _LANES)


def _used(plan):
    return list(dict.fromkeys(x for _, _, wide in plan for _, x in _leaves(wide)))


def _start(copies):
    for c in copies:
        c.start()


def _wait(copies):
    for c in copies:
        c.wait()


def _attention_rounds(tokens, memories, n_mem, seg, shared, out):
    rows = n_mem + seg
    lane = jax.lax.broadcasted_iota(jnp.int32, (rows, _LANES), 1)
    row = jax.lax.broadcasted_iota(jnp.int32, (rows, _LANES), 0)
    visible = (row < n_mem) | (lane >= 3 * seg) | (row - n_mem >= lane % seg)
    upper = jax.lax.broadcasted_iota(jnp.int32, (n_mem, _LANES), 0) < n_mem // 2
    zeros, lowest, masked = [jnp.full((rows, _LANES), value, jnp.float32)
                             for value in (0.0, -jnp.inf, _MASKED * _LOG2E)]
    select = jax.lax.select

    @functools.lru_cache(maxsize=None)
    def window(i, slot, n=rows):
        j = jax.lax.broadcasted_iota(jnp.int32, (n, _LANES), 1)
        at = 3 * seg + slot * n_mem
        return ((j >= i * seg) & (j < (i + 1) * seg)) | ((j >= at) & (j < at + n_mem))

    def windows(triple):
        slots = (0, 1, 2 + triple[2][1])
        return slots, [window(i, slot) for i, slot in enumerate(slots)]

    def stacked(which, triple):
        return ([tokens(which, *problem) for problem in triple]
                + [memories(which, triple[0][0]), memories(which, triple[2][0])])

    def query(x, layer):
        mem = _unpack(memories(0, x)).astype(jnp.float32)[layer * n_mem:(layer + 1) * n_mem]
        return _stack([mem, _unpack(tokens(0, x, layer)).astype(jnp.float32)])

    def by_rows(slots, piece):
        parts = [piece(i, i) for i in range(3)]
        for pair in range(2):
            a, b = [piece(slots.index(slot) if slot in slots else None, 3 + pair)
                    for slot in (2 * pair, 2 * pair + 1)]
            parts.append(a if a is b else select(upper, a, b))
        return _unpack(_stack(parts))

    def pick(inside, parts):
        a, b, c = [jnp.broadcast_to(part, zeros.shape) for part in parts]
        return select(inside[0], a, select(inside[1], b, c))

    def softmax(inside, s):
        s = select(visible, s * _SCORE_SCALE, masked)
        p = jnp.exp2(s - pick(inside, [
            jnp.max(select(k, s, lowest), axis=-1, keepdims=True) for k in inside]))
        return p * _reciprocal(pick(inside, [
            jnp.sum(select(k, p, zeros), axis=-1, keepdims=True) for k in inside]))

    def keys(triple):
        return pltpu.bitcast(_unpack(_stack(stacked(1, triple))).T, jnp.uint32)

    def scores(triple, n=3):
        kt = _unpack(keys(triple))
        parts = [_dot(query(*problem), kt) for problem in triple[:n]]
        inside = windows(triple)[1]
        return softmax(inside, pick(inside, parts + parts[:3 - n]))

    def values(triple, p, n=3):
        v = _unpack(_stack(stacked(2, triple)))
        for problem, k in zip(triple[:n], windows(triple)[1]):
            out[problem] = _dot(select(k, p, zeros), v)

    def both(triple, earlier, p):
        slots, inside = windows(triple)
        assert slots == windows(earlier)[0]
        kt, v, q = keys(triple), stacked(2, earlier), [query(*problem) for problem in triple]

        ends = list(itertools.accumulate([0] + [part.shape[0] for part in v]))
        parts = ([kt[a:b] for a, b in zip(ends, ends[1:])], v)
        blank = {part.shape: jnp.zeros_like(part) for part in (v[0], v[-1])}

        @functools.lru_cache(maxsize=None)
        def columns(which, part, i, keep=True):
            words = parts[which][part]
            if i is None:
                return blank[words.shape]
            pair = (words, blank[words.shape])
            return select(window(i, slots[i], words.shape[0]), *pair[::1 if keep else -1])

        s = _dot(pick(inside, q), by_rows(slots, lambda i, part: columns(0, part, i)))
        o = _dot(select(inside[0] | inside[1] | inside[2], p, zeros),
                 by_rows(slots, lambda i, part: columns(1, part, i)))
        mixed = [_dot(select(inside[i], p, q[i]), by_rows(
            slots, lambda j, part: columns(1, part, i, False) if j == i else columns(0, part, i)))
                 for i in range(3)]
        for problem, k, x in zip(earlier, inside, mixed):
            out[problem] = select(k, o, x)
        return softmax(inside, s + pick(inside, mixed))

    order = _used(_OUTPUT_PLAN)
    pairs = [((x, 0), (x, 1), (x, 0)) for x in order[:2]]
    triples = [((order[i + 2 * layer], 0), (order[i + 2 * layer], 1), (order[i + 1], layer))
               for i in range(2, len(order), 3) for layer in range(2)]
    rounds = [triples[i:i + _MXUS] for i in range(0, len(triples), _MXUS)]
    first = [scores(pair, 2) for pair in pairs]
    yield
    waiting = []
    for group in rounds[:1] if shared else rounds:
        waiting.append([(triple, scores(triple)) for triple in group])
        yield
    for pair, p in zip(pairs, first):
        values(pair, p, 2)
    for group in rounds[len(waiting):]:
        waiting = [[(triple, both(triple, *done)) for triple, done in zip(group, waiting[0])]]
        yield
    for group in waiting:
        for done in group:
            values(*done)
        yield


class _Kernel:
    def __init__(self, seg, xt_hbm, mem0_hbm, wq_hbm, wk_hbm, wv_hbm, wot_hbm, w1_hbm, w3_hbm,
                 w2t_hbm, outt_hbm, mem0_ref, tile_ref, x_ref, attention_ref, ffn_ref, wo_ref,
                 w1_ref, w3_ref, q_ref, k_ref, v_ref, count_ref, sems):
        self.seg, self.n_mem = seg, mem0_hbm.shape[0]
        self.n_pairs = (x_ref.shape[0] // seg - _LAG) // 2
        self.n_first = 1 + pl.cdiv(self.n_pairs * _PACKED, _LANES)
        self.xt_hbm, self.outt_hbm, self.wot_hbm, self.w2t_hbm = xt_hbm, outt_hbm, wot_hbm, w2t_hbm
        self.qkv_hbm, self.up_hbm = (wq_hbm, wk_hbm, wv_hbm), (w1_hbm, w3_hbm)
        self.mem0_ref, self.tile_ref, self.x_ref = mem0_ref, tile_ref, x_ref
        self.wo_ref, self.up_refs, self.sems = wo_ref, (w1_ref, w3_ref), sems
        self.attention, self.ffn = [
            [_Tiles(ref, _LANES, i * ref.shape[0] // n) for i in range(n)]
            for ref, n in ((attention_ref, 4), (ffn_ref, 3))]
        ring = (self.n_pairs + 2) * _PACKED
        self.ahead = [_Tiles(ref, _PACKED) for ref in (q_ref, k_ref, v_ref)]
        self.current = [_Tiles(ref, _PACKED + seg, _HEADS.n_tiles * ring)
                        for ref in (q_ref, k_ref, v_ref)]
        self.mem_copy = pltpu.make_async_copy(mem0_hbm, mem0_ref.at[0], sems.at[_LAG])

        @pl.loop(0, count_ref.shape[0])
        def _(i):
            count_ref[i] = i

        self.zero = count_ref[0]

    def x_copy(self, i, sem):
        return pltpu.make_async_copy(self.xt_hbm.at[:, _lane_tile(i)], self.tile_ref.at[i], sem)

    def up_copies(self, r):
        rows = pl.ds(pl.multiple_of(r * 8, 8), 8)
        return [pltpu.make_async_copy(src.bitcast(jnp.uint32).at[:, rows, :], dst.at[r % 2],
                                      self.sems.at[r])
                for src, dst in zip(self.up_hbm, self.up_refs)]

    def put_ahead(self, which, x, value, at):
        for r in range(0, value.shape[0], _PACKED):
            self.ahead[which].store((at + r) // _PACKED * _HEADS.n_tiles + x, value[r:r + _PACKED])

    def build_output(self, chosen, pacer):
        return _build_transposed(self.attention[3], _HEADS, chosen,
                                 lambda u, x: self.wo_ref[x, _unit_words(u), :], pacer)

    def start_up(self, even_ref, odd_ref, sems):
        stages = (even_ref, odd_ref, even_ref)
        rows = self.n_pairs * _PACKED // 2
        pacer = _Pacer(self.zero)

        def pair_copy(which, p, sem):
            return pltpu.make_async_copy(self.qkv_hbm[which].bitcast(jnp.uint32).at[:, p, :],
                                         stages[which].at[p], sems.at[sem])

        def build(which, j, hold=lambda words: words):
            def raw(u, x):
                words = hold(stages[which][x // 2, u * _UNIT:(u + 1) * _UNIT, :])
                return pltpu.bitcast(words & jnp.uint32(0xFFFF0000) if x % 2 else words << 16,
                                     jnp.float32)

            self.attention[which].store(j, _stack(list(map(_gather(raw), _HEADS.weights[j]))))

        def sweep(which, plan, n=rows):
            def lhs(key):
                if key not in slots:
                    slots[key] = len(slots)
                    sums.store(slots[key], fresh(key))
                return sums.load(slots[key], n)

            def weight(j):
                build(which, j)
                return self.attention[which].load(j)

            def done(x, sets):
                for h, value in enumerate(sets):
                    self.put_ahead(which, x, value, h * rows)

            chores = (build(which, j, pacer.hold)
                      for j in range(len(plan), len(_HEADS.weights)))
            return _expand(plan, lhs, weight, 2, done), chores

        def chunk(product):
            return sum(cut <= _HEADS.last_tile(product[0]) // 2 for cut in _QUERY_CUTS[1:])

        queue = [[self.x_copy(i, sems.at[0]) for i in range(1, self.n_first)]]
        queue += [[pair_copy(0, p, 4 + c) for p in range(a, b)]
                  for c, (a, b) in enumerate(zip(_QUERY_CUTS, _QUERY_CUTS[1:]))]
        queue += [[pair_copy(1, p, 1) for p in range(odd_ref.shape[0])]]

        def advance():
            _wait(queue.pop(0))
            for copies in queue[1:2]:
                _start(copies)

        _start(queue[0] + queue[1])
        advance()
        x = _stack([self.tile_ref[i].astype(jnp.float32).T for i in range(1, self.n_first)])
        self.x_ref[pl.ds(_LANES, x.shape[0]), :] = x
        normed = _layernorm(x[:2 * rows])
        fresh, slots = _operands([normed[:rows], normed[rows:]], jnp.float32), {}
        sums = _Tiles(self.ffn[0].ref, rows)

        plan = sorted(_SWEEP_PLAN, key=chunk)
        passes, chores = sweep(0, plan)
        for c in range(len(_QUERY_CUTS) - 2):
            advance()
            _take(passes, sum(chunk(product) <= c for product in plan) // _MXUS * _MXUS
                  - sum(chunk(product) < c for product in plan) // _MXUS * _MXUS)
        advance()
        _run(pacer.spread(passes, chores, 0.5))
        _run(chores)

        advance()
        pl.loop(0, even_ref.shape[0])(lambda p: pair_copy(2, p, 2).start())
        output_copies = [
            pltpu.make_async_copy(self.wot_hbm.bitcast(jnp.uint32), self.wo_ref, sems.at[3]),
            self.x_copy(0, sems.at[3])]
        passes, chores = sweep(1, _SWEEP_PLAN)
        passes = pacer.spread(passes, chores, 0.25)
        _take(passes, _OUTPUT_COPY_AT)
        _start(output_copies)
        _run(passes)
        _run(chores)

        pl.loop(0, even_ref.shape[0])(lambda p: pair_copy(2, p, 2).wait())
        passes, chores = sweep(2, _SWEEP_PLAN, rows - _HELD_BACK)
        _take(pacer.spread(passes, chores, 0.5), _OUTPUT_BUILD_AT)
        _run(chores)
        _wait(output_copies)
        _start([self.mem_copy] + self.up_copies(0) + self.up_copies(1))
        self.x_ref[:_LANES, :] = self.tile_ref[0].astype(jnp.float32).T
        chores = self.build_output([j for j, _, _ in _HEADS.single], pacer)
        _run(pacer.spread(passes, chores,
                          len(_HEADS.single) / (len(plan) - _OUTPUT_BUILD_AT - _MXUS)))
        _run(chores)
        self.mem_copy.wait()


class _Layers:
    def __init__(self, kernel, w2_ref, act_ref, out_ref, pair_ref, old_ref,
                 normed_ref, rows_ref, sems):
        self.k = kernel
        self.w2_ref, self.act_ref, self.out_ref, self.sems = w2_ref, act_ref, out_ref, sems
        self.pair_ref, self.old_ref = pair_ref, old_ref
        self.normed_ref, self.rows_ref = normed_ref, rows_ref
        self.folded = list(_fold(dict.fromkeys(_HEADS.places)))
        self.pacer = _Pacer(kernel.zero)

    def gated(self, sets):
        lhs = _operands(sets, jnp.bfloat16)
        gates = {}

        def gate(x, parts):
            gates[x] = parts

        def up(x, parts):
            for h, g in enumerate(gates[x]):
                self.act_ref[x, h] = g * _reciprocal(1.0 + jnp.exp2(g * -_LOG2E)) * parts[h]

        yield from _expand(_UP_PLAN, lhs, self.k.ffn[0].load, 2, gate)
        yield from _expand(_UP_PLAN, lhs, self.k.ffn[1].load, 2, up)

    def down(self):
        totals = [{}, {}]
        passes = _reduce(_DOWN_PLAN, lambda h, x: self.act_ref[x, h], self.k.ffn[2].load,
                         totals, jnp.bfloat16)
        return passes, lambda: [_merge(_fold(t)) for t in totals]

    def single_step(self, normed, mem, filler=(), lead=0, skip=0, pace=lambda which, p: p):
        plan, weights = _HEADS.single, self.k.attention
        lhs = _operands([_stack([mem, normed])], jnp.float32)
        shape = (mem.shape[0] + normed.shape[0] - skip, mem.shape[0] + normed.shape[0])
        i = jax.lax.broadcasted_iota(jnp.int32, shape, 0) + skip
        visible = (i < mem.shape[0]) | (i >= jax.lax.broadcasted_iota(jnp.int32, shape, 1))
        qkv, probs, heads, totals = {}, {}, {}, {}

        def project(which):
            def keep(x, parts):
                qkv[which, x] = parts[0].astype(jnp.bfloat16) if which else parts[0]

            rows = (lambda key: lhs(key)[skip:]) if skip and not which else lhs
            return pace(which, _expand(plan, rows, weights[which].load, 1, keep))

        def scores():
            for x in _used(plan):
                s = jax.lax.dot_general(qkv[0, x], qkv[1, x], (((1,), (1,)), ((), ())),
                                        preferred_element_type=jnp.float32)
                s = jnp.where(visible, s * _SCORE_SCALE, _MASKED * _LOG2E)
                p = jnp.exp2(s - jnp.max(s, axis=-1, keepdims=True))
                probs[x] = p * _reciprocal(jnp.sum(p, axis=-1, keepdims=True))
                if len(probs) % _MXUS == 0:
                    yield

        def values():
            for x in _used(plan):
                heads[x] = _dot(probs[x], qkv[2, x])
                if len(heads) % _MXUS == 0:
                    yield

        def head(h, x):
            while x not in heads:
                next(rounds)
            return heads[x]

        rounds = values()
        output = pace(3, _reduce(plan, head, weights[3].load, [totals], jnp.float32))
        _run(project(0))
        _run(project(1))
        _run(itertools.chain(itertools.islice(filler, lead), project(2)), scores(), 15,
             (len(plan) + lead - 16) // _HEADS.n_tiles * _MXUS)
        if lead:
            _run(itertools.chain(filler, output), rounds, 15, 8)
        else:
            _take(rounds, 3)
            _run(output, rounds, 3, 8)
        return _merge(_fold(totals))

    def double_step(self, j, second, mems, x2, timing, filler, pace):
        k, seg, n_mem = self.k, self.k.seg, self.k.n_mem
        put = k.n_pairs + 3 * j + second
        x1 = k.x_ref[pl.ds(pl.multiple_of(_LANES + put * _PACKED, _PACKED), (1 + second) * _PACKED), :]
        normed = _stack([_layernorm(x1), _layernorm(x2)])
        half = normed.shape[0] // 2
        lhs = _operands([_stack([mems[0], normed[:half]]), _stack([mems[1], normed[half:]])],
                        jnp.float32 if (n_mem + half) % _PACKED else jnp.bfloat16)
        size, step = k.n_pairs + 2, _HEADS.n_tiles * _PACKED
        later = [[ring.shifted((put + i) % size, size - 1, step) for ring in k.ahead]
                 for i in range(1 + second)]
        now = [ring.shifted((4 * j + 2 * second) % size, size - 2, step) for ring in k.ahead]
        base = second * _HEADS.n_tiles
        heads, totals = {}, [{}, {}]

        def project(which):
            def keep(x, parts):
                rows = _stack([p[n_mem:] for p in parts])
                k.current[which].store(base + x, _stack([p[:n_mem] for p in parts] + [rows[-seg:]]))
                for i, rings in enumerate(later):
                    rings[which].store(x, rows[i * _PACKED:(i + 1) * _PACKED])

            return pace(which, _expand(_QKV_PLAN, lhs, k.attention[which].load, 2, keep))

        def tokens(which, x, layer):
            if layer:
                return k.current[which].load_words(base + x, seg, _PACKED)
            return _stack([now[which].load_words(i * _HEADS.n_tiles + x) for i in range(2)])

        def head(layer, x):
            while (x, layer) not in heads:
                next(rounds)
            return heads[x, layer]

        rounds = _attention_rounds(
            tokens, lambda which, x: k.current[which].load_words(base + x, _PACKED),
            n_mem, seg, timing.filler > 0, heads)
        _run(project(0))
        _run(project(1))
        _run(project(2), itertools.islice(rounds, 2 if timing.filler else 6),
             timing.scores_at, timing.scores_gap)
        output = _reduce(_OUTPUT_PLAN, head, k.attention[3].load, totals, jnp.float32)
        _run(itertools.chain(itertools.islice(filler, timing.filler), output), rounds,
             timing.rounds_at, timing.rounds_gap)
        return [_fold(t) for t in totals]

    def under_keys(self, chores, gap):
        def pace(which, passes):
            yield from self.pacer.spread(passes, chores, (which == 1) / gap)
            if which == 1:
                _run(chores)

        return pace

    def pair(self, j, mems, x2, filler, between, timings, pace):
        seg, n_mem = self.k.seg, self.k.n_mem
        x1 = self.k.x_ref[pl.ds(pl.multiple_of((2 * j + _LAG) * seg, seg), 2 * seg), :]
        out = [_merge(t) for t in self.double_step(j, 0, mems, x2[:seg], timings[0], filler, pace)]

        def park():
            for h, x in enumerate((x1, x2)):
                for r in range(0, seg, 8):
                    first = self.pacer.hold_rows(x[r:r + 8]) + out[h][n_mem + r:n_mem + r + 8]
                    self.pair_ref[h, r:r + 8, :] = first
                    self.normed_ref[h, r:r + 8, :] = _layernorm(first)
                    yield
                    rows = slice(seg + r, seg + r + 8)
                    self.pair_ref[h, rows, :] = self.pacer.hold_rows(x[rows])
                    yield

        _take(filler, between)
        tiles = self.double_step(j, 1, [o[:n_mem] for o in out], x2[seg:], timings[1], filler,
                                 self.under_keys(park(), timings[1].chores_gap))
        for h in range(2):
            for i, key in enumerate(self.folded):
                self.out_ref[h, i] = tiles[h][key]

    def finish_pair(self):
        seg, n_mem = self.k.seg, self.k.n_mem
        out = [_merge({key: self.out_ref[h, i] for i, key in enumerate(self.folded)})
               for h in range(2)]
        second = [self.pair_ref[h, seg:, :] + out[h][n_mem:] for h in range(2)]
        return ([o[:n_mem] for o in out],
                [_stack([self.pair_ref[h, :seg, :], second[h]]) for h in range(2)],
                self.gated([_stack([self.normed_ref[h], _layernorm(second[h])])
                            for h in range(2)]))

    def gated_pair(self, j, mems, x2, xs, filler, taken, first, final=None):
        def hand_over():
            for r in range(0, xs[0].shape[0], 8):
                if final is not None:
                    i, at = divmod(r, self.k.seg)
                    self.rows_ref[j % 2 * 2 + i, at:at + 8, :] = (
                        self.pacer.hold_rows(self.old_ref[1, r:r + 8, :]) + final[r:r + 8])
                for h in (1, 0):
                    self.old_ref[h, r:r + 8, :] = self.pacer.hold_rows(xs[h][r:r + 8])
                    yield
            if final is not None:
                rows = _stack([self.rows_ref[i] for i in range(_LAG)])
                self.k.tile_ref[j // 2 - 1] = rows.T.astype(self.k.tile_ref.dtype)

        between = 2 * len(_UP_PLAN) - taken - first.filler - _SECOND_STEP.filler
        assert between >= 0
        self.pair(j, mems, x2, filler, between, (first, _SECOND_STEP),
                  self.under_keys(hand_over(), first.chores_gap))

    def close_ffn(self):
        mems, xs, filler = self.finish_pair()
        passes, result = self.down()
        _take(passes, _GATES_AT)
        _take(filler, _GATES_INSIDE)
        _run(passes)
        y = result()
        _take(filler, _GATES_AFTER)
        return mems, xs, filler, y

    def steady(self, j):
        mems, xs, filler, y = self.close_ffn()
        self.gated_pair(j, mems, self.old_ref[0] + y[0], xs, filler,
                        _GATES_INSIDE + _GATES_AFTER, _FIRST_STEP, y[1])

    def ramp_up(self):
        k, seg, pacer = self.k, self.k.seg, self.pacer
        rest = range(k.n_first, k.tile_ref.shape[0])
        x_copies = [k.x_copy(i, self.sems.at[1]) for i in rest]
        half = self.w2_ref.shape[1] // 2
        w2_copies = [
            pltpu.make_async_copy(k.w2t_hbm.bitcast(jnp.uint32).at[:, pl.ds(i * half, half)],
                                  self.w2_ref.at[:, pl.ds(i * half, half)], self.sems.at[i])
            for i in range(2)]

        def head_step(r, mem):
            _wait(k.up_copies(r))
            pl.when((r > 0) & (r + 1 < _LAG))(lambda: _start(k.up_copies(r + 1)))
            pl.when(r + 2 == _LAG)(w2_copies[0].start)
            pl.when(r + 1 == _LAG)(lambda: _start(w2_copies[1:] + x_copies))
            local, slot = _Pacer(k.zero), r % 2
            chores = itertools.chain(*[
                _build_rows(tiles.shifted(r, _LAG - 1, _PACKED), _HIDDEN,
                            [j for j, _, _ in _UP_PLAN],
                            lambda u, x, ref=ref: local.hold(ref[slot, u, :, _lane_tile(x)]))
                for ref, tiles in zip(k.up_refs, k.ffn)])
            _take(chores, 30)
            rows = pl.ds(pl.multiple_of(r * seg, seg), seg)
            out = self.single_step(
                self.rows_ref[r], mem,
                pace=lambda which, passes: local.spread(passes, chores, _HEAD_CHORES[which]))
            _run(chores)
            k.x_ref[rows, :] = k.x_ref[rows, :] + out[k.n_mem:]
            return out[:k.n_mem]

        def held_back():
            ends = [(h + 1) * k.n_pairs * _PACKED // 2 - _HELD_BACK for h in range(2)]
            assert ends[0] >= 4 * seg

            def done(x, sets):
                for at, value in zip(ends, sets):
                    k.put_ahead(2, x, value, at)

            return _expand(_QKV_PLAN, _operands([self.normed_ref[h] for h in range(2)],
                                                jnp.bfloat16), k.attention[2].load, 2, done)

        def transpose_in():
            for i in rest:
                x = _unpack(pacer.hold(k.tile_ref.bitcast(jnp.uint32)[i]))
                k.x_ref[_lane_tile(i), :] = x.astype(jnp.float32).T
                yield

        mem0 = k.mem0_ref[0].astype(jnp.float32)
        for r in range(_LAG):
            self.rows_ref[r] = _layernorm(k.x_ref[pl.ds(r * seg, seg), :])
        for h in range(2):
            at = _LANES + (h + 1) * k.n_pairs * _PACKED // 2 - _HELD_BACK
            self.normed_ref[h] = _layernorm(k.x_ref[pl.ds(at, _HELD_BACK), :])
        mem1 = jax.lax.fori_loop(0, _LAG, head_step, mem0)

        def build_down(late):
            chosen = [j for j, _, _ in _DOWN_PLAN
                      if (_HIDDEN.last_tile(j) * _LANES >= half) == late]
            return _build_transposed(
                k.ffn[2], _HIDDEN, chosen,
                lambda u, x: self.w2_ref[_unit_words(u), _lane_tile(x)], pacer)

        _wait(w2_copies[:1])
        spare = held_back()
        xs = [k.x_ref[pl.ds(h * 2 * seg, 2 * seg), :] for h in range(2)]
        _take(spare, 56)
        passes, chores = self.gated([_layernorm(x) for x in xs]), build_down(False)
        _take(pacer.spread(passes, chores, 0.4), 260)
        _run(chores)
        _wait(w2_copies[1:] + x_copies)
        chores = build_down(True)
        _run(pacer.spread(passes, chores, 0.45))
        passes, result = self.down()
        _run(pacer.spread(passes, chores, 0.25))
        xs = [x + y for x, y in zip(xs, result())]

        _take(spare, 72)
        single = [j for j, _, _ in _HEADS.single]
        _run(k.build_output([j for j, _, _ in _OUTPUT_PLAN if j not in single], pacer))
        self.pair(0, [mem1, mem0], xs[0], spare, 52, (_BARE_STEP, _BARE_STEP),
                  self.under_keys(transpose_in(), 20))
        _run(spare)
        mems, ready, filler = self.finish_pair()
        extra = _GATES_INSIDE + _GATES_AFTER
        self.gated_pair(1, mems, xs[1], ready, filler, 0,
                        _FIRST_STEP._replace(filler=_FIRST_STEP.filler + extra))

    def wind_down(self):
        k, seg, n_mem = self.k, self.k.seg, self.k.n_mem
        last = k.tile_ref.shape[0] - 1
        copies = [pltpu.make_async_copy(k.tile_ref.at[i], k.outt_hbm.at[:, _lane_tile(i)],
                                        self.sems.at[0]) for i in range(last + 1)]

        def step(x, mem, **options):
            out = self.single_step(_layernorm(x), mem, **options)
            return x + out[-seg:], out[:n_mem]

        _start(copies[:last - 1])
        mems, xs, filler, y = self.close_ffn()
        older = [self.old_ref[h] + y[h] for h in range(2)]
        x0, mem = step(older[0][:seg], mems[1], filler=itertools.islice(filler, 128), lead=48)
        _run(filler)
        passes, result = self.down()
        x1, mem = step(older[0][seg:], mem, filler=passes, lead=128)
        newer = [x + y for x, y in zip(xs, result())]
        k.tile_ref[last - 1] = _stack([older[1], newer[1]]).T.astype(k.tile_ref.dtype)
        x2, mem = step(newer[0][:seg], mem)
        copies[last - 1].start()
        x3, _ = step(newer[0][seg:], mem, skip=n_mem)
        xs = [_stack([x0, x1]), _stack([x2, x3])]
        _run(self.gated([_layernorm(x) for x in xs]))
        passes, result = self.down()
        _run(passes)
        k.tile_ref[last] = (_stack(xs) + _stack(result())).T.astype(k.tile_ref.dtype)
        copies[last].start()
        _wait(copies)


def _kernel(*refs, seg):
    kernel = _Kernel(seg, *refs)
    d_model, rows = _UNITS * _UNIT, kernel.n_mem + seg

    def run_layers(*scratch):
        layers = _Layers(kernel, *scratch)
        layers.ramp_up()
        pl.loop(2, kernel.n_pairs)(layers.steady)
        layers.wind_down()

    pl.run_scoped(
        kernel.start_up,
        *[pltpu.VMEM((_HEADS.n_tiles // 2, d_model, _LANES), jnp.uint32)] * 2,
        pltpu.SemaphoreType.DMA((3 + len(_QUERY_CUTS),)))
    pl.run_scoped(
        run_layers,
        pltpu.VMEM((d_model // 2, _HIDDEN.n_tiles * _LANES), jnp.uint32),
        pltpu.VMEM((_HIDDEN.n_tiles, 2, 2 * seg, _LANES), jnp.float32),
        pltpu.VMEM((2, _UNITS + 1, rows, _LANES), jnp.float32),
        *[pltpu.VMEM((2, 2 * seg, d_model), jnp.float32)] * 2,
        pltpu.VMEM((2, seg, d_model), jnp.float32),
        pltpu.VMEM((_LAG, seg, d_model), jnp.float32),
        pltpu.SemaphoreType.DMA((2,)))


@functools.partial(jax.jit, static_argnames=("A_seg_len",))
def pallas_interleave_layers__memory_aug_recurrent_mem_tr__glu_gated_swiglu__prompt_kernel(
    A_x: jax.Array,
    A_mem0: jax.Array,
    A_Wq: jax.Array,
    A_Wk: jax.Array,
    A_Wv: jax.Array,
    A_Wo: jax.Array,
    A_seg_len: int,
    B_x: jax.Array,
    B_w1: jax.Array,
    B_w3: jax.Array,
    B_w2: jax.Array,
):
    del B_x
    _, n_tok, d_model = A_x.shape
    n_mem, d_ff = A_mem0.shape[1], B_w1.shape[1]
    assert A_x.shape[0] == 1 and _LAG * A_seg_len == _LANES and 2 * n_mem == _PACKED
    assert A_Wq.shape == (_UNITS * _UNIT, _HEADS.n_tiles, _LANES) and n_tok % _LANES == 0
    assert d_ff == _HIDDEN.n_tiles * _LANES
    hbm = pl.BlockSpec(memory_space=pltpu.HBM)
    out_t = pl.pallas_call(
        functools.partial(_kernel, seg=A_seg_len),
        out_shape=jax.ShapeDtypeStruct((d_model, n_tok), A_x.dtype),
        in_specs=[hbm] * 9,
        out_specs=hbm,
        scratch_shapes=[
            pltpu.VMEM((8, n_mem, d_model), A_mem0.dtype),
            pltpu.VMEM((n_tok // _LANES, d_model, _LANES), A_x.dtype),
            pltpu.VMEM((n_tok, d_model), jnp.float32),
            pltpu.VMEM((4 * len(_HEADS.weights) * _LANES, _LANES), jnp.bfloat16),
            pltpu.VMEM((3 * len(_UP_PLAN) * _LANES, _LANES), jnp.bfloat16),
            pltpu.VMEM((_HEADS.n_tiles, d_model // 2, _LANES), jnp.uint32),
            *[pltpu.VMEM((2, _UNITS, 8, d_ff), jnp.uint32)] * 2,
            *[pltpu.VMEM((_HEADS.n_tiles * (n_tok // 4 + 2 * (_PACKED + A_seg_len)), _LANES),
                         jnp.bfloat16)] * 3,
            pltpu.SMEM((2,), jnp.int32),
            pltpu.SemaphoreType.DMA((_LAG + 1,)),
        ],
        compiler_params=pltpu.CompilerParams(vmem_limit_bytes=127 * 1024 * 1024),
    )(A_x.reshape(n_tok, d_model).T, A_mem0.reshape(n_mem, d_model), A_Wq, A_Wk, A_Wv,
      A_Wo.transpose(0, 2, 1), B_w1.reshape(_UNITS, _UNIT, d_ff),
      B_w3.reshape(_UNITS, _UNIT, d_ff), B_w2.T)
    return out_t.T.reshape(A_x.shape)
```
